```python
import jax
import jax.numpy as jnp

def _softmax(x, axis=-1):
    return jax.nn.softmax(x, axis=axis)

def _gelu(x):
    return jax.nn.gelu(x, approximate=True)

def _silu(x):
    return jax.nn.silu(x)

def _sigmoid(x):
    return jax.nn.sigmoid(x)

def _layernorm(x, axis=-1, eps=1e-05):
    m = jnp.mean(x, axis=axis, keepdims=True)
    v = jnp.var(x, axis=axis, keepdims=True)
    return (x - m) / jnp.sqrt(v + eps)

def _scatter_add(tgt, idx, src, axis=0):
    return tgt.at[idx].add(src)

def _segment_sum(src, seg, n):
    return jax.ops.segment_sum(src, seg, n)

class _Rng:

    def __init__(self, key):
        self._k = key

    def _next(self):
        self._k, sub = jax.random.split(self._k)
        return sub

    def normal(self, shape):
        return jax.random.normal(self._next(), shape, dtype=jnp.bfloat16)

    def randint(self, lo, hi, shape):
        return jax.random.randint(self._next(), shape, lo, hi, dtype=jnp.int32)

    def uniform(self, shape, lo=0.0, hi=1.0):
        return jax.random.uniform(self._next(), shape, jnp.bfloat16, lo, hi)

    def permutation(self, n):
        return jax.random.permutation(self._next(), n)
kernel_name = 'recurrent_scan__memory_aug_recurrent_mem_tr__mixer_s_mlp__prompt'

def setup_inputs():
    _rng = _Rng(jax.random.key(int.from_bytes(__import__("os").urandom(4), "little")))
    _w = lambda a: (lambda t: t.astype(jnp.bfloat16) if jnp.issubdtype(t.dtype, jnp.floating) else t)(jnp.asarray(a))

    def _A_setup():
        B, S, Dm = (1, 2048, 1024)
        H, Dh = (32, 128)
        M, seg = (8, 32)
        seg = min(seg, S)
        S = S // seg * seg
        return {'x': _w((lambda *s: _rng.normal(s) * 0.05)(B, S, Dm)), 'mem0': _w((lambda *s: _rng.normal(s) * 0.05)(B, M, Dm)), 'Wq': _w((lambda *s: _rng.normal(s) * 0.05)(Dm, H, Dh) * Dm ** (-0.5)), 'Wk': _w((lambda *s: _rng.normal(s) * 0.05)(Dm, H, Dh) * Dm ** (-0.5)), 'Wv': _w((lambda *s: _rng.normal(s) * 0.05)(Dm, H, Dh) * Dm ** (-0.5)), 'Wo': _w((lambda *s: _rng.normal(s) * 0.05)(H, Dh, Dm) * (H * Dh) ** (-0.5)), 'seg_len': seg}
    _A_in = _A_setup()

    def _B_setup():
        B, S, D, F = (1, 2048, 1024, 3584)
        return {'x': _w((lambda *s: _rng.normal(s) * 0.05)(B, S, D)), 'w1': _w((lambda *s: _rng.normal(s) * 0.05)(D, D) * D ** (-0.5)), 'w2': _w((lambda *s: _rng.normal(s) * 0.05)(D, D) * D ** (-0.5)), 'w3': _w((lambda *s: _rng.normal(s) * 0.05)(D, F) * D ** (-0.5)), 'w4': _w((lambda *s: _rng.normal(s) * 0.05)(F, D) * F ** (-0.5))}
    _B_in = _B_setup()
    return {'A_x': _A_in['x'], 'A_mem0': _A_in['mem0'], 'A_Wq': _A_in['Wq'], 'A_Wk': _A_in['Wk'], 'A_Wv': _A_in['Wv'], 'A_Wo': _A_in['Wo'], 'A_seg_len': _A_in['seg_len'], 'B_x': _B_in['x'], 'B_w1': _B_in['w1'], 'B_w2': _B_in['w2'], 'B_w3': _B_in['w3'], 'B_w4': _B_in['w4']}

def reference(A_x, A_mem0, A_Wq, A_Wk, A_Wv, A_Wo, A_seg_len, B_x, B_w1, B_w2, B_w3, B_w4):

    def _A_ref(x, mem0, Wq, Wk, Wv, Wo, seg_len):
        B, S, Dm = x.shape
        H, Dh = (Wq.shape[1], Wq.shape[2])
        M = mem0.shape[1]
        scale = Dh ** (-0.5)
        n_seg = S // seg_len
        L = M + seg_len
        idx = jnp.arange(L)
        mask = (idx[:, None] < M) | (idx[:, None] >= idx[None, :])
        mem = mem0
        outs = []
        for s in range(n_seg):
            xs = x[:, s * seg_len:(s + 1) * seg_len, :].copy()
            h = jnp.concatenate([mem, xs], axis=1)
            q = jnp.einsum('btd,dhe->bhte', h, Wq)
            k = jnp.einsum('btd,dhe->bhte', h, Wk)
            v = jnp.einsum('btd,dhe->bhte', h, Wv)
            scores = jnp.einsum('bhqe,bhke->bhqk', q, k) * scale
            scores = jnp.where(mask[None, None], scores, -1000000000.0)
            p = _softmax(scores, axis=-1)
            o = jnp.einsum('bhqk,bhke->bhqe', p, v)
            o = jnp.einsum('bhte,hed->btd', o, Wo)
            mem = o[:, :M, :].copy()
            outs.append(o[:, M:, :])
        return jnp.concatenate(outs, axis=1)

    def _B_ref(x, w1, w2, w3, w4):
        B, S, D = x.shape
        h = _gelu(_layernorm(x, axis=-1) @ w1)
        c = D // 4
        g0 = jnp.pad(h[:, :, 0 * c:1 * c], ((0, 0), (1, 0), (0, 0)))[:, :S, :]
        g1 = jnp.pad(h[:, :, 1 * c:2 * c], ((0, 0), (0, 1), (0, 0)))[:, 1:, :]
        g2 = jnp.pad(h[:, :, 2 * c:3 * c], ((0, 0), (2, 0), (0, 0)))[:, :S, :]
        g3 = jnp.pad(h[:, :, 3 * c:], ((0, 0), (0, 2), (0, 0)))[:, 2:, :]
        hs = jnp.concatenate([g0, g1, g2, g3], axis=-1) @ w2
        x1 = x + hs
        h2 = _gelu(_layernorm(x1, axis=-1) @ w3) @ w4
        return x1 + h2
    x = A_x
    xn = _layernorm(x, axis=-1)
    s = _A_ref(xn, A_mem0, A_Wq, A_Wk, A_Wv, A_Wo, A_seg_len)
    g = _silu(_B_ref(xn, B_w1, B_w2, B_w3, B_w4))
    return x + s * g
```

```python
import functools

import jax
import jax.numpy as jnp
import jax.experimental.pallas as pl
import jax.experimental.pallas.tpu as pltpu

S, D, H, E, M, SEG, F = 2048, 1024, 32, 128, 8, 32, 3584
G = H // 2
L = M + SEG
PAIR = 2 * SEG
NIT = S // PAIR
BR = 48
PRE = S - NIT * BR
CH = 256
EPS = 1e-5
F32 = jnp.float32
BF16 = jnp.bfloat16
U32 = jnp.uint32


def _ln(x):
    m = jnp.sum(x, axis=-1, keepdims=True) * (1.0 / D)
    xc = x - m
    v = jnp.sum(xc * xc, axis=-1, keepdims=True) * (1.0 / D)
    return xc * jax.lax.rsqrt(v + EPS)


def _gelu(x):
    c1 = 0.7978845608028654
    c2 = c1 * 0.044715
    t = jnp.tanh(x * (c1 + c2 * (x * x)))
    hx = 0.5 * x
    return hx + hx * t


def _silu(x):
    hx = 0.5 * x
    return hx + hx * jnp.tanh(hx)


def _w(ref_val):
    return pltpu.bitcast(ref_val, BF16)


def _dot(a, b):
    return jnp.dot(a, b, preferred_element_type=F32)


def _kernel(x_hbm, mem_hbm, wq_hbm, wk_hbm, wv_hbm, wo_hbm, w1_hbm, w2_hbm, w3_hbm, w4_hbm,
            out_hbm,
            x_v, xn_v, h_v, g_v, mem0_v, mem_v, s_v, o_stage, fill_v,
            wqkv_v, wo_v, w1_v, w2_v, w3_v, w4_v,
            sem_x, sem_w, sem_qkv, sem_o):
    scale = float(E) ** -0.5

    nch = S // CH
    x_cp = [pltpu.make_async_copy(x_hbm.at[pl.ds(c * CH, CH)], x_v.at[pl.ds(c * CH, CH)], sem_x.at[c])
            for c in range(nch)]
    mem_cp = pltpu.make_async_copy(mem_hbm, mem0_v, sem_w.at[0])
    w1_cp = pltpu.make_async_copy(w1_hbm.bitcast(U32), w1_v, sem_w.at[1])
    w2_cp = pltpu.make_async_copy(w2_hbm.bitcast(U32), w2_v, sem_w.at[2])
    w3_cp = pltpu.make_async_copy(w3_hbm.bitcast(U32), w3_v, sem_w.at[3])
    w4_cp = pltpu.make_async_copy(w4_hbm.bitcast(U32), w4_v, sem_w.at[4])
    wo_cp = pltpu.make_async_copy(wo_hbm.bitcast(U32), wo_v, sem_w.at[5])
    qkv_cp = []
    for p, w_hbm in enumerate((wq_hbm, wk_hbm, wv_hbm)):
        src = w_hbm.bitcast(U32)
        qkv_cp.append([
            pltpu.make_async_copy(src.at[:, b, j, :], wqkv_v.at[j, 2 * p + b], sem_qkv.at[p])
            for j in range(G) for b in range(2)])

    x_cp[0].start()
    w1_cp.start()
    for c in range(1, nch):
        x_cp[c].start()
    w2_cp.start()
    mem_cp.start()
    w3_cp.start()
    w4_cp.start()
    for p in range(3):
        for cp in qkv_cp[p]:
            cp.start()
    wo_cp.start()

    r = jax.lax.broadcasted_iota(jnp.int32, (2 * L, 2 * L), 0)
    c = jax.lax.broadcasted_iota(jnp.int32, (2 * L, 2 * L), 1)
    same = (r < L) == (c < L)
    rr = jnp.where(r < L, r, r - L)
    cc = jnp.where(c < L, c, c - L)
    ok = (rr < M) | (rr >= cc)
    fill_v[...] = jnp.where(same, jnp.where(ok, 0.0, -1e9), -jnp.inf).astype(F32)
    h_v[pl.ds(0, 8), :] = jnp.zeros((8, D), F32)
    h_v[pl.ds(S + 8, 8), :] = jnp.zeros((8, D), F32)

    w1_cp.wait()
    for c in range(nch):
        x_cp[c].wait()

    def stage1(c, carry):
        r0 = pl.multiple_of(c * CH, CH)
        xn = _ln(x_v[pl.ds(r0, CH), :].astype(F32)).astype(BF16).astype(F32)
        xn_v[pl.ds(r0, CH), :] = xn
        z = _ln(xn).astype(BF16)
        h_v[pl.ds(r0 + 8, CH), :] = _gelu(_dot(z, _w(w1_v[...])))
        return carry

    jax.lax.fori_loop(0, nch, stage1, 0)

    w2_cp.wait()
    q4 = D // 4

    def stage2(c, carry):
        r0 = pl.multiple_of(c * CH, CH)
        hb = h_v[pl.ds(r0, CH + 16), :]
        hs = jnp.concatenate([
            hb[7:7 + CH, 0 * q4:1 * q4],
            hb[9:9 + CH, 1 * q4:2 * q4],
            hb[6:6 + CH, 2 * q4:3 * q4],
            hb[10:10 + CH, 3 * q4:4 * q4]], axis=1).astype(BF16)
        g_v[pl.ds(r0, CH), :] = xn_v[pl.ds(r0, CH), :] + _dot(hs, _w(w2_v[...]))
        return carry

    jax.lax.fori_loop(0, nch, stage2, 0)

    w3_cp.wait()
    w4_cp.wait()

    def mlp_up(r0, n):
        x1 = g_v[pl.ds(r0, n), :]
        z = _ln(x1).astype(BF16)
        return _gelu(_dot(z, _w(w3_v[...]))).astype(BF16)

    def mlp_down(r0, n, h3):
        y = g_v[pl.ds(r0, n), :] + _dot(h3, _w(w4_v[...]))
        g_v[pl.ds(r0, n), :] = _silu(y)

    def stage3(c, carry):
        r0 = pl.multiple_of(c * 128, 128)
        mlp_down(r0, 128, mlp_up(r0, 128))
        return carry

    jax.lax.fori_loop(0, PRE // 128, stage3, 0)

    for p in range(3):
        for cp in qkv_cp[p]:
            cp.wait()

    def conv(i, carry):
        r0 = pl.multiple_of(i * 8, 8)
        for j in range(G):
            for p in range(3):
                a = wqkv_v[j, 2 * p, pl.ds(r0, 8), :]
                b = wqkv_v[j, 2 * p + 1, pl.ds(r0, 8), :]
                wqkv_v[j, 2 * p, pl.ds(r0, 8), :] = (a & jnp.uint32(0xFFFF)) | (b << 16)
                wqkv_v[j, 2 * p + 1, pl.ds(r0, 8), :] = (a >> 16) | (b & jnp.uint32(0xFFFF0000))
        return carry

    jax.lax.fori_loop(0, D // 16, conv, 0)
    wo_cp.wait()
    mem_cp.wait()
    mem_v[...] = mem0_v[...].astype(F32)

    def out_cp(j, slot):
        return pltpu.make_async_copy(
            o_stage.at[slot], out_hbm.at[pl.ds(pl.multiple_of(j * PAIR, PAIR), PAIR)], sem_o.at[slot])

    def segment(lhs, qkv_extra, o_extra, first):
        qkv_left, o_left = [None] * G, [None] * G
        qkv, sc, olhs = [None] * G, [None] * G, [None] * G

        def do_qkv(g):
            ys = [_dot(lhs, _w(wqkv_v[g, c])) for c in range(6)]
            if first:
                qkv_left[g] = [y[L:] for y in ys]
                ys = [y[:L] for y in ys]
            else:
                ys = [jnp.concatenate([y[:M], e, y[M:]], axis=0) for y, e in zip(ys, qkv_extra[g])]
            qkv[g] = [jnp.concatenate([ys[2 * p], ys[2 * p + 1]], axis=0).astype(BF16) for p in range(3)]

        def do_s(g):
            q, k, _ = qkv[g]
            s = jax.lax.dot_general(q, k, (((1,), (1,)), ((), ())), preferred_element_type=F32)
            fill = fill_v[...]
            s = jnp.where(fill == 0.0, s * scale, fill)
            e = jnp.exp(s - jnp.max(s, axis=-1, keepdims=True))
            sc[g] = (e.astype(BF16), 1.0 / jnp.sum(e, axis=-1, keepdims=True))

        def do_pv(g):
            e, rl = sc[g]
            o = _dot(e, qkv[g][2]) * rl
            oh = [o[:L], o[L:]]
            if first:
                o_left[g] = [t[32:] for t in oh]
                oh = [t[:32] for t in oh]
            else:
                oh = [jnp.concatenate([t[:M], x, t[M:]], axis=0) for t, x in zip(oh, o_extra[g])]
            olhs[g] = jnp.concatenate(oh, axis=1).astype(BF16)

        def do_wo(g0, g1):
            a = jnp.concatenate(olhs[g0:g1], axis=1)
            return _dot(a, _w(wo_v[g0 * E:g1 * E, :]))

        for g in range(G):
            do_qkv(g)
            if g >= 2:
                do_pv(g - 2)
            if g >= 1:
                do_s(g - 1)
        acc = do_wo(0, 6)
        do_s(G - 1)
        do_pv(G - 2)
        acc = acc + do_wo(6, 12)
        do_pv(G - 1)
        acc = acc + do_wo(12, 14)
        acc = acc + do_wo(14, 16)
        return acc, qkv_left, o_left

    def body(j, carry):
        t0 = pl.multiple_of(j * PAIR, PAIR)
        b0 = pl.multiple_of(PRE + j * BR, 16)
        slot = j % 2
        lhs = jnp.concatenate([mem_v[...], xn_v[pl.ds(t0, 40), :]], axis=0).astype(BF16)
        ra, qkv_left, o_left = segment(lhs, None, None, True)
        s_v[pl.ds(0, 24), :] = ra[M:]
        mem = ra[:M].astype(BF16).astype(F32)
        h3 = mlp_up(b0, BR)
        lhs = jnp.concatenate([mem, xn_v[pl.ds(t0 + 40, 24), :]], axis=0).astype(BF16)
        rb, _, _ = segment(lhs, qkv_left, o_left, False)
        s_v[pl.ds(24, 40), :] = rb[M:]
        mem_v[...] = rb[:M].astype(BF16).astype(F32)
        mlp_down(b0, BR, h3)

        @pl.when(j >= 2)
        def _():
            out_cp(j - 2, slot).wait()

        o_stage[slot] = (x_v[pl.ds(t0, PAIR), :].astype(F32)
                         + s_v[...] * g_v[pl.ds(t0, PAIR), :]).astype(BF16)
        out_cp(j, slot).start()
        return carry

    jax.lax.fori_loop(0, NIT, body, 0)
    out_cp(NIT - 2, 0).wait()
    out_cp(NIT - 1, 1).wait()


@functools.partial(jax.jit, static_argnames=("A_seg_len",))
def pallas_recurrent_scan__memory_aug_recurrent_mem_tr__mixer_s_mlp__prompt_kernel(
    A_x: jax.Array,
    A_mem0: jax.Array,
    A_Wq: jax.Array,
    A_Wk: jax.Array,
    A_Wv: jax.Array,
    A_Wo: jax.Array,
    A_seg_len,
    B_x: jax.Array,
    B_w1: jax.Array,
    B_w2: jax.Array,
    B_w3: jax.Array,
    B_w4: jax.Array,
):
    assert A_seg_len == SEG and A_x.shape == (1, S, D) and A_Wq.shape == (D, H, E)
    del B_x
    any_spec = pl.BlockSpec(memory_space=pl.ANY)
    out = pl.pallas_call(
        _kernel,
        out_shape=jax.ShapeDtypeStruct((S, D), BF16),
        in_specs=[any_spec] * 10,
        out_specs=any_spec,
        scratch_shapes=[
            pltpu.VMEM((S, D), BF16),
            pltpu.VMEM((S, D), F32),
            pltpu.VMEM((S + 16, D), F32),
            pltpu.VMEM((S, D), F32),
            pltpu.VMEM((M, D), BF16),
            pltpu.VMEM((M, D), F32),
            pltpu.VMEM((PAIR, D), F32),
            pltpu.VMEM((2, PAIR, D), BF16),
            pltpu.VMEM((2 * L, 2 * L), F32),
            pltpu.VMEM((G, 6, D // 2, E), U32),
            pltpu.VMEM((H * E // 2, D), U32),
            pltpu.VMEM((D // 2, D), U32),
            pltpu.VMEM((D // 2, D), U32),
            pltpu.VMEM((D // 2, F), U32),
            pltpu.VMEM((F // 2, D), U32),
            pltpu.SemaphoreType.DMA((S // CH,)),
            pltpu.SemaphoreType.DMA((6,)),
            pltpu.SemaphoreType.DMA((3,)),
            pltpu.SemaphoreType.DMA((2,)),
        ],
        compiler_params=pltpu.CompilerParams(vmem_limit_bytes=110 * 1024 * 1024),
    )(
        A_x.reshape(S, D),
        A_mem0.reshape(M, D),
        A_Wq.reshape(D // 2, 2, H, E),
        A_Wk.reshape(D // 2, 2, H, E),
        A_Wv.reshape(D // 2, 2, H, E),
        A_Wo.reshape(H * E, D),
        B_w1, B_w2, B_w3, B_w4,
    )
    return out.reshape(1, S, D)
```

```python
import functools

import jax
import jax.numpy as jnp
import jax.experimental.pallas as pl
import jax.experimental.pallas.tpu as pltpu

S, D, H, E, M, SEG, F = 2048, 1024, 32, 128, 8, 32, 3584
G = H // 2
L = M + SEG
PAIR = 2 * SEG
NIT = S // PAIR
BR = 48
PRE = S - NIT * BR
CH = 256
NCV = 12
EPS = 1e-5
F32 = jnp.float32
BF16 = jnp.bfloat16
U32 = jnp.uint32


def _ln(x):
    m = jnp.sum(x, axis=-1, keepdims=True) * (1.0 / D)
    xc = x - m
    v = jnp.sum(xc * xc, axis=-1, keepdims=True) * (1.0 / D)
    return xc * jax.lax.rsqrt(v + EPS)


def _gelu(x):
    c1 = 0.7978845608028654
    c2 = c1 * 0.044715
    t = jnp.tanh(x * (c1 + c2 * (x * x)))
    hx = 0.5 * x
    return hx + hx * t


def _silu(x):
    hx = 0.5 * x
    return hx + hx * jnp.tanh(hx)


def _w(ref_val):
    return pltpu.bitcast(ref_val, BF16)


def _kernel(x_hbm, mem_hbm, wq_hbm, wk_hbm, wv_hbm, wo_hbm, w1_hbm, w2_hbm, w3_hbm, w4_hbm,
            out_hbm,
            x_v, xn_v, h_v, g_v, z_v, mem0_v, mem_v, s_v, o_stage, fill_v,
            wqkv_v, wo_v, w1_v, w2_v, w3_v, w4_v,
            sem_x, sem_w, sem_qkv, sem_o):
    scale = float(E) ** -0.5

    nch = S // CH
    x_cp = [pltpu.make_async_copy(x_hbm.at[pl.ds(c * CH, CH)], x_v.at[pl.ds(c * CH, CH)], sem_x.at[c])
            for c in range(nch)]
    mem_cp = pltpu.make_async_copy(mem_hbm, mem0_v, sem_w.at[0])
    w1_cp = pltpu.make_async_copy(w1_hbm.bitcast(U32), w1_v, sem_w.at[1])
    w2_cp = pltpu.make_async_copy(w2_hbm.bitcast(U32), w2_v, sem_w.at[2])
    w3_cp = pltpu.make_async_copy(w3_hbm.bitcast(U32), w3_v, sem_w.at[3])
    w4_cp = pltpu.make_async_copy(w4_hbm.bitcast(U32), w4_v, sem_w.at[4])
    wo_cp = pltpu.make_async_copy(wo_hbm.bitcast(U32), wo_v, sem_w.at[5])
    srcs = [w.bitcast(U32) for w in (wq_hbm, wk_hbm, wv_hbm)]

    def qkv_cp(n, b):
        return pltpu.make_async_copy(
            srcs[n // G].at[:, b, n % G, :], wqkv_v.at[n, b], sem_qkv.at[n // NCV])

    def qkv_start(n0, n1):
        for n in range(n0, n1):
            for b in range(2):
                qkv_cp(n, b).start()

    x_cp[0].start()
    w1_cp.start()
    for c in range(1, nch):
        x_cp[c].start()
    w2_cp.start()
    mem_cp.start()
    w3_cp.start()
    w4_cp.start()
    qkv_start(0, 20)

    r = jax.lax.broadcasted_iota(jnp.int32, (2 * L, 2 * L), 0)
    c = jax.lax.broadcasted_iota(jnp.int32, (2 * L, 2 * L), 1)
    same = (r < L) == (c < L)
    rr = jnp.where(r < L, r, r - L)
    cc = jnp.where(c < L, c, c - L)
    ok = (rr < M) | (rr >= cc)
    fill_v[...] = jnp.where(same, jnp.where(ok, 0.0, -1e9), -jnp.inf).astype(F32)
    h_v[pl.ds(0, 8), :] = jnp.zeros((8, D), F32)
    h_v[pl.ds(S + 8, 8), :] = jnp.zeros((8, D), F32)

    s_v[...] = jnp.zeros((PAIR, D), F32)

    def norm_chunk(c):
        r0 = pl.multiple_of(c * CH, CH)
        xn = _ln(x_v[pl.ds(r0, CH), :].astype(F32)).astype(BF16).astype(F32)
        xn_v[pl.ds(r0, CH), :] = xn
        z_v[c % 2] = pltpu.bitcast(_ln(xn).astype(BF16), U32)

    x_cp[0].wait()
    norm_chunk(0)
    w1_cp.wait()

    def stage1(c, carry):
        cn = jnp.minimum(c + 1, nch - 1)

        @pl.when(c + 1 < nch)
        def _():
            pltpu.make_async_copy(x_hbm.at[pl.ds(0, CH)], x_v.at[pl.ds(pl.multiple_of(cn * CH, CH), CH)],
                                  sem_x.at[cn]).wait()

        r0 = pl.multiple_of(c * CH, CH)
        z = _w(z_v[c % 2])
        h_v[pl.ds(r0 + 8, CH), :] = _gelu(jnp.dot(z, _w(w1_v[...]), preferred_element_type=F32))
        r1 = pl.multiple_of(cn * CH, CH)
        xn = _ln(x_v[pl.ds(r1, CH), :].astype(F32)).astype(BF16).astype(F32)
        xn_v[pl.ds(r1, CH), :] = xn
        z_v[(c + 1) % 2] = pltpu.bitcast(_ln(xn).astype(BF16), U32)
        return carry

    jax.lax.fori_loop(0, nch, stage1, 0)
    qkv_start(20, 36)

    w2_cp.wait()
    q4 = D // 4

    def stage2(c, carry):
        r0 = pl.multiple_of(c * CH, CH)
        hb = h_v[pl.ds(r0, CH + 16), :]
        hs = jnp.concatenate([
            hb[7:7 + CH, 0 * q4:1 * q4],
            hb[9:9 + CH, 1 * q4:2 * q4],
            hb[6:6 + CH, 2 * q4:3 * q4],
            hb[10:10 + CH, 3 * q4:4 * q4]], axis=1).astype(BF16)
        g_v[pl.ds(r0, CH), :] = xn_v[pl.ds(r0, CH), :] + jnp.dot(hs, _w(w2_v[...]), preferred_element_type=F32)
        return carry

    jax.lax.fori_loop(0, nch, stage2, 0)
    qkv_start(36, 48)
    wo_cp.start()

    w3_cp.wait()
    w4_cp.wait()

    def mlp_up(r0, n):
        x1 = g_v[pl.ds(r0, n), :]
        z = _ln(x1).astype(BF16)
        return _gelu(jnp.dot(z, _w(w3_v[...]), preferred_element_type=F32)).astype(BF16)

    def mlp_down(r0, n, h3):
        y = g_v[pl.ds(r0, n), :] + jnp.dot(h3, _w(w4_v[...]), preferred_element_type=F32)
        g_v[pl.ds(r0, n), :] = _silu(y)

    def stage3(c, carry):
        for _ in range(2 * NCV):
            pltpu.make_async_copy(srcs[0].at[:, 0, 0, :], wqkv_v.at[c * NCV, 0], sem_qkv.at[c]).wait()
        r0 = pl.multiple_of(c * 128, 128)
        h3 = mlp_up(r0, 128)
        for i in range(NCV):
            n = c * NCV + i
            a = wqkv_v[n, 0]
            b = wqkv_v[n, 1]
            wqkv_v[n, 0] = (a & jnp.uint32(0xFFFF)) | (b << 16)
            wqkv_v[n, 1] = (a >> 16) | (b & jnp.uint32(0xFFFF0000))
        mlp_down(r0, 128, h3)
        return carry

    jax.lax.fori_loop(0, PRE // 128, stage3, 0)
    wo_cp.wait()
    mem_cp.wait()
    mem_v[...] = mem0_v[...].astype(F32)

    def out_cp(j):
        return pltpu.make_async_copy(
            o_stage, out_hbm.at[pl.ds(pl.multiple_of(j * PAIR, PAIR), PAIR)], sem_o.at[0])

    def combine(j):
        t0 = pl.multiple_of(j * PAIR, PAIR)
        o_stage[...] = (x_v[pl.ds(t0, PAIR), :].astype(F32)
                        + s_v[...] * g_v[pl.ds(t0, PAIR), :]).astype(BF16)

    def segment(lhs, qkv_extra, o_extra, first):
        qkv_left, o_left = [None] * G, [None] * G
        qkv, sc, olhs = [None] * G, [None] * G, [None] * G

        def do_qkv(g):
            ys = [jnp.dot(lhs, _w(wqkv_v[(c // 2) * G + g, c % 2]), preferred_element_type=F32)
                  for c in range(6)]
            if first:
                qkv_left[g] = [y[L:] for y in ys]
                ys = [y[:L] for y in ys]
            else:
                ys = [jnp.concatenate([y[:M], e, y[M:]], axis=0) for y, e in zip(ys, qkv_extra[g])]
            qkv[g] = [jnp.concatenate([ys[2 * p], ys[2 * p + 1]], axis=0).astype(BF16) for p in range(3)]

        def do_s(g):
            q, k, _ = qkv[g]
            s = jax.lax.dot_general(q, k, (((1,), (1,)), ((), ())), preferred_element_type=F32)
            fill = fill_v[...]
            s = jnp.where(fill == 0.0, s * scale, fill)
            e = jnp.exp(s - jnp.max(s, axis=-1, keepdims=True))
            l = jnp.sum(e, axis=-1, keepdims=True)
            rl = pl.reciprocal(l, approx=True)
            sc[g] = (e.astype(BF16), rl * (2.0 - l * rl))

        def do_pv(g):
            e, rl = sc[g]
            o = jnp.dot(e, qkv[g][2], preferred_element_type=F32) * rl
            oh = [o[:L], o[L:]]
            if first:
                o_left[g] = [t[32:] for t in oh]
                oh = [t[:32] for t in oh]
            else:
                oh = [jnp.concatenate([t[:M], x, t[M:]], axis=0) for t, x in zip(oh, o_extra[g])]
            olhs[g] = jnp.concatenate(oh, axis=1).astype(BF16)

        def do_wo(g0, g1):
            a = jnp.concatenate(olhs[g0:g1], axis=1)
            return jnp.dot(a, _w(wo_v[g0 * E:g1 * E, :]), preferred_element_type=F32)

        for g in range(G):
            do_qkv(g)
            if g >= 2:
                do_pv(g - 2)
            if g >= 1:
                do_s(g - 1)
        acc = do_wo(0, 6)
        do_s(G - 1)
        do_pv(G - 2)
        acc = do_wo(6, 12) + acc
        do_pv(G - 1)
        acc = do_wo(12, 14) + acc
        acc = do_wo(14, 16) + acc
        return acc, qkv_left, o_left

    def body(j, carry):
        jp = jnp.maximum(j - 1, 0)

        @pl.when(j >= 2)
        def _():
            out_cp(jnp.maximum(j - 2, 0)).wait()

        combine(jp)
        t0 = pl.multiple_of(j * PAIR, PAIR)
        b0 = pl.multiple_of(PRE + j * BR, 16)
        lhs = jnp.concatenate([mem_v[...], xn_v[pl.ds(t0, 40), :]], axis=0).astype(BF16)
        ra, qkv_left, o_left = segment(lhs, None, None, True)
        s_v[pl.ds(0, 24), :] = ra[M:]
        mem = ra[:M].astype(BF16).astype(F32)
        h3 = mlp_up(b0, BR)
        lhs = jnp.concatenate([mem, xn_v[pl.ds(t0 + 40, 24), :]], axis=0).astype(BF16)
        rb, _, _ = segment(lhs, qkv_left, o_left, False)
        s_v[pl.ds(24, 40), :] = rb[M:]
        mem_v[...] = rb[:M].astype(BF16).astype(F32)
        mlp_down(b0, BR, h3)

        @pl.when(j >= 1)
        def _():
            out_cp(jp).start()

        return carry

    jax.lax.fori_loop(0, NIT, body, 0)
    out_cp(NIT - 2).wait()
    combine(NIT - 1)
    out_cp(NIT - 1).start()
    out_cp(NIT - 1).wait()


@functools.partial(jax.jit, static_argnames=("A_seg_len",))
def pallas_recurrent_scan__memory_aug_recurrent_mem_tr__mixer_s_mlp__prompt_kernel(
    A_x: jax.Array,
    A_mem0: jax.Array,
    A_Wq: jax.Array,
    A_Wk: jax.Array,
    A_Wv: jax.Array,
    A_Wo: jax.Array,
    A_seg_len,
    B_x: jax.Array,
    B_w1: jax.Array,
    B_w2: jax.Array,
    B_w3: jax.Array,
    B_w4: jax.Array,
):
    assert A_seg_len == SEG and A_x.shape == (1, S, D) and A_Wq.shape == (D, H, E)
    del B_x
    any_spec = pl.BlockSpec(memory_space=pl.ANY)
    out = pl.pallas_call(
        _kernel,
        out_shape=jax.ShapeDtypeStruct((S, D), BF16),
        in_specs=[any_spec] * 10,
        out_specs=any_spec,
        scratch_shapes=[
            pltpu.VMEM((S, D), BF16),
            pltpu.VMEM((S, D), F32),
            pltpu.VMEM((S + 16, D), F32),
            pltpu.VMEM((S, D), F32),
            pltpu.VMEM((2, CH // 2, D), U32),
            pltpu.VMEM((M, D), BF16),
            pltpu.VMEM((M, D), F32),
            pltpu.VMEM((PAIR, D), F32),
            pltpu.VMEM((PAIR, D), BF16),
            pltpu.VMEM((2 * L, 2 * L), F32),
            pltpu.VMEM((3 * G, 2, D // 2, E), U32),
            pltpu.VMEM((H * E // 2, D), U32),
            pltpu.VMEM((D // 2, D), U32),
            pltpu.VMEM((D // 2, D), U32),
            pltpu.VMEM((D // 2, F), U32),
            pltpu.VMEM((F // 2, D), U32),
            pltpu.SemaphoreType.DMA((S // CH,)),
            pltpu.SemaphoreType.DMA((6,)),
            pltpu.SemaphoreType.DMA((3 * G // NCV,)),
            pltpu.SemaphoreType.DMA((1,)),
        ],
        compiler_params=pltpu.CompilerParams(vmem_limit_bytes=110 * 1024 * 1024),
    )(
        A_x.reshape(S, D),
        A_mem0.reshape(M, D),
        A_Wq.reshape(D // 2, 2, H, E),
        A_Wk.reshape(D // 2, 2, H, E),
        A_Wv.reshape(D // 2, 2, H, E),
        A_Wo.reshape(H * E, D),
        B_w1, B_w2, B_w3, B_w4,
    )
    return out.reshape(1, S, D)
```

```python
import functools

import jax
import jax.numpy as jnp
import jax.experimental.pallas as pl
import jax.experimental.pallas.tpu as pltpu

S, D, H, E, M, SEG, F = 2048, 1024, 32, 128, 8, 32, 3584
G = H // 2
L = M + SEG
PAIR = 2 * SEG
NIT = S // PAIR
BR = 48
PRE = S - NIT * BR
RB = 32
CVB = 8
CH = 256
NCV = 12
EPS = 1e-5
F32 = jnp.float32
BF16 = jnp.bfloat16
U32 = jnp.uint32


def _ln(x, dep=None):
    m = jnp.sum(x, axis=-1, keepdims=True) * (1.0 / D)
    if dep is not None:
        m = m + dep
    xc = x - m
    v = jnp.sum(xc * xc, axis=-1, keepdims=True) * (1.0 / D)
    r = jax.lax.rsqrt(v + EPS)
    return xc * r, jnp.where(r < 0.0, 1.0, 0.0)


def _gelu(x):
    c1 = 0.7978845608028654
    c2 = c1 * 0.044715
    t = jnp.tanh(x * (c1 + c2 * (x * x)))
    hx = 0.5 * x
    return hx + hx * t


def _silu(x):
    hx = 0.5 * x
    return hx + hx * jnp.tanh(hx)


def _w(ref_val):
    return pltpu.bitcast(ref_val, BF16)


def _kernel(x_hbm, mem_hbm, wq_hbm, wk_hbm, wv_hbm, wo_hbm, w1_hbm, w2_hbm, w3_hbm, w4_hbm,
            out_hbm,
            x_v, xn_v, h_v, x1_v, za_v, zb_v, mem0_v, mem_v, s_v, o_stage, fill_v, zero_v,
            wqkv_v, wo_v, w1_v, w2_v, w3_v, w4_v,
            sem_x, sem_w, sem_qkv, sem_o):
    scale = float(E) ** -0.5

    nch = S // CH
    x_cp = [pltpu.make_async_copy(x_hbm.at[pl.ds(c * CH, CH)], x_v.at[pl.ds(c * CH, CH)], sem_x.at[c])
            for c in range(nch)]
    mem_cp = pltpu.make_async_copy(mem_hbm, mem0_v, sem_w.at[0])
    w1_cp = pltpu.make_async_copy(w1_hbm.bitcast(U32), w1_v, sem_w.at[1])
    w2_cp = pltpu.make_async_copy(w2_hbm.bitcast(U32), w2_v, sem_w.at[2])
    w3_cp = pltpu.make_async_copy(w3_hbm.bitcast(U32), w3_v, sem_w.at[3])
    w4_cp = pltpu.make_async_copy(w4_hbm.bitcast(U32), w4_v, sem_w.at[4])
    wo_cp = pltpu.make_async_copy(wo_hbm.bitcast(U32), wo_v, sem_w.at[5])
    srcs = [w.bitcast(U32) for w in (wq_hbm, wk_hbm, wv_hbm)]

    def qkv_cp(n, b):
        return pltpu.make_async_copy(
            srcs[n // G].at[:, b, n % G, :], wqkv_v.at[n, b], sem_qkv.at[n // NCV])

    def qkv_start(n0, n1):
        for n in range(n0, n1):
            for b in range(2):
                qkv_cp(n, b).start()

    x_cp[0].start()
    w1_cp.start()
    for c in range(1, nch):
        x_cp[c].start()
    w2_cp.start()
    mem_cp.start()
    w3_cp.start()
    w4_cp.start()
    qkv_start(0, 20)

    r = jax.lax.broadcasted_iota(jnp.int32, (2 * L, 2 * L), 0)
    c = jax.lax.broadcasted_iota(jnp.int32, (2 * L, 2 * L), 1)
    same = (r < L) == (c < L)
    rr = jnp.where(r < L, r, r - L)
    cc = jnp.where(c < L, c, c - L)
    ok = (rr < M) | (rr >= cc)
    fill_v[...] = jnp.where(same, jnp.where(ok, 0.0, -1e9), -jnp.inf).astype(F32)
    h_v[pl.ds(0, 8), :] = jnp.zeros((8, D), F32)
    h_v[pl.ds(S + 8, 8), :] = jnp.zeros((8, D), F32)

    s_v[...] = jnp.zeros((PAIR, D), F32)
    zero_v[...] = jnp.zeros((8, E), U32)

    def norm_chunk(c, z_ref, rb):
        dep = None
        for b in range(CH // rb):
            r0 = pl.multiple_of(c * CH + b * rb, rb)
            xn, _ = _ln(x_v[pl.ds(r0, rb), :].astype(F32), dep)
            xn = xn.astype(BF16).astype(F32)
            xn_v[pl.ds(r0, rb), :] = xn
            z, dep = _ln(xn)
            z_ref[pl.ds(b * rb // 2, rb // 2), :] = pltpu.bitcast(z.astype(BF16), U32)

    def x_wait(c):
        pltpu.make_async_copy(x_hbm.at[pl.ds(0, CH)], x_v.at[pl.ds(pl.multiple_of(c * CH, CH), CH)],
                              sem_x.at[c]).wait()

    def up1(c, z_ref):
        r0 = pl.multiple_of(c * CH, CH)
        h_v[pl.ds(r0 + 8, CH), :] = _gelu(jnp.dot(_w(z_ref[...]), _w(w1_v[...]), preferred_element_type=F32))

    x_cp[0].wait()
    norm_chunk(0, za_v, CH)
    w1_cp.wait()

    def stage1(i, carry):
        cn = jnp.minimum(2 * i + 2, nch - 1)
        x_wait(2 * i + 1)

        @pl.when(2 * i + 2 < nch)
        def _():
            x_wait(cn)

        up1(2 * i, za_v)
        norm_chunk(2 * i + 1, zb_v, RB)
        up1(2 * i + 1, zb_v)
        norm_chunk(cn, za_v, RB)
        return carry

    jax.lax.fori_loop(0, nch // 2, stage1, 0)
    qkv_start(20, 36)

    w2_cp.wait()
    q4 = D // 4

    def stage2(c, carry):
        r0 = pl.multiple_of(c * CH, CH)
        hb = h_v[pl.ds(r0, CH + 16), :]
        hs = jnp.concatenate([
            hb[7:7 + CH, 0 * q4:1 * q4],
            hb[9:9 + CH, 1 * q4:2 * q4],
            hb[6:6 + CH, 2 * q4:3 * q4],
            hb[10:10 + CH, 3 * q4:4 * q4]], axis=1).astype(BF16)
        x1_v[pl.ds(r0, CH), :] = xn_v[pl.ds(r0, CH), :] + jnp.dot(hs, _w(w2_v[...]), preferred_element_type=F32)
        return carry

    jax.lax.fori_loop(0, nch, stage2, 0)
    qkv_start(36, 48)
    wo_cp.start()

    w3_cp.wait()
    w4_cp.wait()

    def mlp_up(r0, n):
        x1 = x1_v[pl.ds(r0, n), :]
        z = _ln(x1)[0].astype(BF16)
        return _gelu(jnp.dot(z, _w(w3_v[...]), preferred_element_type=F32)).astype(BF16)

    def mlp_down(r0, n, h3):
        y = x1_v[pl.ds(r0, n), :] + jnp.dot(h3, _w(w4_v[...]), preferred_element_type=F32)
        h_v[pl.ds(r0, n), :] = _silu(y)

    def norm3(c, rb):
        dep = None
        for b in range(128 // rb):
            z, dep = _ln(x1_v[pl.ds(pl.multiple_of(c * 128 + b * rb, rb), rb), :], dep)
            za_v[pl.ds(b * rb // 2, rb // 2), :] = pltpu.bitcast(z.astype(BF16), U32)

    norm3(0, 128)

    def stage3(c, carry):
        for _ in range(2 * NCV):
            pltpu.make_async_copy(srcs[0].at[:, 0, 0, :], wqkv_v.at[c * NCV, 0], sem_qkv.at[c]).wait()
        r0 = pl.multiple_of(c * 128, 128)
        z = _w(za_v[pl.ds(0, 64), :])
        h3 = _gelu(jnp.dot(z, _w(w3_v[...]), preferred_element_type=F32)).astype(BF16)
        zero = zero_v[...]
        dep = zero
        for i in range(NCV):
            n = c * NCV + i
            for r in range(0, D // 2, CVB):
                a = wqkv_v[n, 0, pl.ds(r, CVB), :]
                a = jnp.concatenate([a[:8] | dep, a[8:]], axis=0) if CVB > 8 else a | dep
                b = wqkv_v[n, 1, pl.ds(r, CVB), :]
                lo = (a & jnp.uint32(0xFFFF)) | (b << 16)
                wqkv_v[n, 0, pl.ds(r, CVB), :] = lo
                wqkv_v[n, 1, pl.ds(r, CVB), :] = (a >> 16) | (b & jnp.uint32(0xFFFF0000))
                dep = lo[:8] & zero
        mlp_down(r0, 128, h3)
        norm3(jnp.minimum(c + 1, PRE // 128 - 1), 16)
        return carry

    jax.lax.fori_loop(0, PRE // 128, stage3, 0)
    wo_cp.wait()
    mem_cp.wait()
    mem_v[...] = mem0_v[...].astype(F32)

    def out_cp(j):
        return pltpu.make_async_copy(
            o_stage.at[j % 2], out_hbm.at[pl.ds(pl.multiple_of(j * PAIR, PAIR), PAIR)], sem_o.at[j % 2])

    def combine(j):
        t0 = pl.multiple_of(j * PAIR, PAIR)
        o_stage[j % 2] = (x_v[pl.ds(t0, PAIR), :].astype(F32)
                          + s_v[...] * h_v[pl.ds(t0, PAIR), :]).astype(BF16)

    def segment(lhs, qkv_extra, o_extra, first):
        qkv_left, o_left = [None] * G, [None] * G
        qkv, sc, olhs = [None] * G, [None] * G, [None] * G

        def do_qkv(g):
            ys = [jnp.dot(lhs, _w(wqkv_v[(c // 2) * G + g, c % 2]), preferred_element_type=F32)
                  for c in range(6)]
            if first:
                qkv_left[g] = [y[L:] for y in ys]
                ys = [y[:L] for y in ys]
            else:
                ys = [jnp.concatenate([y[:M], e, y[M:]], axis=0) for y, e in zip(ys, qkv_extra[g])]
            qkv[g] = [jnp.concatenate([ys[2 * p], ys[2 * p + 1]], axis=0).astype(BF16) for p in range(3)]

        def do_s(g):
            q, k, _ = qkv[g]
            s = jax.lax.dot_general(q, k, (((1,), (1,)), ((), ())), preferred_element_type=F32)
            fill = fill_v[...]
            s = jnp.where(fill == 0.0, s * scale, fill)
            e = jnp.exp(s - jnp.max(s, axis=-1, keepdims=True))
            l = jnp.sum(e, axis=-1, keepdims=True)
            rl = pl.reciprocal(l, approx=True)
            sc[g] = (e.astype(BF16), rl * (2.0 - l * rl))

        def do_pv(g):
            e, rl = sc[g]
            o = jnp.dot(e, qkv[g][2], preferred_element_type=F32) * rl
            oh = [o[:L], o[L:]]
            if first:
                o_left[g] = [t[32:] for t in oh]
                oh = [t[:32] for t in oh]
            else:
                oh = [jnp.concatenate([t[:M], x, t[M:]], axis=0) for t, x in zip(oh, o_extra[g])]
            olhs[g] = jnp.concatenate(oh, axis=1).astype(BF16)

        def do_wo(g0, g1):
            a = jnp.concatenate(olhs[g0:g1], axis=1)
            return jnp.dot(a, _w(wo_v[g0 * E:g1 * E, :]), preferred_element_type=F32)

        for g in range(G):
            do_qkv(g)
            if g >= 2:
                do_pv(g - 2)
            if g >= 1:
                do_s(g - 1)
        acc = do_wo(0, 6)
        do_s(G - 1)
        do_pv(G - 2)
        acc = do_wo(6, 12) + acc
        do_pv(G - 1)
        acc = do_wo(12, 14) + acc
        acc = do_wo(14, 16) + acc
        return acc, qkv_left, o_left

    def body(j, carry):
        @pl.when(j >= 3)
        def _():
            out_cp(jnp.maximum(j - 3, 0)).wait()

        combine(jnp.maximum(j - 1, 0))
        t0 = pl.multiple_of(j * PAIR, PAIR)
        b0 = pl.multiple_of(PRE + j * BR, 16)
        lhs = jnp.concatenate([mem_v[...], xn_v[pl.ds(t0, 40), :]], axis=0).astype(BF16)
        ra, qkv_left, o_left = segment(lhs, None, None, True)
        s_v[pl.ds(0, 24), :] = ra[M:]
        mem = ra[:M].astype(BF16).astype(F32)
        h3 = mlp_up(b0, BR)
        lhs = jnp.concatenate([mem, xn_v[pl.ds(t0 + 40, 24), :]], axis=0).astype(BF16)
        rb, _, _ = segment(lhs, qkv_left, o_left, False)
        s_v[pl.ds(24, 40), :] = rb[M:]
        mem_v[...] = rb[:M].astype(BF16).astype(F32)
        mlp_down(b0, BR, h3)

        @pl.when(j >= 1)
        def _():
            out_cp(jnp.maximum(j - 1, 0)).start()

        return carry

    jax.lax.fori_loop(0, NIT, body, 0)
    out_cp(NIT - 3).wait()
    combine(NIT - 1)
    out_cp(NIT - 1).start()
    out_cp(NIT - 2).wait()
    out_cp(NIT - 1).wait()


@functools.partial(jax.jit, static_argnames=("A_seg_len",))
def pallas_recurrent_scan__memory_aug_recurrent_mem_tr__mixer_s_mlp__prompt_kernel(
    A_x: jax.Array,
    A_mem0: jax.Array,
    A_Wq: jax.Array,
    A_Wk: jax.Array,
    A_Wv: jax.Array,
    A_Wo: jax.Array,
    A_seg_len,
    B_x: jax.Array,
    B_w1: jax.Array,
    B_w2: jax.Array,
    B_w3: jax.Array,
    B_w4: jax.Array,
):
    assert A_seg_len == SEG and A_x.shape == (1, S, D) and A_Wq.shape == (D, H, E)
    del B_x
    any_spec = pl.BlockSpec(memory_space=pl.ANY)
    out = pl.pallas_call(
        _kernel,
        out_shape=jax.ShapeDtypeStruct((S, D), BF16),
        in_specs=[any_spec] * 10,
        out_specs=any_spec,
        scratch_shapes=[
            pltpu.VMEM((S, D), BF16),
            pltpu.VMEM((S, D), F32),
            pltpu.VMEM((S + 16, D), F32),
            pltpu.VMEM((S, D), F32),
            pltpu.VMEM((CH // 2, D), U32),
            pltpu.VMEM((CH // 2, D), U32),
            pltpu.VMEM((M, D), BF16),
            pltpu.VMEM((M, D), F32),
            pltpu.VMEM((PAIR, D), F32),
            pltpu.VMEM((2, PAIR, D), BF16),
            pltpu.VMEM((2 * L, 2 * L), F32),
            pltpu.VMEM((8, E), U32),
            pltpu.VMEM((3 * G, 2, D // 2, E), U32),
            pltpu.VMEM((H * E // 2, D), U32),
            pltpu.VMEM((D // 2, D), U32),
            pltpu.VMEM((D // 2, D), U32),
            pltpu.VMEM((D // 2, F), U32),
            pltpu.VMEM((F // 2, D), U32),
            pltpu.SemaphoreType.DMA((S // CH,)),
            pltpu.SemaphoreType.DMA((6,)),
            pltpu.SemaphoreType.DMA((3 * G // NCV,)),
            pltpu.SemaphoreType.DMA((2,)),
        ],
        compiler_params=pltpu.CompilerParams(vmem_limit_bytes=110 * 1024 * 1024),
    )(
        A_x.reshape(S, D),
        A_mem0.reshape(M, D),
        A_Wq.reshape(D // 2, 2, H, E),
        A_Wk.reshape(D // 2, 2, H, E),
        A_Wv.reshape(D // 2, 2, H, E),
        A_Wo.reshape(H * E, D),
        B_w1, B_w2, B_w3, B_w4,
    )
    return out.reshape(1, S, D)
```

```python
import functools

import jax
import jax.numpy as jnp
import jax.experimental.pallas as pl
import jax.experimental.pallas.tpu as pltpu

S, D, H, E, M, SEG, F = 2048, 1024, 32, 128, 8, 32, 3584
G = H // 2
L = M + SEG
PAIR = 2 * SEG
NIT = S // PAIR
U = 1
OB = U * PAIR
BR = 48
PRE = S - NIT * BR
RB = 32
CVB = 8
CH2 = 512
CH = 256
NCV = 12
EPS = 1e-5
F32 = jnp.float32
BF16 = jnp.bfloat16
U32 = jnp.uint32


def _ln(x, dep=None):
    m = jnp.sum(x, axis=-1, keepdims=True) * (1.0 / D)
    if dep is not None:
        m = m + dep
    xc = x - m
    v = jnp.sum(xc * xc, axis=-1, keepdims=True) * (1.0 / D)
    r = jax.lax.rsqrt(v + EPS)
    return xc * r, jnp.where(r < 0.0, 1.0, 0.0)


def _gelu(x):
    c1 = 0.7978845608028654
    c2 = c1 * 0.044715
    t = jnp.tanh(x * (c1 + c2 * (x * x)))
    hx = 0.5 * x
    return hx + hx * t


def _silu(x):
    hx = 0.5 * x
    return hx + hx * jnp.tanh(hx)


def _w(ref_val):
    return pltpu.bitcast(ref_val, BF16)


def _kernel(x_hbm, mem_hbm, wq_hbm, wk_hbm, wv_hbm, wo_hbm, w1_hbm, w2_hbm, w3_hbm, w4_hbm,
            out_hbm,
            x_v, xn_v, h_v, x1_v, za_v, zb_v, mem0_v, mem_v, s_v, o_stage, fill_v, zero_v,
            wqkv_v, wo_v, w1_v, w2_v, w3_v, w4_v,
            sem_x, sem_w, sem_qkv, sem_o):
    scale = float(E) ** -0.5

    nch = S // CH
    x_cp = [pltpu.make_async_copy(x_hbm.at[pl.ds(c * CH, CH)], x_v.at[pl.ds(c * CH, CH)], sem_x.at[c])
            for c in range(nch)]
    mem_cp = pltpu.make_async_copy(mem_hbm, mem0_v, sem_w.at[0])
    q4 = D // 4
    w1_cp = [pltpu.make_async_copy(w1_hbm.bitcast(U32).at[:, pl.ds(q * q4, q4)],
                                   w1_v.at[:, pl.ds(q * q4, q4)], sem_w.at[6 + q]) for q in range(4)]
    w2_cp = pltpu.make_async_copy(w2_hbm.bitcast(U32), w2_v, sem_w.at[2])
    w3_cp = pltpu.make_async_copy(w3_hbm.bitcast(U32), w3_v, sem_w.at[3])
    w4_cp = pltpu.make_async_copy(w4_hbm.bitcast(U32), w4_v, sem_w.at[4])
    wo_cp = pltpu.make_async_copy(wo_hbm.bitcast(U32), wo_v, sem_w.at[5])
    srcs = [w.bitcast(U32) for w in (wq_hbm, wk_hbm, wv_hbm)]

    def qkv_cp(n, b):
        return pltpu.make_async_copy(
            srcs[n // G].at[:, b, n % G, :], wqkv_v.at[n, b], sem_qkv.at[n // NCV])

    def qkv_start(n0, n1):
        for n in range(n0, n1):
            for b in range(2):
                qkv_cp(n, b).start()

    x_cp[0].start()
    w1_cp[0].start()
    x_cp[1].start()
    w1_cp[1].start()
    w1_cp[2].start()
    w1_cp[3].start()
    for c in range(2, nch):
        x_cp[c].start()
    w2_cp.start()
    mem_cp.start()
    w3_cp.start()
    w4_cp.start()
    qkv_start(0, 20)

    r = jax.lax.broadcasted_iota(jnp.int32, (2 * L, 2 * L), 0)
    c = jax.lax.broadcasted_iota(jnp.int32, (2 * L, 2 * L), 1)
    same = (r < L) == (c < L)
    rr = jnp.where(r < L, r, r - L)
    cc = jnp.where(c < L, c, c - L)
    ok = (rr < M) | (rr >= cc)
    fill_v[...] = jnp.where(same, jnp.where(ok, 0.0, -1e9), -jnp.inf).astype(F32)
    h_v[pl.ds(0, 8), :] = jnp.zeros((8, D), F32)
    h_v[pl.ds(S + 8, 8), :] = jnp.zeros((8, D), F32)

    s_v[...] = jnp.zeros((OB, D), F32)
    zero_v[...] = jnp.zeros((8, E), U32)

    def norm_chunk(c, z_ref, rb):
        dep = None
        for b in range(CH // rb):
            r0 = pl.multiple_of(c * CH + b * rb, rb)
            xn, _ = _ln(x_v[pl.ds(r0, rb), :].astype(F32), dep)
            xn = xn.astype(BF16).astype(F32)
            xn_v[pl.ds(r0, rb), :] = xn
            z, dep = _ln(xn)
            z_ref[pl.ds(b * rb // 2, rb // 2), :] = pltpu.bitcast(z.astype(BF16), U32)

    def x_wait(c):
        pltpu.make_async_copy(x_hbm.at[pl.ds(0, CH)], x_v.at[pl.ds(pl.multiple_of(c * CH, CH), CH)],
                              sem_x.at[c]).wait()

    def up1(c, z_ref):
        r0 = pl.multiple_of(c * CH, CH)
        h_v[pl.ds(r0 + 8, CH), :] = _gelu(jnp.dot(_w(z_ref[...]), _w(w1_v[...]), preferred_element_type=F32))

    def up1q(c, z_ref, q, nq):
        w = _w(w1_v[:, pl.ds(q * q4, nq * q4)])
        h_v[pl.ds(c * CH + 8, CH), pl.ds(q * q4, nq * q4)] = _gelu(
            jnp.dot(_w(z_ref[...]), w, preferred_element_type=F32))

    x_cp[0].wait()
    norm_chunk(0, za_v, CH)
    w1_cp[0].wait()
    up1q(0, za_v, 0, 1)
    x_cp[1].wait()
    norm_chunk(1, zb_v, CH)
    w1_cp[1].wait()
    up1q(1, zb_v, 0, 1)
    up1q(0, za_v, 1, 1)
    up1q(1, zb_v, 1, 1)
    w1_cp[2].wait()
    w1_cp[3].wait()
    x_cp[2].wait()
    up1q(0, za_v, 2, 2)
    up1q(1, zb_v, 2, 2)
    norm_chunk(2, za_v, 2 * RB)

    def stage1(i, carry):
        cn = jnp.minimum(2 * i + 2, nch - 1)
        x_wait(2 * i + 1)

        @pl.when(2 * i + 2 < nch)
        def _():
            x_wait(cn)

        up1(2 * i, za_v)
        norm_chunk(2 * i + 1, zb_v, RB)
        up1(2 * i + 1, zb_v)
        norm_chunk(cn, za_v, RB)
        return carry

    jax.lax.fori_loop(1, nch // 2, stage1, 0)
    qkv_start(20, 36)

    w2_cp.wait()

    def norm3(c, rb):
        dep = None
        for b in range(128 // rb):
            z, dep = _ln(x1_v[pl.ds(pl.multiple_of(c * 128 + b * rb, rb), rb), :], dep)
            za_v[pl.ds(b * rb // 2, rb // 2), :] = pltpu.bitcast(z.astype(BF16), U32)

    x1_v[pl.ds(0, 128), :] = jnp.zeros((128, D), F32)

    def stage2(c, carry):
        norm3(0, 16)
        r0 = pl.multiple_of(c * CH2, CH2)
        hb = h_v[pl.ds(r0, CH2 + 16), :]
        hs = jnp.concatenate([
            hb[7:7 + CH2, 0 * q4:1 * q4],
            hb[9:9 + CH2, 1 * q4:2 * q4],
            hb[6:6 + CH2, 2 * q4:3 * q4],
            hb[10:10 + CH2, 3 * q4:4 * q4]], axis=1).astype(BF16)
        x1_v[pl.ds(r0, CH2), :] = xn_v[pl.ds(r0, CH2), :] + jnp.dot(hs, _w(w2_v[...]), preferred_element_type=F32)
        return carry

    jax.lax.fori_loop(0, S // CH2, stage2, 0)
    qkv_start(36, 48)
    wo_cp.start()

    w3_cp.wait()
    w4_cp.wait()

    def mlp_up(r0, n):
        x1 = x1_v[pl.ds(r0, n), :]
        z = _ln(x1)[0].astype(BF16)
        return _gelu(jnp.dot(z, _w(w3_v[...]), preferred_element_type=F32)).astype(BF16)

    def mlp_down(r0, n, h3):
        y = x1_v[pl.ds(r0, n), :] + jnp.dot(h3, _w(w4_v[...]), preferred_element_type=F32)
        h_v[pl.ds(r0, n), :] = _silu(y)

    def stage3(c, carry):
        blk = wqkv_v.at[pl.ds(c * NCV, NCV)]
        pltpu.make_async_copy(blk, blk, sem_qkv.at[c]).wait()
        r0 = pl.multiple_of(c * 128, 128)
        z = _w(za_v[pl.ds(0, 64), :])
        h3 = _gelu(jnp.dot(z, _w(w3_v[...]), preferred_element_type=F32)).astype(BF16)
        zero = zero_v[...]
        dep = zero
        for i in range(NCV):
            n = c * NCV + i
            for r in range(0, D // 2, CVB):
                a = wqkv_v[n, 0, pl.ds(r, CVB), :]
                a = jnp.concatenate([a[:8] | dep, a[8:]], axis=0) if CVB > 8 else a | dep
                b = wqkv_v[n, 1, pl.ds(r, CVB), :]
                lo = (a & jnp.uint32(0xFFFF)) | (b << 16)
                wqkv_v[n, 0, pl.ds(r, CVB), :] = lo
                wqkv_v[n, 1, pl.ds(r, CVB), :] = (a >> 16) | (b & jnp.uint32(0xFFFF0000))
                dep = lo[:8] & zero
        mlp_down(r0, 128, h3)
        norm3(jnp.minimum(c + 1, PRE // 128 - 1), 16)
        return carry

    jax.lax.fori_loop(0, PRE // 128, stage3, 0)
    wo_cp.wait()
    mem_cp.wait()
    mem_v[...] = mem0_v[...].astype(F32)

    def out_cp(j):
        return pltpu.make_async_copy(
            o_stage.at[j % 2], out_hbm.at[pl.ds(pl.multiple_of(j * OB, OB), OB)], sem_o.at[j % 2])

    def combine(j):
        t0 = pl.multiple_of(j * OB, OB)
        o_stage[j % 2] = (x_v[pl.ds(t0, OB), :].astype(F32)
                          + s_v[...] * h_v[pl.ds(t0, OB), :]).astype(BF16)

    def segment(lhs, qkv_extra, o_extra, first):
        qkv_left, o_left = [None] * G, [None] * G
        qkv, sc, olhs = [None] * G, [None] * G, [None] * G

        def do_qkv(g):
            ys = [jnp.dot(lhs, _w(wqkv_v[(c // 2) * G + g, c % 2]), preferred_element_type=F32)
                  for c in range(6)]
            if first:
                qkv_left[g] = [y[L:] for y in ys]
                ys = [y[:L] for y in ys]
            else:
                ys = [jnp.concatenate([y[:M], e, y[M:]], axis=0) for y, e in zip(ys, qkv_extra[g])]
            qkv[g] = [jnp.concatenate([ys[2 * p], ys[2 * p + 1]], axis=0).astype(BF16) for p in range(3)]

        def do_s(g):
            q, k, _ = qkv[g]
            s = jax.lax.dot_general(q, k, (((1,), (1,)), ((), ())), preferred_element_type=F32)
            fill = fill_v[...]
            s = jnp.where(fill == 0.0, s * scale, fill)
            e = jnp.exp(s - jnp.max(s, axis=-1, keepdims=True))
            l = jnp.sum(e, axis=-1, keepdims=True)
            rl = pl.reciprocal(l, approx=True)
            sc[g] = (e.astype(BF16), rl * (2.0 - l * rl))

        def do_pv(g):
            e, rl = sc[g]
            o = jnp.dot(e, qkv[g][2], preferred_element_type=F32) * rl
            oh = [o[:L], o[L:]]
            if first:
                o_left[g] = [t[32:] for t in oh]
                oh = [t[:32] for t in oh]
            else:
                oh = [jnp.concatenate([t[:M], x, t[M:]], axis=0) for t, x in zip(oh, o_extra[g])]
            olhs[g] = jnp.concatenate(oh, axis=1).astype(BF16)

        def do_wo(g0, g1):
            a = jnp.concatenate(olhs[g0:g1], axis=1)
            return jnp.dot(a, _w(wo_v[g0 * E:g1 * E, :]), preferred_element_type=F32)

        for g in range(G):
            do_qkv(g)
            if g >= 2:
                do_pv(g - 2)
            if g >= 1:
                do_s(g - 1)
        acc = do_wo(0, 6)
        do_s(G - 1)
        do_pv(G - 2)
        acc = do_wo(6, 12) + acc
        do_pv(G - 1)
        acc = do_wo(12, 14) + acc
        acc = do_wo(14, 16) + acc
        return acc, qkv_left, o_left

    def body(j, carry):
        @pl.when(j >= 3)
        def _():
            out_cp(jnp.maximum(j - 3, 0)).wait()

        combine(jnp.maximum(j - 1, 0))
        mem = mem_v[...]
        for u in range(U):
            t0 = pl.multiple_of(j * OB + u * PAIR, PAIR)
            b0 = pl.multiple_of(PRE + (j * U + u) * BR, 16)
            lhs = jnp.concatenate([mem, xn_v[pl.ds(t0, 40), :]], axis=0).astype(BF16)
            ra, qkv_left, o_left = segment(lhs, None, None, True)
            s_v[pl.ds(u * PAIR, 24), :] = ra[M:]
            mem = ra[:M].astype(BF16).astype(F32)
            h3 = mlp_up(b0, BR)
            lhs = jnp.concatenate([mem, xn_v[pl.ds(t0 + 40, 24), :]], axis=0).astype(BF16)
            rb, _, _ = segment(lhs, qkv_left, o_left, False)
            s_v[pl.ds(u * PAIR + 24, 40), :] = rb[M:]
            mem = rb[:M].astype(BF16).astype(F32)
            mlp_down(b0, BR, h3)
        mem_v[...] = mem

        @pl.when(j >= 1)
        def _():
            out_cp(jnp.maximum(j - 1, 0)).start()

        return carry

    nj = NIT // U
    jax.lax.fori_loop(0, nj, body, 0)
    out_cp(nj - 3).wait()
    combine(nj - 1)
    out_cp(nj - 1).start()
    out_cp(nj - 2).wait()
    out_cp(nj - 1).wait()


@functools.partial(jax.jit, static_argnames=("A_seg_len",))
def pallas_recurrent_scan__memory_aug_recurrent_mem_tr__mixer_s_mlp__prompt_kernel(
    A_x: jax.Array,
    A_mem0: jax.Array,
    A_Wq: jax.Array,
    A_Wk: jax.Array,
    A_Wv: jax.Array,
    A_Wo: jax.Array,
    A_seg_len,
    B_x: jax.Array,
    B_w1: jax.Array,
    B_w2: jax.Array,
    B_w3: jax.Array,
    B_w4: jax.Array,
):
    assert A_seg_len == SEG and A_x.shape == (1, S, D) and A_Wq.shape == (D, H, E)
    del B_x
    any_spec = pl.BlockSpec(memory_space=pl.ANY)
    out = pl.pallas_call(
        _kernel,
        out_shape=jax.ShapeDtypeStruct((S, D), BF16),
        in_specs=[any_spec] * 10,
        out_specs=any_spec,
        scratch_shapes=[
            pltpu.VMEM((S, D), BF16),
            pltpu.VMEM((S, D), F32),
            pltpu.VMEM((S + 16, D), F32),
            pltpu.VMEM((S, D), F32),
            pltpu.VMEM((CH // 2, D), U32),
            pltpu.VMEM((CH // 2, D), U32),
            pltpu.VMEM((M, D), BF16),
            pltpu.VMEM((M, D), F32),
            pltpu.VMEM((OB, D), F32),
            pltpu.VMEM((2, OB, D), BF16),
            pltpu.VMEM((2 * L, 2 * L), F32),
            pltpu.VMEM((8, E), U32),
            pltpu.VMEM((3 * G, 2, D // 2, E), U32),
            pltpu.VMEM((H * E // 2, D), U32),
            pltpu.VMEM((D // 2, D), U32),
            pltpu.VMEM((D // 2, D), U32),
            pltpu.VMEM((D // 2, F), U32),
            pltpu.VMEM((F // 2, D), U32),
            pltpu.SemaphoreType.DMA((S // CH,)),
            pltpu.SemaphoreType.DMA((10,)),
            pltpu.SemaphoreType.DMA((3 * G // NCV,)),
            pltpu.SemaphoreType.DMA((2,)),
        ],
        compiler_params=pltpu.CompilerParams(vmem_limit_bytes=110 * 1024 * 1024),
    )(
        A_x.reshape(S, D),
        A_mem0.reshape(M, D),
        A_Wq.reshape(D // 2, 2, H, E),
        A_Wk.reshape(D // 2, 2, H, E),
        A_Wv.reshape(D // 2, 2, H, E),
        A_Wo.reshape(H * E, D),
        B_w1, B_w2, B_w3, B_w4,
    )
    return out.reshape(1, S, D)
```

```python
import functools

import jax
import jax.numpy as jnp
import jax.experimental.pallas as pl
import jax.experimental.pallas.tpu as pltpu

S, D, H, E, M, SEG, F = 2048, 1024, 32, 128, 8, 32, 3584
G = H // 2
L = M + SEG
PAIR = 2 * SEG
NIT = S // PAIR
U = 1
OB = U * PAIR
BR = 48
PRE = S - NIT * BR
RB = 16
CVB = 8
CH2 = 512
CH = 256
NCV = 12
EPS = 1e-5
F32 = jnp.float32
BF16 = jnp.bfloat16
U32 = jnp.uint32


def _ln(x, dep=None):
    m = jnp.sum(x, axis=-1, keepdims=True) * (1.0 / D)
    if dep is not None:
        m = m + dep
    xc = x - m
    v = jnp.sum(xc * xc, axis=-1, keepdims=True) * (1.0 / D)
    r = jax.lax.rsqrt(v + EPS)
    return xc * r, jnp.where(r < 0.0, 1.0, 0.0)


def _gelu(x):
    c1 = 0.7978845608028654
    c2 = c1 * 0.044715
    t = jnp.tanh(x * (c1 + c2 * (x * x)))
    hx = 0.5 * x
    return hx + hx * t


def _silu(x):
    hx = 0.5 * x
    return hx + hx * jnp.tanh(hx)


def _w(ref_val):
    return pltpu.bitcast(ref_val, BF16)


def _kernel(x_hbm, mem_hbm, wq_hbm, wk_hbm, wv_hbm, wo_hbm, w1_hbm, w2_hbm, w3_hbm, w4_hbm,
            out_hbm,
            x_v, xn_v, h_v, x1_v, za_v, zb_v, mem0_v, mem_v, s_v, o_stage, fill_v, zero_v,
            wqkv_v, wo_v, w1_v, w2_v, w3_v, w4_v,
            sem_x, sem_w, sem_qkv, sem_o):
    scale = float(E) ** -0.5

    nch = S // CH
    x_cp = [pltpu.make_async_copy(x_hbm.at[pl.ds(c * CH, CH)], x_v.at[pl.ds(c * CH, CH)], sem_x.at[c])
            for c in range(nch)]
    mem_cp = pltpu.make_async_copy(mem_hbm, mem0_v, sem_w.at[0])
    q4 = D // 4
    w1_cp = [pltpu.make_async_copy(w1_hbm.bitcast(U32).at[:, pl.ds(q * q4, q4)],
                                   w1_v.at[:, pl.ds(q * q4, q4)], sem_w.at[6 + q]) for q in range(4)]
    w2_cp = pltpu.make_async_copy(w2_hbm.bitcast(U32), w2_v, sem_w.at[2])
    w3_cp = pltpu.make_async_copy(w3_hbm.bitcast(U32), w3_v, sem_w.at[3])
    w4_cp = pltpu.make_async_copy(w4_hbm.bitcast(U32), w4_v, sem_w.at[4])
    wo_cp = pltpu.make_async_copy(wo_hbm.bitcast(U32), wo_v, sem_w.at[5])
    srcs = [w.bitcast(U32) for w in (wq_hbm, wk_hbm, wv_hbm)]

    def qkv_cp(n, b):
        return pltpu.make_async_copy(
            srcs[n // G].at[:, b, n % G, :], wqkv_v.at[n, b], sem_qkv.at[n // NCV])

    def qkv_start(n0, n1):
        for n in range(n0, n1):
            for b in range(2):
                qkv_cp(n, b).start()

    x_cp[0].start()
    w1_cp[0].start()
    x_cp[1].start()
    w1_cp[1].start()
    w1_cp[2].start()
    w1_cp[3].start()
    for c in range(2, nch):
        x_cp[c].start()
    w2_cp.start()
    mem_cp.start()
    w3_cp.start()
    w4_cp.start()
    qkv_start(0, 20)

    r = jax.lax.broadcasted_iota(jnp.int32, (2 * L, 2 * L), 0)
    c = jax.lax.broadcasted_iota(jnp.int32, (2 * L, 2 * L), 1)
    same = (r < L) == (c < L)
    rr = jnp.where(r < L, r, r - L)
    cc = jnp.where(c < L, c, c - L)
    ok = (rr < M) | (rr >= cc)
    fill_v[...] = jnp.where(same, jnp.where(ok, 0.0, -1e9), -jnp.inf).astype(F32)
    h_v[pl.ds(0, 8), :] = jnp.zeros((8, D), F32)
    h_v[pl.ds(S + 8, 8), :] = jnp.zeros((8, D), F32)

    s_v[...] = jnp.zeros((OB, D), F32)
    zero_v[...] = jnp.zeros((8, E), U32)

    def norm_chunk(c, z_ref, rb):
        deps = [None, None]
        for b in range(CH // rb):
            r0 = pl.multiple_of(c * CH + b * rb, rb)
            xn, mid = _ln(x_v[pl.ds(r0, rb), :].astype(F32), deps[b % 2])
            if b == 0:
                deps[1] = mid
            xn = xn.astype(BF16).astype(F32)
            xn_v[pl.ds(r0, rb), :] = xn
            z, deps[b % 2] = _ln(xn)
            z_ref[pl.ds(b * rb // 2, rb // 2), :] = pltpu.bitcast(z.astype(BF16), U32)

    def x_wait(c):
        pltpu.make_async_copy(x_hbm.at[pl.ds(0, CH)], x_v.at[pl.ds(pl.multiple_of(c * CH, CH), CH)],
                              sem_x.at[c]).wait()

    def up1(c, z_ref):
        r0 = pl.multiple_of(c * CH, CH)
        h_v[pl.ds(r0 + 8, CH), :] = _gelu(jnp.dot(_w(z_ref[...]), _w(w1_v[...]), preferred_element_type=F32))

    def up1q(c, z_ref, q, nq):
        w = _w(w1_v[:, pl.ds(q * q4, nq * q4)])
        h_v[pl.ds(c * CH + 8, CH), pl.ds(q * q4, nq * q4)] = _gelu(
            jnp.dot(_w(z_ref[...]), w, preferred_element_type=F32))

    x_cp[0].wait()
    norm_chunk(0, za_v, CH)
    w1_cp[0].wait()
    up1q(0, za_v, 0, 1)
    x_cp[1].wait()
    norm_chunk(1, zb_v, CH)
    w1_cp[1].wait()
    up1q(1, zb_v, 0, 1)
    up1q(0, za_v, 1, 1)
    up1q(1, zb_v, 1, 1)
    w1_cp[2].wait()
    w1_cp[3].wait()
    x_cp[2].wait()
    up1q(0, za_v, 2, 2)
    up1q(1, zb_v, 2, 2)
    norm_chunk(2, za_v, 2 * RB)

    def stage1(i, carry):
        cn = jnp.minimum(2 * i + 2, nch - 1)
        x_wait(2 * i + 1)

        @pl.when(2 * i + 2 < nch)
        def _():
            x_wait(cn)

        up1(2 * i, za_v)
        norm_chunk(2 * i + 1, zb_v, RB)
        up1(2 * i + 1, zb_v)
        norm_chunk(cn, za_v, RB)
        return carry

    jax.lax.fori_loop(1, nch // 2, stage1, 0)
    qkv_start(20, 36)

    w2_cp.wait()

    def norm3(c, rb):
        dep = None
        for b in range(128 // rb):
            z, dep = _ln(x1_v[pl.ds(pl.multiple_of(c * 128 + b * rb, rb), rb), :], dep)
            za_v[pl.ds(b * rb // 2, rb // 2), :] = pltpu.bitcast(z.astype(BF16), U32)

    x1_v[pl.ds(0, 128), :] = jnp.zeros((128, D), F32)

    def stage2(c, carry):
        norm3(0, 16)
        r0 = pl.multiple_of(c * CH2, CH2)
        hb = h_v[pl.ds(r0, CH2 + 16), :]
        hs = jnp.concatenate([
            hb[7:7 + CH2, 0 * q4:1 * q4],
            hb[9:9 + CH2, 1 * q4:2 * q4],
            hb[6:6 + CH2, 2 * q4:3 * q4],
            hb[10:10 + CH2, 3 * q4:4 * q4]], axis=1).astype(BF16)
        x1_v[pl.ds(r0, CH2), :] = xn_v[pl.ds(r0, CH2), :] + jnp.dot(hs, _w(w2_v[...]), preferred_element_type=F32)
        return carry

    jax.lax.fori_loop(0, S // CH2, stage2, 0)
    qkv_start(36, 48)
    wo_cp.start()

    w3_cp.wait()
    w4_cp.wait()

    def mlp_up(r0, n):
        x1 = x1_v[pl.ds(r0, n), :]
        z = _ln(x1)[0].astype(BF16)
        return _gelu(jnp.dot(z, _w(w3_v[...]), preferred_element_type=F32)).astype(BF16)

    def mlp_down(r0, n, h3):
        y = x1_v[pl.ds(r0, n), :] + jnp.dot(h3, _w(w4_v[...]), preferred_element_type=F32)
        h_v[pl.ds(r0, n), :] = _silu(y)

    def stage3(c, carry):
        blk = wqkv_v.at[pl.ds(c * NCV, NCV)]
        pltpu.make_async_copy(blk, blk, sem_qkv.at[c]).wait()
        r0 = pl.multiple_of(c * 128, 128)
        z = _w(za_v[pl.ds(0, 64), :])
        h3 = _gelu(jnp.dot(z, _w(w3_v[...]), preferred_element_type=F32)).astype(BF16)
        zero = zero_v[...]
        dep = zero
        for i in range(NCV):
            n = c * NCV + i
            for r in range(0, D // 2, CVB):
                a = wqkv_v[n, 0, pl.ds(r, CVB), :]
                a = jnp.concatenate([a[:8] | dep, a[8:]], axis=0) if CVB > 8 else a | dep
                b = wqkv_v[n, 1, pl.ds(r, CVB), :]
                lo = (a & jnp.uint32(0xFFFF)) | (b << 16)
                wqkv_v[n, 0, pl.ds(r, CVB), :] = lo
                wqkv_v[n, 1, pl.ds(r, CVB), :] = (a >> 16) | (b & jnp.uint32(0xFFFF0000))
                dep = lo[:8] & zero
        mlp_down(r0, 128, h3)
        norm3(jnp.minimum(c + 1, PRE // 128 - 1), 16)
        return carry

    jax.lax.fori_loop(0, PRE // 128, stage3, 0)
    wo_cp.wait()
    mem_cp.wait()
    mem_v[...] = mem0_v[...].astype(F32)

    def out_cp(j):
        return pltpu.make_async_copy(
            o_stage.at[j % 2], out_hbm.at[pl.ds(pl.multiple_of(j * OB, OB), OB)], sem_o.at[j % 2])

    def combine(j):
        t0 = pl.multiple_of(j * OB, OB)
        o_stage[j % 2] = (x_v[pl.ds(t0, OB), :].astype(F32)
                          + s_v[...] * h_v[pl.ds(t0, OB), :]).astype(BF16)

    def segment(lhs, qkv_extra, o_extra, first):
        qkv_left, o_left = [None] * G, [None] * G
        qkv, sc, olhs = [None] * G, [None] * G, [None] * G

        def do_qkv(g):
            ys = [jnp.dot(lhs, _w(wqkv_v[(c // 2) * G + g, c % 2]), preferred_element_type=F32)
                  for c in range(6)]
            if first:
                qkv_left[g] = [y[L:] for y in ys]
                ys = [y[:L] for y in ys]
            else:
                ys = [jnp.concatenate([y[:M], e, y[M:]], axis=0) for y, e in zip(ys, qkv_extra[g])]
            qkv[g] = [jnp.concatenate([ys[2 * p], ys[2 * p + 1]], axis=0).astype(BF16) for p in range(3)]

        def do_s(g):
            q, k, _ = qkv[g]
            s = jax.lax.dot_general(q, k, (((1,), (1,)), ((), ())), preferred_element_type=F32)
            fill = fill_v[...]
            s = jnp.where(fill == 0.0, s * scale, fill)
            e = jnp.exp(s - jnp.max(s, axis=-1, keepdims=True))
            l = jnp.sum(e, axis=-1, keepdims=True)
            rl = pl.reciprocal(l, approx=True)
            sc[g] = (e.astype(BF16), rl * (2.0 - l * rl))

        def do_pv(g):
            e, rl = sc[g]
            o = jnp.dot(e, qkv[g][2], preferred_element_type=F32) * rl
            oh = [o[:L], o[L:]]
            if first:
                o_left[g] = [t[32:] for t in oh]
                oh = [t[:32] for t in oh]
            else:
                oh = [jnp.concatenate([t[:M], x, t[M:]], axis=0) for t, x in zip(oh, o_extra[g])]
            olhs[g] = jnp.concatenate(oh, axis=1).astype(BF16)

        def do_wo(g0, g1):
            a = jnp.concatenate(olhs[g0:g1], axis=1)
            return jnp.dot(a, _w(wo_v[g0 * E:g1 * E, :]), preferred_element_type=F32)

        for g in range(G):
            do_qkv(g)
            if g >= 2:
                do_pv(g - 2)
            if g >= 1:
                do_s(g - 1)
        acc = do_wo(0, 6)
        do_s(G - 1)
        do_pv(G - 2)
        acc = do_wo(6, 12) + acc
        do_pv(G - 1)
        acc = do_wo(12, 14) + acc
        acc = do_wo(14, 16) + acc
        return acc, qkv_left, o_left

    def body(j, carry):
        @pl.when(j >= 3)
        def _():
            out_cp(jnp.maximum(j - 3, 0)).wait()

        combine(jnp.maximum(j - 1, 0))
        mem = mem_v[...]
        for u in range(U):
            t0 = pl.multiple_of(j * OB + u * PAIR, PAIR)
            b0 = pl.multiple_of(PRE + (j * U + u) * BR, 16)
            lhs = jnp.concatenate([mem, xn_v[pl.ds(t0, 40), :]], axis=0).astype(BF16)
            ra, qkv_left, o_left = segment(lhs, None, None, True)
            s_v[pl.ds(u * PAIR, 24), :] = ra[M:]
            mem = ra[:M].astype(BF16).astype(F32)
            h3 = mlp_up(b0, BR)
            lhs = jnp.concatenate([mem, xn_v[pl.ds(t0 + 40, 24), :]], axis=0).astype(BF16)
            rb, _, _ = segment(lhs, qkv_left, o_left, False)
            s_v[pl.ds(u * PAIR + 24, 40), :] = rb[M:]
            mem = rb[:M].astype(BF16).astype(F32)
            mlp_down(b0, BR, h3)
        mem_v[...] = mem

        @pl.when(j >= 1)
        def _():
            out_cp(jnp.maximum(j - 1, 0)).start()

        return carry

    nj = NIT // U
    jax.lax.fori_loop(0, nj, body, 0)
    out_cp(nj - 3).wait()
    combine(nj - 1)
    out_cp(nj - 1).start()
    out_cp(nj - 2).wait()
    out_cp(nj - 1).wait()


@functools.partial(jax.jit, static_argnames=("A_seg_len",))
def pallas_recurrent_scan__memory_aug_recurrent_mem_tr__mixer_s_mlp__prompt_kernel(
    A_x: jax.Array,
    A_mem0: jax.Array,
    A_Wq: jax.Array,
    A_Wk: jax.Array,
    A_Wv: jax.Array,
    A_Wo: jax.Array,
    A_seg_len,
    B_x: jax.Array,
    B_w1: jax.Array,
    B_w2: jax.Array,
    B_w3: jax.Array,
    B_w4: jax.Array,
):
    assert A_seg_len == SEG and A_x.shape == (1, S, D) and A_Wq.shape == (D, H, E)
    del B_x
    any_spec = pl.BlockSpec(memory_space=pl.ANY)
    out = pl.pallas_call(
        _kernel,
        out_shape=jax.ShapeDtypeStruct((S, D), BF16),
        in_specs=[any_spec] * 10,
        out_specs=any_spec,
        scratch_shapes=[
            pltpu.VMEM((S, D), BF16),
            pltpu.VMEM((S, D), F32),
            pltpu.VMEM((S + 16, D), F32),
            pltpu.VMEM((S, D), F32),
            pltpu.VMEM((CH // 2, D), U32),
            pltpu.VMEM((CH // 2, D), U32),
            pltpu.VMEM((M, D), BF16),
            pltpu.VMEM((M, D), F32),
            pltpu.VMEM((OB, D), F32),
            pltpu.VMEM((2, OB, D), BF16),
            pltpu.VMEM((2 * L, 2 * L), F32),
            pltpu.VMEM((8, E), U32),
            pltpu.VMEM((3 * G, 2, D // 2, E), U32),
            pltpu.VMEM((H * E // 2, D), U32),
            pltpu.VMEM((D // 2, D), U32),
            pltpu.VMEM((D // 2, D), U32),
            pltpu.VMEM((D // 2, F), U32),
            pltpu.VMEM((F // 2, D), U32),
            pltpu.SemaphoreType.DMA((S // CH,)),
            pltpu.SemaphoreType.DMA((10,)),
            pltpu.SemaphoreType.DMA((3 * G // NCV,)),
            pltpu.SemaphoreType.DMA((2,)),
        ],
        compiler_params=pltpu.CompilerParams(vmem_limit_bytes=110 * 1024 * 1024),
    )(
        A_x.reshape(S, D),
        A_mem0.reshape(M, D),
        A_Wq.reshape(D // 2, 2, H, E),
        A_Wk.reshape(D // 2, 2, H, E),
        A_Wv.reshape(D // 2, 2, H, E),
        A_Wo.reshape(H * E, D),
        B_w1, B_w2, B_w3, B_w4,
    )
    return out.reshape(1, S, D)
```

```python
import jax
import jax.numpy as jnp
import jax.experimental.pallas as pl
import jax.experimental.pallas.tpu as pltpu

S, D, H, E, M, SEG, F = 2048, 1024, 32, 128, 8, 32, 3584
G = H // 2
L = M + SEG
PAIR = 2 * SEG
NIT = S // PAIR
U = 1
OB = U * PAIR
BR = 48
PRE = S - NIT * BR
RB = 16
CVB = 8
CH2 = 512
CH = 256
NCV = 12
EPS = 1e-5
F32 = jnp.float32
BF16 = jnp.bfloat16
U32 = jnp.uint32


def _ln(x, dep=None):
    m = jnp.sum(x, axis=-1, keepdims=True) * (1.0 / D)
    if dep is not None:
        m = m + dep
    xc = x - m
    v = jnp.sum(xc * xc, axis=-1, keepdims=True) * (1.0 / D)
    r = jax.lax.rsqrt(v + EPS)
    return xc * r, jnp.where(r < 0.0, 1.0, 0.0)


def _gelu(x):
    c1 = 0.7978845608028654
    c2 = c1 * 0.044715
    t = jnp.tanh(x * (c1 + c2 * (x * x)))
    hx = 0.5 * x
    return hx + hx * t


def _silu(x):
    hx = 0.5 * x
    return hx + hx * jnp.tanh(hx)


def _w(ref_val):
    return pltpu.bitcast(ref_val, BF16)


def _kernel(x_hbm, mem_hbm, wq_hbm, wk_hbm, wv_hbm, wo_hbm, w1_hbm, w2_hbm, w3_hbm, w4_hbm,
            out_hbm,
            x_v, xn_v, h_v, x1_v, za_v, zb_v, mem0_v, mem_v, s_v, o_stage, fill_v, zero_v,
            wqkv_v, wo_v, w1_v, w2_v, w3_v, w4_v,
            sem_x, sem_w, sem_qkv, sem_o):
    scale = float(E) ** -0.5

    nch = S // CH
    x_cp = [pltpu.make_async_copy(x_hbm.at[pl.ds(c * CH, CH)], x_v.at[pl.ds(c * CH, CH)], sem_x.at[c])
            for c in range(nch)]
    mem_cp = pltpu.make_async_copy(mem_hbm, mem0_v, sem_w.at[0])
    q4 = D // 4
    w1_cp = [pltpu.make_async_copy(w1_hbm.bitcast(U32).at[:, pl.ds(q * q4, q4)],
                                   w1_v.at[:, pl.ds(q * q4, q4)], sem_w.at[6 + q]) for q in range(4)]
    w2_cp = pltpu.make_async_copy(w2_hbm.bitcast(U32), w2_v, sem_w.at[2])
    w3_cp = pltpu.make_async_copy(w3_hbm.bitcast(U32), w3_v, sem_w.at[3])
    w4_cp = pltpu.make_async_copy(w4_hbm.bitcast(U32), w4_v, sem_w.at[4])
    wo_cp = pltpu.make_async_copy(wo_hbm.bitcast(U32), wo_v, sem_w.at[5])
    srcs = [w.bitcast(U32) for w in (wq_hbm, wk_hbm, wv_hbm)]

    def qkv_cp(n, b):
        return pltpu.make_async_copy(
            srcs[n // G].at[:, b, n % G, :], wqkv_v.at[n, b], sem_qkv.at[n // NCV])

    def qkv_start(n0, n1):
        for n in range(n0, n1):
            for b in range(2):
                qkv_cp(n, b).start()

    x_cp[0].start()
    w1_cp[0].start()
    x_cp[1].start()
    w1_cp[1].start()
    w1_cp[2].start()
    w1_cp[3].start()
    for c in range(2, nch):
        x_cp[c].start()
    w2_cp.start()
    mem_cp.start()
    w3_cp.start()
    w4_cp.start()
    qkv_start(0, 20)

    r = jax.lax.broadcasted_iota(jnp.int32, (2 * L, 2 * L), 0)
    c = jax.lax.broadcasted_iota(jnp.int32, (2 * L, 2 * L), 1)
    same = (r < L) == (c < L)
    rr = jnp.where(r < L, r, r - L)
    cc = jnp.where(c < L, c, c - L)
    ok = (rr < M) | (rr >= cc)
    fill_v[...] = jnp.where(same, jnp.where(ok, 0.0, -1e9), -jnp.inf).astype(F32)
    h_v[pl.ds(0, 8), :] = jnp.zeros((8, D), F32)
    h_v[pl.ds(S + 8, 8), :] = jnp.zeros((8, D), F32)

    s_v[...] = jnp.zeros((OB, D), F32)
    zero_v[...] = jnp.zeros((8, E), U32)

    def norm_chunk(c, z_ref, rb):
        deps = [None, None]
        for b in range(CH // rb):
            r0 = pl.multiple_of(c * CH + b * rb, rb)
            xn, mid = _ln(x_v[pl.ds(r0, rb), :].astype(F32), deps[b % 2])
            if b == 0:
                deps[1] = mid
            xn = xn.astype(BF16).astype(F32)
            xn_v[pl.ds(r0, rb), :] = xn
            z, deps[b % 2] = _ln(xn)
            z_ref[pl.ds(b * rb // 2, rb // 2), :] = pltpu.bitcast(z.astype(BF16), U32)

    def x_wait(c):
        rows = pl.ds(pl.multiple_of(c * CH, CH), CH)
        pltpu.make_async_copy(x_hbm.at[rows], x_v.at[rows], sem_x.at[c]).wait()

    def up1(c, z_ref):
        r0 = pl.multiple_of(c * CH, CH)
        h_v[pl.ds(r0 + 8, CH), :] = _gelu(jnp.dot(_w(z_ref[...]), _w(w1_v[...]), preferred_element_type=F32))

    def up1q(c, z_ref, q, nq):
        w = _w(w1_v[:, pl.ds(q * q4, nq * q4)])
        h_v[pl.ds(c * CH + 8, CH), pl.ds(q * q4, nq * q4)] = _gelu(
            jnp.dot(_w(z_ref[...]), w, preferred_element_type=F32))

    x_cp[0].wait()
    norm_chunk(0, za_v, CH)
    w1_cp[0].wait()
    up1q(0, za_v, 0, 1)
    x_cp[1].wait()
    norm_chunk(1, zb_v, CH)
    w1_cp[1].wait()
    up1q(1, zb_v, 0, 1)
    up1q(0, za_v, 1, 1)
    up1q(1, zb_v, 1, 1)
    w1_cp[2].wait()
    w1_cp[3].wait()
    x_cp[2].wait()
    up1q(0, za_v, 2, 2)
    up1q(1, zb_v, 2, 2)
    norm_chunk(2, za_v, 2 * RB)

    def stage1(i, carry):
        cn = jnp.minimum(2 * i + 2, nch - 1)
        x_wait(2 * i + 1)

        @pl.when(2 * i + 2 < nch)
        def _():
            x_wait(cn)

        up1(2 * i, za_v)
        norm_chunk(2 * i + 1, zb_v, RB)
        up1(2 * i + 1, zb_v)
        norm_chunk(cn, za_v, RB)
        return carry

    jax.lax.fori_loop(1, nch // 2, stage1, 0)
    qkv_start(20, 36)

    w2_cp.wait()

    def norm3(c, rb):
        dep = None
        for b in range(128 // rb):
            z, dep = _ln(x1_v[pl.ds(pl.multiple_of(c * 128 + b * rb, rb), rb), :], dep)
            za_v[pl.ds(b * rb // 2, rb // 2), :] = pltpu.bitcast(z.astype(BF16), U32)

    x1_v[pl.ds(0, 128), :] = jnp.zeros((128, D), F32)

    def stage2(c, carry):
        norm3(0, 16)
        r0 = pl.multiple_of(c * CH2, CH2)
        hb = h_v[pl.ds(r0, CH2 + 16), :]
        hs = jnp.concatenate([
            hb[7:7 + CH2, 0 * q4:1 * q4],
            hb[9:9 + CH2, 1 * q4:2 * q4],
            hb[6:6 + CH2, 2 * q4:3 * q4],
            hb[10:10 + CH2, 3 * q4:4 * q4]], axis=1).astype(BF16)
        x1_v[pl.ds(r0, CH2), :] = xn_v[pl.ds(r0, CH2), :] + jnp.dot(hs, _w(w2_v[...]), preferred_element_type=F32)
        return carry

    jax.lax.fori_loop(0, S // CH2, stage2, 0)
    qkv_start(36, 48)
    wo_cp.start()

    w3_cp.wait()
    w4_cp.wait()

    def mlp_up(r0, n):
        x1 = x1_v[pl.ds(r0, n), :]
        z = _ln(x1)[0].astype(BF16)
        return _gelu(jnp.dot(z, _w(w3_v[...]), preferred_element_type=F32)).astype(BF16)

    def mlp_down(r0, n, h3):
        y = x1_v[pl.ds(r0, n), :] + jnp.dot(h3, _w(w4_v[...]), preferred_element_type=F32)
        h_v[pl.ds(r0, n), :] = _silu(y)

    def stage3(c, carry):
        blk = wqkv_v.at[pl.ds(c * NCV, NCV)]
        pltpu.make_async_copy(blk, blk, sem_qkv.at[c]).wait()
        r0 = pl.multiple_of(c * 128, 128)
        z = _w(za_v[pl.ds(0, 64), :])
        h3 = _gelu(jnp.dot(z, _w(w3_v[...]), preferred_element_type=F32)).astype(BF16)
        zero = zero_v[...]
        dep = zero
        for i in range(NCV):
            n = c * NCV + i
            for r in range(0, D // 2, CVB):
                a = wqkv_v[n, 0, pl.ds(r, CVB), :]
                a = jnp.concatenate([a[:8] | dep, a[8:]], axis=0) if CVB > 8 else a | dep
                b = wqkv_v[n, 1, pl.ds(r, CVB), :]
                lo = (a & jnp.uint32(0xFFFF)) | (b << 16)
                wqkv_v[n, 0, pl.ds(r, CVB), :] = lo
                wqkv_v[n, 1, pl.ds(r, CVB), :] = (a >> 16) | (b & jnp.uint32(0xFFFF0000))
                dep = lo[:8] & zero
        mlp_down(r0, 128, h3)
        norm3(jnp.minimum(c + 1, PRE // 128 - 1), 16)
        return carry

    jax.lax.fori_loop(0, PRE // 128, stage3, 0)
    wo_cp.wait()
    mem_cp.wait()
    mem_v[...] = mem0_v[...].astype(F32)

    def out_cp(j):
        return pltpu.make_async_copy(
            o_stage.at[j % 2], out_hbm.at[pl.ds(pl.multiple_of(j * OB, OB), OB)], sem_o.at[j % 2])

    def combine(j):
        t0 = pl.multiple_of(j * OB, OB)
        o_stage[j % 2] = (x_v[pl.ds(t0, OB), :].astype(F32)
                          + s_v[...] * h_v[pl.ds(t0, OB), :]).astype(BF16)

    def segment(lhs, qkv_extra, o_extra, first):
        qkv_left, o_left = [None] * G, [None] * G
        qkv, sc, olhs = [None] * G, [None] * G, [None] * G

        def do_qkv(g):
            ys = [jnp.dot(lhs, _w(wqkv_v[(c // 2) * G + g, c % 2]), preferred_element_type=F32)
                  for c in range(6)]
            if first:
                qkv_left[g] = [y[L:] for y in ys]
                ys = [y[:L] for y in ys]
            else:
                ys = [jnp.concatenate([y[:M], e, y[M:]], axis=0) for y, e in zip(ys, qkv_extra[g])]
            qkv[g] = [jnp.concatenate([ys[2 * p], ys[2 * p + 1]], axis=0).astype(BF16) for p in range(3)]

        def do_s(g):
            q, k, _ = qkv[g]
            s = jax.lax.dot_general(q, k, (((1,), (1,)), ((), ())), preferred_element_type=F32)
            fill = fill_v[...]
            s = jnp.where(fill == 0.0, s * scale, fill)
            e = jnp.exp(s - jnp.max(s, axis=-1, keepdims=True))
            l = jnp.sum(e, axis=-1, keepdims=True)
            rl = pl.reciprocal(l, approx=True)
            sc[g] = (e.astype(BF16), rl * (2.0 - l * rl))

        def do_pv(g):
            e, rl = sc[g]
            o = jnp.dot(e, qkv[g][2], preferred_element_type=F32) * rl
            oh = [o[:L], o[L:]]
            if first:
                o_left[g] = [t[32:] for t in oh]
                oh = [t[:32] for t in oh]
            else:
                oh = [jnp.concatenate([t[:M], x, t[M:]], axis=0) for t, x in zip(oh, o_extra[g])]
            olhs[g] = jnp.concatenate(oh, axis=1).astype(BF16)

        def do_wo(g0, g1):
            a = jnp.concatenate(olhs[g0:g1], axis=1)
            return jnp.dot(a, _w(wo_v[g0 * E:g1 * E, :]), preferred_element_type=F32)

        for g in range(G):
            do_qkv(g)
            if g >= 2:
                do_pv(g - 2)
            if g >= 1:
                do_s(g - 1)
        acc = do_wo(0, 6)
        do_s(G - 1)
        do_pv(G - 2)
        acc = do_wo(6, 12) + acc
        do_pv(G - 1)
        acc = do_wo(12, 14) + acc
        acc = do_wo(14, 16) + acc
        return acc, qkv_left, o_left

    def body(j, carry):
        @pl.when(j >= 3)
        def _():
            out_cp(jnp.maximum(j - 3, 0)).wait()

        combine(jnp.maximum(j - 1, 0))
        mem = mem_v[...]
        for u in range(U):
            t0 = pl.multiple_of(j * OB + u * PAIR, PAIR)
            b0 = pl.multiple_of(PRE + (j * U + u) * BR, 16)
            lhs = jnp.concatenate([mem, xn_v[pl.ds(t0, 40), :]], axis=0).astype(BF16)
            ra, qkv_left, o_left = segment(lhs, None, None, True)
            s_v[pl.ds(u * PAIR, 24), :] = ra[M:]
            mem = ra[:M].astype(BF16).astype(F32)
            h3 = mlp_up(b0, BR)
            lhs = jnp.concatenate([mem, xn_v[pl.ds(t0 + 40, 24), :]], axis=0).astype(BF16)
            rb, _, _ = segment(lhs, qkv_left, o_left, False)
            s_v[pl.ds(u * PAIR + 24, 40), :] = rb[M:]
            mem = rb[:M].astype(BF16).astype(F32)
            mlp_down(b0, BR, h3)
        mem_v[...] = mem

        @pl.when(j >= 1)
        def _():
            out_cp(jnp.maximum(j - 1, 0)).start()

        return carry

    nj = NIT // U
    jax.lax.fori_loop(0, nj, body, 0)
    out_cp(nj - 3).wait()
    combine(nj - 1)
    out_cp(nj - 1).start()
    out_cp(nj - 2).wait()
    out_cp(nj - 1).wait()


@jax.jit
def pallas_recurrent_scan__memory_aug_recurrent_mem_tr__mixer_s_mlp__prompt_kernel(
    A_x: jax.Array,
    A_mem0: jax.Array,
    A_Wq: jax.Array,
    A_Wk: jax.Array,
    A_Wv: jax.Array,
    A_Wo: jax.Array,
    A_seg_len: jax.Array,
    B_x: jax.Array,
    B_w1: jax.Array,
    B_w2: jax.Array,
    B_w3: jax.Array,
    B_w4: jax.Array,
):
    del A_seg_len, B_x
    assert A_x.shape == (1, S, D) and A_mem0.shape == (1, M, D) and A_Wq.shape == (D, H, E)
    assert B_w3.shape == (D, F)
    any_spec = pl.BlockSpec(memory_space=pl.ANY)
    out = pl.pallas_call(
        _kernel,
        out_shape=jax.ShapeDtypeStruct((S, D), BF16),
        in_specs=[any_spec] * 10,
        out_specs=any_spec,
        scratch_shapes=[
            pltpu.VMEM((S, D), BF16),
            pltpu.VMEM((S, D), F32),
            pltpu.VMEM((S + 16, D), F32),
            pltpu.VMEM((S, D), F32),
            pltpu.VMEM((CH // 2, D), U32),
            pltpu.VMEM((CH // 2, D), U32),
            pltpu.VMEM((M, D), BF16),
            pltpu.VMEM((M, D), F32),
            pltpu.VMEM((OB, D), F32),
            pltpu.VMEM((2, OB, D), BF16),
            pltpu.VMEM((2 * L, 2 * L), F32),
            pltpu.VMEM((8, E), U32),
            pltpu.VMEM((3 * G, 2, D // 2, E), U32),
            pltpu.VMEM((H * E // 2, D), U32),
            pltpu.VMEM((D // 2, D), U32),
            pltpu.VMEM((D // 2, D), U32),
            pltpu.VMEM((D // 2, F), U32),
            pltpu.VMEM((F // 2, D), U32),
            pltpu.SemaphoreType.DMA((S // CH,)),
            pltpu.SemaphoreType.DMA((10,)),
            pltpu.SemaphoreType.DMA((3 * G // NCV,)),
            pltpu.SemaphoreType.DMA((2,)),
        ],
        compiler_params=pltpu.CompilerParams(vmem_limit_bytes=110 * 1024 * 1024, disable_bounds_checks=True, disable_semaphore_checks=True),
    )(
        A_x.reshape(S, D),
        A_mem0.reshape(M, D),
        A_Wq.reshape(D // 2, 2, H, E),
        A_Wk.reshape(D // 2, 2, H, E),
        A_Wv.reshape(D // 2, 2, H, E),
        A_Wo.reshape(H * E, D),
        B_w1, B_w2, B_w3, B_w4,
    )
    return out.reshape(1, S, D)
```

```python
import jax
import jax.numpy as jnp
import jax.experimental.pallas as pl
import jax.experimental.pallas.tpu as pltpu

S, D, H, E, M, SEG, F = 2048, 1024, 32, 128, 8, 32, 3584
G = H // 2
L = M + SEG
PAIR = 2 * SEG
NIT = S // PAIR
U = 2
OB = U * PAIR
BR = 80
CH3 = 128
PRE = S - NIT // U * BR
RB = 16
CVB = 8
CH2 = 512
CH = 256
NCV = 3 * G // (PRE // CH3)
LAG = 4
EPS = 1e-5
F32 = jnp.float32
BF16 = jnp.bfloat16
U32 = jnp.uint32


def _ln(x, dep=None):
    m = jnp.sum(x, axis=-1, keepdims=True) * (1.0 / D)
    if dep is not None:
        m = m + dep
    xc = x - m
    v = jnp.sum(xc * xc, axis=-1, keepdims=True) * (1.0 / D)
    r = jax.lax.rsqrt(v + EPS)
    return xc * r, jnp.where(r < 0.0, 1.0, 0.0)


def _gelu(x):
    c1 = 0.7978845608028654
    c2 = c1 * 0.044715
    t = jnp.tanh(x * (c1 + c2 * (x * x)))
    hx = 0.5 * x
    return hx + hx * t


def _silu(x):
    hx = 0.5 * x
    return hx + hx * jnp.tanh(hx)


def _w(ref_val):
    return pltpu.bitcast(ref_val, BF16)


def _kernel(x_hbm, mem_hbm, wq_hbm, wk_hbm, wv_hbm, wo_hbm, w1_hbm, w2_hbm, w3_hbm, w4_hbm,
            out_hbm,
            x_v, xn_v, h_v, x1_v, za_v, zb_v, mem0_v, mem_v, s_v, o_stage, fill_v, zero_v,
            wqkv_v, wo_v, w1_v, w2_v, w3_v, w4_v,
            sem_x, sem_w, sem_qkv, sem_o):
    scale = float(E) ** -0.5

    nch = S // CH
    x_cp = [pltpu.make_async_copy(x_hbm.at[pl.ds(c * CH, CH)], x_v.at[pl.ds(c * CH, CH)], sem_x.at[c])
            for c in range(nch)]
    mem_cp = pltpu.make_async_copy(mem_hbm, mem0_v, sem_w.at[0])
    q4 = D // 4
    w1_cp = [pltpu.make_async_copy(w1_hbm.bitcast(U32).at[:, pl.ds(q * q4, q4)],
                                   w1_v.at[:, pl.ds(q * q4, q4)], sem_w.at[6 + q]) for q in range(4)]
    w2_cp = pltpu.make_async_copy(w2_hbm.bitcast(U32), w2_v, sem_w.at[2])
    w3_cp = pltpu.make_async_copy(w3_hbm.bitcast(U32), w3_v, sem_w.at[3])
    w4_cp = pltpu.make_async_copy(w4_hbm.bitcast(U32), w4_v, sem_w.at[4])
    wo_cp = pltpu.make_async_copy(wo_hbm.bitcast(U32), wo_v, sem_w.at[5])
    srcs = [w.bitcast(U32) for w in (wq_hbm, wk_hbm, wv_hbm)]

    def qkv_cp(n, b):
        return pltpu.make_async_copy(
            srcs[n // G].at[:, b, n % G, :], wqkv_v.at[n, b], sem_qkv.at[n // NCV])

    def qkv_start(n0, n1):
        for n in range(n0, n1):
            for b in range(2):
                qkv_cp(n, b).start()

    x_cp[0].start()
    w1_cp[0].start()
    x_cp[1].start()
    w1_cp[1].start()
    w1_cp[2].start()
    w1_cp[3].start()
    for c in range(2, nch):
        x_cp[c].start()
    w2_cp.start()
    mem_cp.start()
    w3_cp.start()
    w4_cp.start()
    qkv_start(0, 20)

    r = jax.lax.broadcasted_iota(jnp.int32, (2 * L, 2 * L), 0)
    c = jax.lax.broadcasted_iota(jnp.int32, (2 * L, 2 * L), 1)
    same = (r < L) == (c < L)
    rr = jnp.where(r < L, r, r - L)
    cc = jnp.where(c < L, c, c - L)
    ok = (rr < M) | (rr >= cc)
    fill_v[...] = jnp.where(same, jnp.where(ok, 0.0, -1e9), -jnp.inf).astype(F32)
    h_v[pl.ds(0, 8), :] = jnp.zeros((8, D), F32)
    h_v[pl.ds(S + 8, 8), :] = jnp.zeros((8, D), F32)

    s_v[...] = jnp.zeros((OB, D), F32)
    zero_v[...] = jnp.zeros((8, E), U32)

    def norm_chunk(c, z_ref, rb):
        deps = [None, None]
        for b in range(CH // rb):
            r0 = pl.multiple_of(c * CH + b * rb, rb)
            xn, mid = _ln(x_v[pl.ds(r0, rb), :].astype(F32), deps[b % 2])
            if b == 0:
                deps[1] = mid
            xn = xn.astype(BF16).astype(F32)
            xn_v[pl.ds(r0, rb), :] = xn
            z, deps[b % 2] = _ln(xn)
            z_ref[pl.ds(b * rb // 2, rb // 2), :] = pltpu.bitcast(z.astype(BF16), U32)

    def x_wait(c):
        rows = pl.ds(pl.multiple_of(c * CH, CH), CH)
        pltpu.make_async_copy(x_hbm.at[rows], x_v.at[rows], sem_x.at[c]).wait()

    def up1(c, z_ref):
        r0 = pl.multiple_of(c * CH, CH)
        h_v[pl.ds(r0 + 8, CH), :] = _gelu(jnp.dot(_w(z_ref[...]), _w(w1_v[...]), preferred_element_type=F32))

    def up1q(c, z_ref, q, nq):
        w = _w(w1_v[:, pl.ds(q * q4, nq * q4)])
        h_v[pl.ds(c * CH + 8, CH), pl.ds(q * q4, nq * q4)] = _gelu(
            jnp.dot(_w(z_ref[...]), w, preferred_element_type=F32))

    x_cp[0].wait()
    norm_chunk(0, za_v, CH)
    w1_cp[0].wait()
    up1q(0, za_v, 0, 1)
    x_cp[1].wait()
    norm_chunk(1, zb_v, CH)
    w1_cp[1].wait()
    up1q(1, zb_v, 0, 1)
    up1q(0, za_v, 1, 1)
    up1q(1, zb_v, 1, 1)
    w1_cp[2].wait()
    w1_cp[3].wait()
    x_cp[2].wait()
    up1q(0, za_v, 2, 2)
    up1q(1, zb_v, 2, 2)
    norm_chunk(2, za_v, 2 * RB)

    def stage1(i, carry):
        cn = jnp.minimum(2 * i + 2, nch - 1)
        x_wait(2 * i + 1)

        @pl.when(2 * i + 2 < nch)
        def _():
            x_wait(cn)

        up1(2 * i, za_v)
        norm_chunk(2 * i + 1, zb_v, RB)
        up1(2 * i + 1, zb_v)
        norm_chunk(cn, za_v, RB)
        return carry

    jax.lax.fori_loop(1, nch // 2, stage1, 0)
    qkv_start(20, 36)

    w2_cp.wait()

    def norm3(c, rb):
        dep = None
        for b in range(CH3 // rb):
            z, dep = _ln(x1_v[pl.ds(pl.multiple_of(c * CH3 + b * rb, rb), rb), :], dep)
            za_v[pl.ds(b * rb // 2, rb // 2), :] = pltpu.bitcast(z.astype(BF16), U32)

    x1_v[pl.ds(0, CH3), :] = jnp.zeros((CH3, D), F32)

    def stage2(c, carry):
        norm3(0, 16)
        r0 = pl.multiple_of(c * CH2, CH2)
        hb = h_v[pl.ds(r0, CH2 + 16), :]
        hs = jnp.concatenate([
            hb[7:7 + CH2, 0 * q4:1 * q4],
            hb[9:9 + CH2, 1 * q4:2 * q4],
            hb[6:6 + CH2, 2 * q4:3 * q4],
            hb[10:10 + CH2, 3 * q4:4 * q4]], axis=1).astype(BF16)
        x1_v[pl.ds(r0, CH2), :] = xn_v[pl.ds(r0, CH2), :] + jnp.dot(hs, _w(w2_v[...]), preferred_element_type=F32)
        return carry

    jax.lax.fori_loop(0, S // CH2, stage2, 0)
    qkv_start(36, 48)
    wo_cp.start()

    w3_cp.wait()
    w4_cp.wait()

    def mlp_down(r0, n, h3):
        y = x1_v[pl.ds(r0, n), :] + jnp.dot(h3, _w(w4_v[...]), preferred_element_type=F32)
        h_v[pl.ds(r0, n), :] = _silu(y)

    def stage3(c, carry):
        blk = wqkv_v.at[pl.ds(c * NCV, NCV)]
        pltpu.make_async_copy(blk, blk, sem_qkv.at[c]).wait()
        r0 = pl.multiple_of(c * CH3, CH3)
        z = _w(za_v[pl.ds(0, CH3 // 2), :])
        h3 = _gelu(jnp.dot(z, _w(w3_v[...]), preferred_element_type=F32)).astype(BF16)
        zero = zero_v[...]
        dep = zero
        for i in range(NCV):
            n = c * NCV + i
            for r in range(0, D // 2, CVB):
                a = wqkv_v[n, 0, pl.ds(r, CVB), :]
                a = jnp.concatenate([a[:8] | dep, a[8:]], axis=0) if CVB > 8 else a | dep
                b = wqkv_v[n, 1, pl.ds(r, CVB), :]
                lo = (a & jnp.uint32(0xFFFF)) | (b << 16)
                wqkv_v[n, 0, pl.ds(r, CVB), :] = lo
                wqkv_v[n, 1, pl.ds(r, CVB), :] = (a >> 16) | (b & jnp.uint32(0xFFFF0000))
                dep = lo[:8] & zero
        mlp_down(r0, CH3, h3)
        norm3(jnp.minimum(c + 1, PRE // CH3 - 1), 16)
        return carry

    jax.lax.fori_loop(0, PRE // CH3, stage3, 0)
    wo_cp.wait()
    mem_cp.wait()
    mem_v[...] = mem0_v[...].astype(F32)

    def out_cp(j):
        return pltpu.make_async_copy(
            o_stage.at[j % 2], out_hbm.at[pl.ds(pl.multiple_of(j * OB, OB), OB)], sem_o.at[j % 2])

    def combine(j):
        t0 = pl.multiple_of(j * OB, OB)
        o_stage[j % 2] = (x_v[pl.ds(t0, OB), :].astype(F32)
                          + s_v[...] * h_v[pl.ds(t0, OB), :]).astype(BF16)

    def segment(lhs, qkv_extra, o_extra, first):
        qkv_left, o_left = [None] * G, [None] * G
        qkv, sc, olhs = [None] * G, [None] * G, [None] * G

        def do_qkv(g):
            ys = [jnp.dot(lhs, _w(wqkv_v[(c // 2) * G + g, c % 2]), preferred_element_type=F32)
                  for c in range(6)]
            if first:
                qkv_left[g] = [y[L:] for y in ys]
                ys = [y[:L] for y in ys]
            else:
                ys = [jnp.concatenate([y[:M], e, y[M:]], axis=0) for y, e in zip(ys, qkv_extra[g])]
            qkv[g] = [jnp.concatenate([ys[2 * p], ys[2 * p + 1]], axis=0).astype(BF16) for p in range(3)]

        def do_s(g):
            q, k, _ = qkv[g]
            s = jax.lax.dot_general(q, k, (((1,), (1,)), ((), ())), preferred_element_type=F32)
            fill = fill_v[...]
            s = jnp.where(fill == 0.0, s * scale, fill)
            if g >= LAG:
                w = pltpu.bitcast(olhs[g - LAG], U32)
                parts = [w[r:r + 8, c * E:(c + 1) * E] for r in range(0, w.shape[0], 8) for c in range(2)]
                t = parts[0]
                for q_ in parts[1:]:
                    t = t | q_
                zf = pltpu.bitcast(t & zero_v[...], F32)[:, :2 * L]
                s = jnp.concatenate([s[:8] + zf, s[8:]], axis=0)
            e = jnp.exp(s - jnp.max(s, axis=-1, keepdims=True))
            l = jnp.sum(e, axis=-1, keepdims=True)
            rl = pl.reciprocal(l, approx=True)
            sc[g] = (e.astype(BF16), rl * (2.0 - l * rl))

        def do_pv(g):
            e, rl = sc[g]
            o = jnp.dot(e, qkv[g][2], preferred_element_type=F32) * rl
            oh = [o[:L], o[L:]]
            if first:
                o_left[g] = [t[32:] for t in oh]
                oh = [t[:32] for t in oh]
            else:
                oh = [jnp.concatenate([t[:M], x, t[M:]], axis=0) for t, x in zip(oh, o_extra[g])]
            olhs[g] = jnp.concatenate(oh, axis=1).astype(BF16)

        def do_wo(g0, g1):
            a = jnp.concatenate(olhs[g0:g1], axis=1)
            return jnp.dot(a, _w(wo_v[g0 * E:g1 * E, :]), preferred_element_type=F32)

        for g in range(0, G, 2):
            do_qkv(g)
            do_qkv(g + 1)
            for f, i in ((do_pv, g - 3), (do_pv, g - 2), (do_s, g - 1), (do_s, g)):
                if i >= 0:
                    f(i)
        acc = do_wo(0, 6)
        do_s(G - 1)
        do_pv(G - 3)
        do_pv(G - 2)
        acc = do_wo(6, 12) + acc
        do_pv(G - 1)
        acc = do_wo(12, 14) + acc
        acc = do_wo(14, 16) + acc
        return acc, qkv_left, o_left

    def body(j, carry):
        @pl.when(j >= 3)
        def _():
            out_cp(jnp.maximum(j - 3, 0)).wait()

        combine(jnp.maximum(j - 1, 0))
        b0 = pl.multiple_of(PRE + j * BR, 16)
        z = _ln(x1_v[pl.ds(b0, BR), :])[0].astype(BF16)
        h3 = []

        def up(c0, c1):
            h3.append(_gelu(jnp.dot(z, _w(w3_v[:, c0:c1]), preferred_element_type=F32)).astype(BF16))

        fillers = [lambda: up(0, 10 * E), lambda: up(10 * E, 19 * E), lambda: up(19 * E, F),
                   lambda: mlp_down(b0, BR, jnp.concatenate(h3, axis=1))]
        mem = mem_v[...]
        for u in range(U):
            t0 = pl.multiple_of(j * OB + u * PAIR, PAIR)
            lhs = jnp.concatenate([mem, xn_v[pl.ds(t0, 40), :]], axis=0).astype(BF16)
            ra, qkv_left, o_left = segment(lhs, None, None, True)
            s_v[pl.ds(u * PAIR, 24), :] = ra[M:]
            mem = ra[:M].astype(BF16).astype(F32)
            fillers[2 * u]()
            lhs = jnp.concatenate([mem, xn_v[pl.ds(t0 + 40, 24), :]], axis=0).astype(BF16)
            rb, _, _ = segment(lhs, qkv_left, o_left, False)
            s_v[pl.ds(u * PAIR + 24, 40), :] = rb[M:]
            mem = rb[:M].astype(BF16).astype(F32)
            fillers[2 * u + 1]()
        mem_v[...] = mem

        @pl.when(j >= 1)
        def _():
            out_cp(jnp.maximum(j - 1, 0)).start()

        return carry

    nj = NIT // U
    jax.lax.fori_loop(0, nj, body, 0)
    out_cp(nj - 3).wait()
    combine(nj - 1)
    out_cp(nj - 1).start()
    out_cp(nj - 2).wait()
    out_cp(nj - 1).wait()


@jax.jit
def pallas_recurrent_scan__memory_aug_recurrent_mem_tr__mixer_s_mlp__prompt_kernel(
    A_x: jax.Array,
    A_mem0: jax.Array,
    A_Wq: jax.Array,
    A_Wk: jax.Array,
    A_Wv: jax.Array,
    A_Wo: jax.Array,
    A_seg_len: jax.Array,
    B_x: jax.Array,
    B_w1: jax.Array,
    B_w2: jax.Array,
    B_w3: jax.Array,
    B_w4: jax.Array,
):
    del A_seg_len, B_x
    assert A_x.shape == (1, S, D) and A_mem0.shape == (1, M, D) and A_Wq.shape == (D, H, E)
    assert B_w3.shape == (D, F)
    any_spec = pl.BlockSpec(memory_space=pl.ANY)
    out = pl.pallas_call(
        _kernel,
        out_shape=jax.ShapeDtypeStruct((S, D), BF16),
        in_specs=[any_spec] * 10,
        out_specs=any_spec,
        scratch_shapes=[
            pltpu.VMEM((S, D), BF16),
            pltpu.VMEM((S, D), F32),
            pltpu.VMEM((S + 16, D), F32),
            pltpu.VMEM((S, D), F32),
            pltpu.VMEM((CH // 2, D), U32),
            pltpu.VMEM((CH // 2, D), U32),
            pltpu.VMEM((M, D), BF16),
            pltpu.VMEM((M, D), F32),
            pltpu.VMEM((OB, D), F32),
            pltpu.VMEM((2, OB, D), BF16),
            pltpu.VMEM((2 * L, 2 * L), F32),
            pltpu.VMEM((8, E), U32),
            pltpu.VMEM((3 * G, 2, D // 2, E), U32),
            pltpu.VMEM((H * E // 2, D), U32),
            pltpu.VMEM((D // 2, D), U32),
            pltpu.VMEM((D // 2, D), U32),
            pltpu.VMEM((D // 2, F), U32),
            pltpu.VMEM((F // 2, D), U32),
            pltpu.SemaphoreType.DMA((S // CH,)),
            pltpu.SemaphoreType.DMA((10,)),
            pltpu.SemaphoreType.DMA((3 * G // NCV,)),
            pltpu.SemaphoreType.DMA((2,)),
        ],
        compiler_params=pltpu.CompilerParams(vmem_limit_bytes=110 * 1024 * 1024, disable_bounds_checks=True, disable_semaphore_checks=True),
    )(
        A_x.reshape(S, D),
        A_mem0.reshape(M, D),
        A_Wq.reshape(D // 2, 2, H, E),
        A_Wk.reshape(D // 2, 2, H, E),
        A_Wv.reshape(D // 2, 2, H, E),
        A_Wo.reshape(H * E, D),
        B_w1, B_w2, B_w3, B_w4,
    )
    return out.reshape(1, S, D)
```

```python
import jax
import jax.numpy as jnp
import jax.experimental.pallas as pl
import jax.experimental.pallas.tpu as pltpu

S, D, H, E, M, SEG, F = 2048, 1024, 32, 128, 8, 32, 3584
G = H // 2
L = M + SEG
PAIR = 2 * SEG
NIT = S // PAIR
U = 2
OB = U * PAIR
BR = 80
CH3 = 128
PRE = S - NIT // U * BR
RB = 16
CVB = 8
CH2 = 512
CH = 256
NCV = 3 * G // (PRE // CH3)
LAG = 4
CHK = 0
NCH = 2
NCHB = 2
NVB = 1
GV = 16
VLAG = 1
GVB = 16
WOB = 8
KC = 4
QCHAIN = False
TAIL_UP = (0, 0, 0)
NV = 2
LM = L - 8 * NV
LOG2E = 1.4426950408889634
EPS = 1e-5
F32 = jnp.float32
BF16 = jnp.bfloat16
U32 = jnp.uint32


def _ln(x, dep=None):
    m = jnp.sum(x, axis=-1, keepdims=True) * (1.0 / D)
    if dep is not None:
        m = m + dep
    xc = x - m
    v = jnp.sum(xc * xc, axis=-1, keepdims=True) * (1.0 / D)
    r = jax.lax.rsqrt(v + EPS)
    return xc * r, jnp.where(r < 0.0, 1.0, 0.0)


def _gelu(x):
    c1 = 0.7978845608028654
    c2 = c1 * 0.044715
    t = jnp.tanh(x * (c1 + c2 * (x * x)))
    hx = 0.5 * x
    return hx + hx * t


def _silu(x):
    hx = 0.5 * x
    return hx + hx * jnp.tanh(hx)


def _w(ref_val):
    return pltpu.bitcast(ref_val, BF16)


def _kernel(x_hbm, mem_hbm, wq_hbm, wk_hbm, wv_hbm, wo_hbm, w1_hbm, w2_hbm, w3_hbm, w4_hbm,
            out_hbm,
            x_v, xn_v, h_v, x1_v, za_v, zb_v, mem0_v, mem_v, s_v, o_stage, fill_v, fillb_v, fillc_v, kv_v, zero_v,
            wqkv_v, wo_v, w1_v, w2_v, w3_v, w4_v,
            sem_x, sem_w, sem_qkv, sem_o):
    scale = float(E) ** -0.5

    nch = S // CH
    x_cp = [pltpu.make_async_copy(x_hbm.at[pl.ds(c * CH, CH)], x_v.at[pl.ds(c * CH, CH)], sem_x.at[c])
            for c in range(nch)]
    mem_cp = pltpu.make_async_copy(mem_hbm, mem0_v, sem_w.at[0])
    q4 = D // 4
    w1_cp = [pltpu.make_async_copy(w1_hbm.bitcast(U32).at[:, pl.ds(q * q4, q4)],
                                   w1_v.at[:, pl.ds(q * q4, q4)], sem_w.at[6 + q]) for q in range(4)]
    w2_cp = pltpu.make_async_copy(w2_hbm.bitcast(U32), w2_v, sem_w.at[2])
    w3_cp = pltpu.make_async_copy(w3_hbm.bitcast(U32), w3_v, sem_w.at[3])
    w4_cp = pltpu.make_async_copy(w4_hbm.bitcast(U32), w4_v, sem_w.at[4])
    wo_cp = pltpu.make_async_copy(wo_hbm.bitcast(U32), wo_v, sem_w.at[5])
    srcs = [w.bitcast(U32) for w in (wq_hbm, wk_hbm, wv_hbm)]

    def qkv_cp(n, b):
        return pltpu.make_async_copy(
            srcs[n // G].at[:, b, n % G, :], wqkv_v.at[n, b], sem_qkv.at[n // NCV])

    def qkv_start(n0, n1):
        for n in range(n0, n1):
            for b in range(2):
                qkv_cp(n, b).start()

    x_cp[0].start()
    w1_cp[0].start()
    x_cp[1].start()
    w1_cp[1].start()
    w1_cp[2].start()
    w1_cp[3].start()
    for c in range(2, nch):
        x_cp[c].start()
    w2_cp.start()
    mem_cp.start()
    w3_cp.start()
    w4_cp.start()
    qkv_start(0, 20)

    for ref, lm in ((fill_v, LM), (fillb_v, L - 8 * NVB), (fillc_v, L)):
        r = jax.lax.broadcasted_iota(jnp.int32, (2 * lm, 2 * L), 0)
        c = jax.lax.broadcasted_iota(jnp.int32, (2 * lm, 2 * L), 1)
        same = (r < lm) == (c < L)
        rr = jnp.where(r < lm, r, r - lm)
        cc = jnp.where(c < L, c, c - L)
        ok = (rr < M) | (rr + (L - lm) >= cc)
        ref[...] = jnp.where(same, jnp.where(ok, 0.0, -1e9), -jnp.inf).astype(F32)
    h_v[pl.ds(0, 8), :] = jnp.zeros((8, D), F32)
    h_v[pl.ds(S + 8, 8), :] = jnp.zeros((8, D), F32)

    s_v[...] = jnp.zeros((OB, D), F32)
    zero_v[...] = jnp.zeros((8, E), U32)

    def norm_chunk(c, z_ref, rb):
        deps = [None, None]
        for b in range(CH // rb):
            r0 = pl.multiple_of(c * CH + b * rb, rb)
            xn, mid = _ln(x_v[pl.ds(r0, rb), :].astype(F32), deps[b % 2])
            if b == 0:
                deps[1] = mid
            xn = xn.astype(BF16).astype(F32)
            xn_v[pl.ds(r0, rb), :] = xn
            z, deps[b % 2] = _ln(xn)
            z_ref[pl.ds(b * rb // 2, rb // 2), :] = pltpu.bitcast(z.astype(BF16), U32)

    def x_wait(c):
        rows = pl.ds(pl.multiple_of(c * CH, CH), CH)
        pltpu.make_async_copy(x_hbm.at[rows], x_v.at[rows], sem_x.at[c]).wait()

    def up1(c, z_ref):
        r0 = pl.multiple_of(c * CH, CH)
        h_v[pl.ds(r0 + 8, CH), :] = _gelu(jnp.dot(_w(z_ref[...]), _w(w1_v[...]), preferred_element_type=F32))

    def up1q(c, z_ref, q, nq):
        w = _w(w1_v[:, pl.ds(q * q4, nq * q4)])
        h_v[pl.ds(c * CH + 8, CH), pl.ds(q * q4, nq * q4)] = _gelu(
            jnp.dot(_w(z_ref[...]), w, preferred_element_type=F32))

    x_cp[0].wait()
    norm_chunk(0, za_v, CH)
    w1_cp[0].wait()
    up1q(0, za_v, 0, 1)
    x_cp[1].wait()
    norm_chunk(1, zb_v, CH)
    w1_cp[1].wait()
    up1q(1, zb_v, 0, 1)
    up1q(0, za_v, 1, 1)
    up1q(1, zb_v, 1, 1)
    w1_cp[2].wait()
    w1_cp[3].wait()
    x_cp[2].wait()
    up1q(0, za_v, 2, 2)
    up1q(1, zb_v, 2, 2)
    norm_chunk(2, za_v, 2 * RB)

    def stage1(i, carry):
        cn = jnp.minimum(2 * i + 2, nch - 1)
        x_wait(2 * i + 1)

        @pl.when(2 * i + 2 < nch)
        def _():
            x_wait(cn)

        up1(2 * i, za_v)
        norm_chunk(2 * i + 1, zb_v, RB)
        up1(2 * i + 1, zb_v)
        norm_chunk(cn, za_v, RB)
        return carry

    jax.lax.fori_loop(1, nch // 2, stage1, 0)
    qkv_start(20, 36)

    w2_cp.wait()

    def norm3(c, rb):
        dep = None
        for b in range(CH3 // rb):
            z, dep = _ln(x1_v[pl.ds(pl.multiple_of(c * CH3 + b * rb, rb), rb), :], dep)
            za_v[pl.ds(b * rb // 2, rb // 2), :] = pltpu.bitcast(z.astype(BF16), U32)

    x1_v[pl.ds(0, CH3), :] = jnp.zeros((CH3, D), F32)

    def stage2(c, carry):
        norm3(0, 16)
        r0 = pl.multiple_of(c * CH2, CH2)
        hb = h_v[pl.ds(r0, CH2 + 16), :]
        hs = jnp.concatenate([
            hb[7:7 + CH2, 0 * q4:1 * q4],
            hb[9:9 + CH2, 1 * q4:2 * q4],
            hb[6:6 + CH2, 2 * q4:3 * q4],
            hb[10:10 + CH2, 3 * q4:4 * q4]], axis=1).astype(BF16)
        x1_v[pl.ds(r0, CH2), :] = xn_v[pl.ds(r0, CH2), :] + jnp.dot(hs, _w(w2_v[...]), preferred_element_type=F32)
        return carry

    jax.lax.fori_loop(0, S // CH2, stage2, 0)
    qkv_start(36, 48)
    wo_cp.start()

    w3_cp.wait()
    w4_cp.wait()

    def mlp_down(r0, n, h3):
        y = x1_v[pl.ds(r0, n), :] + jnp.dot(h3, _w(w4_v[...]), preferred_element_type=F32)
        h_v[pl.ds(r0, n), :] = _silu(y)

    def stage3(c, carry):
        blk = wqkv_v.at[pl.ds(c * NCV, NCV)]
        pltpu.make_async_copy(blk, blk, sem_qkv.at[c]).wait()
        r0 = pl.multiple_of(c * CH3, CH3)
        z = _w(za_v[pl.ds(0, CH3 // 2), :])
        h3 = _gelu(jnp.dot(z, _w(w3_v[...]), preferred_element_type=F32)).astype(BF16)
        zero = zero_v[...]
        dep = zero
        for i in range(NCV):
            n = c * NCV + i
            for r in range(0, D // 2, CVB):
                a = wqkv_v[n, 0, pl.ds(r, CVB), :]
                a = jnp.concatenate([a[:8] | dep, a[8:]], axis=0) if CVB > 8 else a | dep
                b = wqkv_v[n, 1, pl.ds(r, CVB), :]
                lo = (a & jnp.uint32(0xFFFF)) | (b << 16)
                wqkv_v[n, 0, pl.ds(r, CVB), :] = lo
                wqkv_v[n, 1, pl.ds(r, CVB), :] = (a >> 16) | (b & jnp.uint32(0xFFFF0000))
                dep = lo[:8] & zero
        mlp_down(r0, CH3, h3)
        norm3(jnp.minimum(c + 1, PRE // CH3 - 1), 16)
        return carry

    jax.lax.fori_loop(0, PRE // CH3, stage3, 0)
    wo_cp.wait()
    mem_cp.wait()
    mem_v[...] = mem0_v[...].astype(F32)

    def out_cp(j):
        return pltpu.make_async_copy(
            o_stage.at[j % 2], out_hbm.at[pl.ds(pl.multiple_of(j * OB, OB), OB)], sem_o.at[j % 2])

    def combine(j):
        t0 = pl.multiple_of(j * OB, OB)
        o_stage[j % 2] = (x_v[pl.ds(t0, OB), :].astype(F32)
                          + s_v[...] * h_v[pl.ds(t0, OB), :]).astype(BF16)

    zero_v_f32 = jnp.zeros((8, E), F32)

    def zero_of(x):
        return pltpu.bitcast(pltpu.bitcast(x[:8, :E], U32) & zero_v[...], F32)

    def vpu_attn(slot, g, h, b, dep):
        row = jax.lax.broadcasted_iota(jnp.int32, (8, 1), 0)
        q = (kv_v[slot, g, h, pl.ds(M + 8 * b, 8), :] + dep) * (scale * LOG2E)
        nk = M + 8 * b + 8
        m = acc = l = None
        for k0 in range(0, nk, KC):
            ss = []
            for k in range(k0, k0 + KC):
                t = jnp.sum(q * kv_v[slot, g, 2 + h, pl.ds(k, 8, stride=0), :], axis=-1, keepdims=True)
                if k > nk - 8:
                    t = jnp.where(row >= k - (nk - 8), t, -1e9 * LOG2E)
                ss.append(t)
            ms = ss
            while len(ms) > 1:
                ms = [jnp.maximum(ms[i], ms[i + 1]) for i in range(0, len(ms), 2)]
            if m is None:
                m = ms[0]
            else:
                mn = jnp.maximum(m, ms[0])
                a = jnp.exp2(m - mn)
                m, l, acc = mn, l * a, acc * a
            for i, t in enumerate(ss):
                e = jnp.exp2(t - m)
                t = e * kv_v[slot, g, 4 + h, pl.ds(k0 + i, 8, stride=0), :]
                l = e if l is None else l + e
                acc = t if acc is None else acc + t
            if k0 + KC == nk - CHK * KC:
                dep = zero_of(acc)
            if QCHAIN and k0 + KC < nk:
                q = q + zero_of(jnp.broadcast_to(m, (8, E)))
        rl = pl.reciprocal(l, approx=True)
        return acc * (rl * (2.0 - l * rl)), dep

    def segment(lhs, qkv_extra, o_extra, first, fill_tail):
        qkv_left = [None] * G
        qkv, sc, om, olhs = ([None] * G for _ in range(4))
        ov = [[[None] * NV for _ in range(2)] for _ in range(G)]
        nblks = [(NV if g < GV else 0) if first else (NVB if g < GVB else 0) for g in range(G)]
        slot = 0 if first else 1

        def vpu(g, h, b, chain):
            if ov[g][h][b] is None:
                dep = chain.pop(0)
                ov[g][h][b], dep = vpu_attn(slot, g, h, b, dep)
                chain.append(dep)
            return ov[g][h][b]

        chain = [zero_v_f32] * NCH

        def do_qkv(g):
            ys = [jnp.dot(lhs, _w(wqkv_v[(c // 2) * G + g, c % 2]), preferred_element_type=F32)
                  for c in range(6)]
            if first:
                qkv_left[g] = [y[L:] for y in ys]
                ys = [y[:L] for y in ys]
            else:
                ys = [jnp.concatenate([y[:M], e, y[M:]], axis=0) for y, e in zip(ys, qkv_extra[g])]
            nv = M + 8 * nblks[g]
            if nblks[g]:
                for i in range(6):
                    lo = M if i < 2 else 0
                    kv_v[slot, g, i, pl.ds(lo, nv - lo), :] = ys[i][lo:nv]
            qm = jnp.concatenate([ys[0][:M], ys[0][nv:], ys[1][:M], ys[1][nv:]], axis=0).astype(BF16)
            qkv[g] = [qm] + [jnp.concatenate([ys[2 * p], ys[2 * p + 1]], axis=0).astype(BF16) for p in (1, 2)]

        def anchor(s, vals):
            t = None
            for v in vals:
                w = pltpu.bitcast(v, U32)
                for r in range(0, w.shape[0], 8):
                    for c in range(0, w.shape[1], E):
                        p = w[r:r + 8, c:c + E]
                        t = p if t is None else t | p
            zf = pltpu.bitcast(t & zero_v[...], F32)[:, :2 * L]
            return jnp.concatenate([s[:8] + zf, s[8:]], axis=0)

        def do_s(g):
            q, k, _ = qkv[g]
            s = jax.lax.dot_general(q, k, (((1,), (1,)), ((), ())), preferred_element_type=F32)
            fill = (fillc_v if nblks[g] == 0 else fill_v if first else fillb_v)[...]
            s = jnp.where(fill == 0.0, s * scale, fill)
            if first:
                vals = [olhs[g - 4]] if g >= 4 else []
                if 0 <= g - VLAG < GV:
                    vals += [vpu(g - VLAG, h, b, chain) for b in range(NV) for h in range(2)]
                if vals:
                    s = anchor(s, vals)
            if not first and g >= 8:
                s = anchor(s, om[g - 8])
            e = jnp.exp(s - jnp.max(s, axis=-1, keepdims=True))
            l = jnp.sum(e, axis=-1, keepdims=True)
            rl = pl.reciprocal(l, approx=True)
            sc[g] = (e.astype(BF16), rl * (2.0 - l * rl))

        def do_pv(g):
            e, rl = sc[g]
            o = jnp.dot(e, qkv[g][2], preferred_element_type=F32) * rl
            lm = L - 8 * nblks[g]
            om[g] = [o[:lm], o[lm:]]
            if nblks[g] == 0:
                nmax = NV if first else NVB
                for h in range(2):
                    t = om[g][h]
                    ov[g][h][:nmax] = [t[M + 8 * b:M + 8 * b + 8] for b in range(nmax)]
                    om[g][h] = jnp.concatenate([t[:M], t[M + 8 * nmax:]], axis=0)
            if first:
                set_olhs(g, [[vpu(g, h, b, chain) for b in range(NV - 1)] for h in range(2)])

        def set_olhs(g, mid):
            oh = [jnp.concatenate([t[:M]] + x + [t[M:]], axis=0) for t, x in zip(om[g], mid)]
            olhs[g] = jnp.concatenate(oh, axis=1).astype(BF16)

        def do_wo(g0, g1):
            a = jnp.concatenate(olhs[g0:g1], axis=1)
            return jnp.dot(a, _w(wo_v[g0 * E:g1 * E, :]), preferred_element_type=F32)

        if first:
            for g in range(0, G, 2):
                do_qkv(g)
                do_qkv(g + 1)
                for f, i in ((do_pv, g - 3), (do_pv, g - 2), (do_s, g - 1), (do_s, g)):
                    if i >= 0:
                        f(i)
            acc = do_wo(0, 6)
            do_s(G - 1)
            do_pv(G - 3)
            do_pv(G - 2)
            acc = do_wo(6, 12) + acc
            do_pv(G - 1)
            acc = do_wo(12, 14) + acc
            acc = do_wo(14, 16) + acc
        else:
            for g in range(0, G, 4):
                for i in range(4):
                    do_qkv(g + i)
                for f, i in [(do_pv, g - 5 + i) for i in range(4)] + [(do_s, g - 1 + i) for i in range(4)]:
                    if i >= 0:
                        f(i)
            start = fill_tail[0]()
            do_s(G - 1)
            for i in range(4):
                do_pv(G - 5 + i)
            fill_tail[1]()
            do_pv(G - 1)
            fill_tail[2]()
            chain = [zero_of(start)] * NCHB
            for g in range(G):
                set_olhs(g, [[o_extra(g, h, NV - 1, chain)] + [vpu(g, h, b, chain) for b in range(NVB)]
                             for h in range(2)])
            acc = do_wo(0, WOB)
            acc = do_wo(WOB, G) + acc
        return acc, qkv_left, vpu

    def body(j, carry):
        @pl.when(j >= 3)
        def _():
            out_cp(jnp.maximum(j - 3, 0)).wait()

        combine(jnp.maximum(j - 1, 0))
        b0 = pl.multiple_of(PRE + j * BR, 16)
        x1 = x1_v[pl.ds(b0, BR), :]
        z = _ln(x1)[0].astype(BF16)
        h3 = []

        def up(n):
            c0 = len(h3) * E
            t = jnp.dot(z, _w(w3_v[:, c0:c0 + n * E]), preferred_element_type=F32)
            g_ = _gelu(t).astype(BF16)
            h3.extend(g_[:, i * E:(i + 1) * E] for i in range(n))
            return t

        def down(c0, c1):
            t = jnp.dot(jnp.concatenate(h3, axis=1), _w(w4_v[:, c0 * E:c1 * E]), preferred_element_type=F32)
            h_v[pl.ds(b0, BR), c0 * E:c1 * E] = _silu(x1[:, c0 * E:c1 * E] + t)
            return t

        tails = [[lambda: up(3), lambda: up(3), lambda: up(16)],
                 [lambda: down(0, 1), lambda: down(1, 2), lambda: down(2, 8)]]
        fillers = [lambda: up(2), lambda: up(2), lambda: up(2), lambda: None]
        mem = mem_v[...]
        nb = 8 * (NV - 1)
        for u in range(U):
            t0 = pl.multiple_of(j * OB + u * PAIR, PAIR)
            lhs = jnp.concatenate([mem, xn_v[pl.ds(t0, 40), :]], axis=0).astype(BF16)
            ra, qkv_left, vpu = segment(lhs, None, None, True, None)
            if nb:
                s_v[pl.ds(u * PAIR, nb), :] = ra[M:M + nb]
            s_v[pl.ds(u * PAIR + nb + 8, 24 - nb), :] = ra[M + nb:]
            mem = ra[:M].astype(BF16).astype(F32)
            fillers[2 * u]()
            lhs = jnp.concatenate([mem, xn_v[pl.ds(t0 + 40, 24), :]], axis=0).astype(BF16)
            rb, _, _ = segment(lhs, qkv_left, vpu, False, tails[u])
            s_v[pl.ds(u * PAIR + nb, 8), :] = rb[M:2 * M]
            s_v[pl.ds(u * PAIR + SEG, SEG), :] = rb[2 * M:]
            mem = rb[:M].astype(BF16).astype(F32)
            fillers[2 * u + 1]()
        mem_v[...] = mem

        @pl.when(j >= 1)
        def _():
            out_cp(jnp.maximum(j - 1, 0)).start()

        return carry

    nj = NIT // U
    jax.lax.fori_loop(0, nj, body, 0)
    out_cp(nj - 3).wait()
    combine(nj - 1)
    out_cp(nj - 1).start()
    out_cp(nj - 2).wait()
    out_cp(nj - 1).wait()


@jax.jit
def pallas_recurrent_scan__memory_aug_recurrent_mem_tr__mixer_s_mlp__prompt_kernel(
    A_x: jax.Array,
    A_mem0: jax.Array,
    A_Wq: jax.Array,
    A_Wk: jax.Array,
    A_Wv: jax.Array,
    A_Wo: jax.Array,
    A_seg_len: jax.Array,
    B_x: jax.Array,
    B_w1: jax.Array,
    B_w2: jax.Array,
    B_w3: jax.Array,
    B_w4: jax.Array,
):
    del A_seg_len, B_x
    assert A_x.shape == (1, S, D) and A_mem0.shape == (1, M, D) and A_Wq.shape == (D, H, E)
    assert B_w3.shape == (D, F)
    any_spec = pl.BlockSpec(memory_space=pl.ANY)
    out = pl.pallas_call(
        _kernel,
        out_shape=jax.ShapeDtypeStruct((S, D), BF16),
        in_specs=[any_spec] * 10,
        out_specs=any_spec,
        scratch_shapes=[
            pltpu.VMEM((S, D), BF16),
            pltpu.VMEM((S, D), F32),
            pltpu.VMEM((S + 16, D), F32),
            pltpu.VMEM((S, D), F32),
            pltpu.VMEM((CH // 2, D), U32),
            pltpu.VMEM((CH // 2, D), U32),
            pltpu.VMEM((M, D), BF16),
            pltpu.VMEM((M, D), F32),
            pltpu.VMEM((OB, D), F32),
            pltpu.VMEM((2, OB, D), BF16),
            pltpu.VMEM((2 * LM, 2 * L), F32),
            pltpu.VMEM((2 * (L - 8 * NVB), 2 * L), F32),
            pltpu.VMEM((2 * L, 2 * L), F32),
            pltpu.VMEM((2, G, 6, M + 8 * NV, E), F32),
            pltpu.VMEM((8, E), U32),
            pltpu.VMEM((3 * G, 2, D // 2, E), U32),
            pltpu.VMEM((H * E // 2, D), U32),
            pltpu.VMEM((D // 2, D), U32),
            pltpu.VMEM((D // 2, D), U32),
            pltpu.VMEM((D // 2, F), U32),
            pltpu.VMEM((F // 2, D), U32),
            pltpu.SemaphoreType.DMA((S // CH,)),
            pltpu.SemaphoreType.DMA((10,)),
            pltpu.SemaphoreType.DMA((3 * G // NCV,)),
            pltpu.SemaphoreType.DMA((2,)),
        ],
        compiler_params=pltpu.CompilerParams(vmem_limit_bytes=110 * 1024 * 1024, disable_bounds_checks=True, disable_semaphore_checks=True),
    )(
        A_x.reshape(S, D),
        A_mem0.reshape(M, D),
        A_Wq.reshape(D // 2, 2, H, E),
        A_Wk.reshape(D // 2, 2, H, E),
        A_Wv.reshape(D // 2, 2, H, E),
        A_Wo.reshape(H * E, D),
        B_w1, B_w2, B_w3, B_w4,
    )
    return out.reshape(1, S, D)
```

```python
import jax
import jax.numpy as jnp
import jax.experimental.pallas as pl
import jax.experimental.pallas.tpu as pltpu

S, D, H, E, M, SEG, F = 2048, 1024, 32, 128, 8, 32, 3584
G = H // 2
L = M + SEG
PAIR = 2 * SEG
OB = 4 * SEG
NJ = S // OB
BR = 80
PRE = S - NJ * BR
CH = 256
CH2 = 512
CH3 = 128
RB = 16
NCV = 3 * G // (PRE // CH3)
NV = (2, 1)
NCH = 2
KC = 4
PLAN = (
    dict(wo=((0, 0), (0, 2), (0, 3)), tail=(None,) * 4, cuts=(0, 6, 12, 14, 16), end=("u", 2)),
    dict(wo=((0, 1), (1, 0), (1, 1), (1, 2), (1, 3)), tail=(("u", 3), ("u", 3), ("u", 16), None),
         cuts=(0, 0, 0, 10, 16), end=("u", 2)),
    dict(wo=((2, 0), (2, 2), (2, 3)), tail=(None,) * 4, cuts=(0, 6, 12, 14, 16), end=("u", 2)),
    dict(wo=((2, 1), (3, 0), (3, 1), (3, 2), (3, 3)), tail=(("d", 1), ("d", 1), ("d", 6), None),
         cuts=(0, 0, 0, 10, 16), end=None),
)
EPS = 1e-5
LOG2E = 1.4426950408889634
F32 = jnp.float32
BF16 = jnp.bfloat16
U32 = jnp.uint32


def _ln(x, dep=None):
    m = jnp.sum(x, axis=-1, keepdims=True) * (1.0 / D)
    if dep is not None:
        m = m + dep
    xc = x - m
    v = jnp.sum(xc * xc, axis=-1, keepdims=True) * (1.0 / D)
    r = jax.lax.rsqrt(v + EPS)
    return xc * r, jnp.where(r < 0.0, 1.0, 0.0)


def _gelu(x):
    c1 = 0.7978845608028654
    c2 = c1 * 0.044715
    t = jnp.tanh(x * (c1 + c2 * (x * x)))
    hx = 0.5 * x
    return hx + hx * t


def _silu(x):
    hx = 0.5 * x
    return hx + hx * jnp.tanh(hx)


def _recip(l):
    r = pl.reciprocal(l, approx=True)
    return r * (2.0 - l * r)


def _w(packed):
    return pltpu.bitcast(packed, BF16)


def _kernel(x_hbm, mem_hbm, wq_hbm, wk_hbm, wv_hbm, wo_hbm, w1_hbm, w2_hbm, w3_hbm, w4_hbm,
            out_hbm,
            x_v, xn_v, h_v, x1_v, za_v, zb_v, mem0_v, mem_v, s_v, o_stage, filla_v, fillb_v, kv_v, zero_v,
            wqkv_v, wo_v, w1_v, w2_v, w3_v, w4_v,
            sem_x, sem_w, sem_qkv, sem_o):
    scale = float(E) ** -0.5

    nch = S // CH
    q4 = D // 4
    x_cp = [pltpu.make_async_copy(x_hbm.at[pl.ds(c * CH, CH)], x_v.at[pl.ds(c * CH, CH)], sem_x.at[c])
            for c in range(nch)]
    w1_cp = [pltpu.make_async_copy(w1_hbm.bitcast(U32).at[:, pl.ds(q * q4, q4)],
                                   w1_v.at[:, pl.ds(q * q4, q4)], sem_w.at[q]) for q in range(4)]
    w2_cp = pltpu.make_async_copy(w2_hbm.bitcast(U32), w2_v, sem_w.at[4])
    w3_cp = pltpu.make_async_copy(w3_hbm.bitcast(U32), w3_v, sem_w.at[5])
    w4_cp = pltpu.make_async_copy(w4_hbm.bitcast(U32), w4_v, sem_w.at[6])
    wo_cp = pltpu.make_async_copy(wo_hbm.bitcast(U32), wo_v, sem_w.at[7])
    mem_cp = pltpu.make_async_copy(mem_hbm, mem0_v, sem_w.at[8])
    srcs = [w.bitcast(U32) for w in (wq_hbm, wk_hbm, wv_hbm)]

    def qkv_start(n0, n1):
        for n in range(n0, n1):
            for b in range(2):
                pltpu.make_async_copy(
                    srcs[n // G].at[:, b, n % G, :], wqkv_v.at[n, b], sem_qkv.at[n // NCV]).start()

    x_cp[0].start()
    w1_cp[0].start()
    x_cp[1].start()
    w1_cp[1].start()
    w1_cp[2].start()
    w1_cp[3].start()
    for c in range(2, nch):
        x_cp[c].start()
    w2_cp.start()
    mem_cp.start()
    w3_cp.start()
    w4_cp.start()
    qkv_start(0, 20)

    for ref, nblk in ((filla_v, NV[0]), (fillb_v, NV[1])):
        lm = L - 8 * nblk
        r = jax.lax.broadcasted_iota(jnp.int32, (2 * lm, 2 * L), 0)
        c = jax.lax.broadcasted_iota(jnp.int32, (2 * lm, 2 * L), 1)
        same = (r < lm) == (c < L)
        rr = jnp.where(r < lm, r, r - lm)
        cc = jnp.where(c < L, c, c - L)
        ok = (rr < M) | (rr + 8 * nblk >= cc)
        ref[...] = jnp.where(same, jnp.where(ok, 0.0, -1e9), -jnp.inf).astype(F32)
    h_v[pl.ds(0, 8), :] = jnp.zeros((8, D), F32)
    h_v[pl.ds(S + 8, 8), :] = jnp.zeros((8, D), F32)
    s_v[...] = jnp.zeros((OB, D), F32)
    zero_v[...] = jnp.zeros((8, E), U32)

    def norm_chunk(c, z_ref, rb):
        deps = [None, None]
        for b in range(CH // rb):
            r0 = pl.multiple_of(c * CH + b * rb, rb)
            xn, mid = _ln(x_v[pl.ds(r0, rb), :].astype(F32), deps[b % 2])
            if b == 0:
                deps[1] = mid
            xn = xn.astype(BF16).astype(F32)
            xn_v[pl.ds(r0, rb), :] = xn
            z, deps[b % 2] = _ln(xn)
            z_ref[pl.ds(b * rb // 2, rb // 2), :] = pltpu.bitcast(z.astype(BF16), U32)

    def x_wait(c):
        rows = pl.ds(pl.multiple_of(c * CH, CH), CH)
        pltpu.make_async_copy(x_hbm.at[rows], x_v.at[rows], sem_x.at[c]).wait()

    def up1(c, z_ref):
        r0 = pl.multiple_of(c * CH, CH)
        h_v[pl.ds(r0 + 8, CH), :] = _gelu(jnp.dot(_w(z_ref[...]), _w(w1_v[...]), preferred_element_type=F32))

    def up1q(c, z_ref, q, nq):
        w = _w(w1_v[:, pl.ds(q * q4, nq * q4)])
        h_v[pl.ds(c * CH + 8, CH), pl.ds(q * q4, nq * q4)] = _gelu(
            jnp.dot(_w(z_ref[...]), w, preferred_element_type=F32))

    x_cp[0].wait()
    norm_chunk(0, za_v, CH)
    w1_cp[0].wait()
    up1q(0, za_v, 0, 1)
    x_cp[1].wait()
    norm_chunk(1, zb_v, CH)
    w1_cp[1].wait()
    up1q(1, zb_v, 0, 1)
    up1q(0, za_v, 1, 1)
    up1q(1, zb_v, 1, 1)
    w1_cp[2].wait()
    w1_cp[3].wait()
    x_cp[2].wait()
    up1q(0, za_v, 2, 2)
    up1q(1, zb_v, 2, 2)
    norm_chunk(2, za_v, 2 * RB)

    def stage1(i, carry):
        cn = jnp.minimum(2 * i + 2, nch - 1)
        x_wait(2 * i + 1)

        @pl.when(2 * i + 2 < nch)
        def _():
            x_wait(cn)

        up1(2 * i, za_v)
        norm_chunk(2 * i + 1, zb_v, RB)
        up1(2 * i + 1, zb_v)
        norm_chunk(cn, za_v, RB)
        return carry

    jax.lax.fori_loop(1, nch // 2, stage1, 0)
    qkv_start(20, 36)

    w2_cp.wait()

    def norm3(c, rb):
        dep = None
        for b in range(CH3 // rb):
            z, dep = _ln(x1_v[pl.ds(pl.multiple_of(c * CH3 + b * rb, rb), rb), :], dep)
            za_v[pl.ds(b * rb // 2, rb // 2), :] = pltpu.bitcast(z.astype(BF16), U32)

    x1_v[pl.ds(0, CH3), :] = jnp.zeros((CH3, D), F32)

    def stage2(c, carry):
        norm3(0, 16)
        r0 = pl.multiple_of(c * CH2, CH2)
        hb = h_v[pl.ds(r0, CH2 + 16), :]
        hs = jnp.concatenate([
            hb[7:7 + CH2, 0 * q4:1 * q4],
            hb[9:9 + CH2, 1 * q4:2 * q4],
            hb[6:6 + CH2, 2 * q4:3 * q4],
            hb[10:10 + CH2, 3 * q4:4 * q4]], axis=1).astype(BF16)
        x1_v[pl.ds(r0, CH2), :] = xn_v[pl.ds(r0, CH2), :] + jnp.dot(hs, _w(w2_v[...]), preferred_element_type=F32)
        return carry

    jax.lax.fori_loop(0, S // CH2, stage2, 0)
    qkv_start(36, 48)
    wo_cp.start()

    w3_cp.wait()
    w4_cp.wait()

    def stage3(c, carry):
        blk = wqkv_v.at[pl.ds(c * NCV, NCV)]
        pltpu.make_async_copy(blk, blk, sem_qkv.at[c]).wait()
        r0 = pl.multiple_of(c * CH3, CH3)
        z = _w(za_v[pl.ds(0, CH3 // 2), :])
        h3 = _gelu(jnp.dot(z, _w(w3_v[...]), preferred_element_type=F32)).astype(BF16)
        zero = zero_v[...]
        dep = zero
        for i in range(NCV):
            n = c * NCV + i
            for r in range(0, D // 2, 8):
                a = wqkv_v[n, 0, pl.ds(r, 8), :] | dep
                b = wqkv_v[n, 1, pl.ds(r, 8), :]
                lo = (a & jnp.uint32(0xFFFF)) | (b << 16)
                wqkv_v[n, 0, pl.ds(r, 8), :] = lo
                wqkv_v[n, 1, pl.ds(r, 8), :] = (a >> 16) | (b & jnp.uint32(0xFFFF0000))
                dep = lo & zero
        y = x1_v[pl.ds(r0, CH3), :] + jnp.dot(h3, _w(w4_v[...]), preferred_element_type=F32)
        h_v[pl.ds(r0, CH3), :] = _silu(y)
        norm3(jnp.minimum(c + 1, PRE // CH3 - 1), 16)
        return carry

    jax.lax.fori_loop(0, PRE // CH3, stage3, 0)
    wo_cp.wait()
    mem_cp.wait()
    mem_v[...] = mem0_v[...].astype(F32)

    def out_cp(j):
        return pltpu.make_async_copy(
            o_stage.at[j % 2], out_hbm.at[pl.ds(pl.multiple_of(j * OB, OB), OB)], sem_o.at[j % 2])

    def combine(j):
        t0 = pl.multiple_of(j * OB, OB)
        o_stage[j % 2] = (x_v[pl.ds(t0, OB), :].astype(F32)
                          + s_v[...] * h_v[pl.ds(t0, OB), :]).astype(BF16)

    def zero_of(x):
        return pltpu.bitcast(pltpu.bitcast(x[:8, :E], U32) & zero_v[...], F32)

    def anchor(s, vals):
        t = None
        for v in vals:
            w = pltpu.bitcast(v, U32)
            t = w if t is None else t | w
        zf = pltpu.bitcast(t & zero_v[...], F32)[:, :2 * L]
        return jnp.concatenate([s[:8] + zf, s[8:]], axis=0)

    def vpu_attn(slot, g, h, b, dep):
        row = jax.lax.broadcasted_iota(jnp.int32, (8, 1), 0)
        q = (kv_v[slot, g, h, pl.ds(M + 8 * b, 8), :] + dep) * (scale * LOG2E)
        nk = M + 8 * b + 8
        m = acc = l = None
        for k0 in range(0, nk, KC):
            ss = []
            for k in range(k0, k0 + KC):
                t = jnp.sum(q * kv_v[slot, g, 2 + h, pl.ds(k, 1), :], axis=-1, keepdims=True)
                if k > nk - 8:
                    t = jnp.where(row >= k - (nk - 8), t, -1e9 * LOG2E)
                ss.append(t)
            ms = ss
            while len(ms) > 1:
                ms = [jnp.maximum(ms[i], ms[i + 1]) for i in range(0, len(ms), 2)]
            if m is None:
                m = ms[0]
            else:
                mn = jnp.maximum(m, ms[0])
                a = jnp.exp2(m - mn)
                m, l, acc = mn, l * a, acc * a
            for i, t in enumerate(ss):
                e = jnp.exp2(t - m)
                t = e * kv_v[slot, g, 4 + h, pl.ds(k0 + i, 1), :]
                l = e if l is None else l + e
                acc = t if acc is None else acc + t
        return acc * _recip(l), zero_of(acc)

    def body(j, carry):
        @pl.when(j >= 3)
        def _():
            out_cp(jnp.maximum(j - 3, 0)).wait()

        combine(jnp.maximum(j - 1, 0))

        b0 = pl.multiple_of(PRE + j * BR, 16)
        x1 = x1_v[pl.ds(b0, BR), :]
        z = _ln(x1)[0].astype(BF16)
        h3 = []
        done = [0]

        def fill(spec):
            if spec is None:
                return None
            kind, n = spec
            if kind == "u":
                c0 = len(h3) * E
                t = jnp.dot(z, _w(w3_v[:, c0:c0 + n * E]), preferred_element_type=F32)
                u = _gelu(t).astype(BF16)
                h3.extend(u[:, i * E:(i + 1) * E] for i in range(n))
            else:
                c0, c1 = done[0] * E, (done[0] + n) * E
                done[0] += n
                t = jnp.dot(jnp.concatenate(h3, axis=1), _w(w4_v[:, c0:c1]), preferred_element_type=F32)
                h_v[pl.ds(b0, BR), c0:c1] = _silu(x1[:, c0:c1] + t)
            return t

        o = [[[[None] * 4 for _ in range(2)] for _ in range(G)] for _ in range(4)]
        chain = []

        def get(seg, g, h, blk):
            if o[seg][g][h][blk] is None:
                o[seg][g][h][blk], dep = vpu_attn(seg % 2, g, h, blk, chain.pop(0))
                chain.append(dep)
            return o[seg][g][h][blk]

        def segment(seg, mem, qkv_extra):
            first = seg % 2 == 0
            plan = PLAN[seg]
            t0 = pl.multiple_of(j * OB + (seg // 2) * PAIR, PAIR)
            rows = xn_v[pl.ds(t0, 40), :] if first else xn_v[pl.ds(t0 + 40, 24), :]
            lhs = jnp.concatenate([mem, rows], axis=0).astype(BF16)
            nblk = NV[seg % 2]
            nv, lm = M + 8 * nblk, L - 8 * nblk
            qkv_left, qkv, sc, o_mem = ([None] * G for _ in range(4))
            chain[:] = [jnp.zeros((8, E), F32)] * NCH

            def do_qkv(g):
                ys = [jnp.dot(lhs, _w(wqkv_v[(c // 2) * G + g, c % 2]), preferred_element_type=F32)
                      for c in range(6)]
                if first:
                    qkv_left[g] = [y[L:] for y in ys]
                    ys = [y[:L] for y in ys]
                else:
                    ys = [jnp.concatenate([y[:M], e, y[M:]], axis=0) for y, e in zip(ys, qkv_extra[g])]
                for i in range(6):
                    lo = M if i < 2 else 0
                    kv_v[seg % 2, g, i, pl.ds(lo, nv - lo), :] = ys[i][lo:nv]
                qm = jnp.concatenate([ys[0][:M], ys[0][nv:], ys[1][:M], ys[1][nv:]], axis=0).astype(BF16)
                qkv[g] = [qm] + [jnp.concatenate(ys[c:c + 2], axis=0).astype(BF16) for c in (2, 4)]

            def do_s(g):
                q, k, _ = qkv[g]
                s = jax.lax.dot_general(q, k, (((1,), (1,)), ((), ())), preferred_element_type=F32)
                fl = (filla_v if first else fillb_v)[...]
                s = jnp.where(fl == 0.0, s * scale, fl)
                lag = 4 if first else 8
                vals = []
                if g >= lag:
                    vals += [o_mem[g - lag][h] for h in range(2)]
                    vals += [o[seg][g - lag][h][b] for h in range(2) for b in range(nblk, 4)]
                if first and g >= 1:
                    vals += [get(seg, g - 1, h, b) for b in range(nblk) for h in range(2)]
                if vals:
                    s = anchor(s, vals)
                e = jnp.exp(s - jnp.max(s, axis=-1, keepdims=True))
                sc[g] = (e.astype(BF16), _recip(jnp.sum(e, axis=-1, keepdims=True)))

            def do_pv(g):
                e, rl = sc[g]
                t = jnp.dot(e, qkv[g][2], preferred_element_type=F32) * rl
                o_mem[g] = [t[h * lm:h * lm + M] for h in range(2)]
                for h in range(2):
                    for b in range(nblk, 4):
                        r = h * lm + M + 8 * (b - nblk)
                        o[seg][g][h][b] = t[r:r + 8]

            acc = [None]

            def part(i):
                t = fill(plan["tail"][i])
                if i == 0 and t is not None:
                    chain[:] = [zero_of(t)] * NCH
                g0, g1 = plan["cuts"][i:i + 2]
                if g0 < g1:
                    a = jnp.concatenate(
                        [jnp.concatenate([o_mem[g][h]] + [get(sg, g, h, b) for sg, b in plan["wo"]], axis=0)
                         for g in range(g0, g1) for h in range(2)], axis=1).astype(BF16)
                    t = jnp.dot(a, _w(wo_v[g0 * E:g1 * E, :]), preferred_element_type=F32)
                    acc[0] = t if acc[0] is None else t + acc[0]

            nb = 2 if first else 4
            for g in range(0, G, nb):
                for i in range(nb):
                    do_qkv(g + i)
                for f, i in ([(do_pv, g - nb - 1 + i) for i in range(nb)]
                             + [(do_s, g - 1 + i) for i in range(nb)]):
                    if i >= 0:
                        f(i)
            part(0)
            do_s(G - 1)
            for i in range(nb):
                do_pv(G - 1 - nb + i)
            part(1)
            do_pv(G - 1)
            part(2)
            part(3)
            for i, (sg, b) in enumerate(plan["wo"]):
                s_v[pl.ds(sg * SEG + 8 * b, 8), :] = acc[0][M + 8 * i:M + 8 * i + 8]
            fill(plan["end"])
            return acc[0][:M].astype(BF16).astype(F32), qkv_left

        mem = mem_v[...]
        left = None
        for seg in range(4):
            mem, left = segment(seg, mem, left)
        assert len(h3) == F // E and done[0] == D // E
        mem_v[...] = mem

        @pl.when(j >= 1)
        def _():
            out_cp(jnp.maximum(j - 1, 0)).start()

        return carry

    jax.lax.fori_loop(0, NJ, body, 0)
    out_cp(NJ - 3).wait()
    combine(NJ - 1)
    out_cp(NJ - 1).start()
    out_cp(NJ - 2).wait()
    out_cp(NJ - 1).wait()


@jax.jit
def pallas_recurrent_scan__memory_aug_recurrent_mem_tr__mixer_s_mlp__prompt_kernel(
    A_x: jax.Array,
    A_mem0: jax.Array,
    A_Wq: jax.Array,
    A_Wk: jax.Array,
    A_Wv: jax.Array,
    A_Wo: jax.Array,
    A_seg_len: jax.Array,
    B_x: jax.Array,
    B_w1: jax.Array,
    B_w2: jax.Array,
    B_w3: jax.Array,
    B_w4: jax.Array,
):
    del A_seg_len, B_x
    assert A_x.shape == (1, S, D) and A_mem0.shape == (1, M, D) and A_Wq.shape == (D, H, E)
    assert B_w3.shape == (D, F)
    any_spec = pl.BlockSpec(memory_space=pl.ANY)
    out = pl.pallas_call(
        _kernel,
        out_shape=jax.ShapeDtypeStruct((S, D), BF16),
        in_specs=[any_spec] * 10,
        out_specs=any_spec,
        scratch_shapes=[
            pltpu.VMEM((S, D), BF16),
            pltpu.VMEM((S, D), F32),
            pltpu.VMEM((S + 16, D), F32),
            pltpu.VMEM((S, D), F32),
            pltpu.VMEM((CH // 2, D), U32),
            pltpu.VMEM((CH // 2, D), U32),
            pltpu.VMEM((M, D), BF16),
            pltpu.VMEM((M, D), F32),
            pltpu.VMEM((OB, D), F32),
            pltpu.VMEM((2, OB, D), BF16),
            pltpu.VMEM((2 * (L - 8 * NV[0]), 2 * L), F32),
            pltpu.VMEM((2 * (L - 8 * NV[1]), 2 * L), F32),
            pltpu.VMEM((2, G, 6, M + 8 * max(NV), E), F32),
            pltpu.VMEM((8, E), U32),
            pltpu.VMEM((3 * G, 2, D // 2, E), U32),
            pltpu.VMEM((H * E // 2, D), U32),
            pltpu.VMEM((D // 2, D), U32),
            pltpu.VMEM((D // 2, D), U32),
            pltpu.VMEM((D // 2, F), U32),
            pltpu.VMEM((F // 2, D), U32),
            pltpu.SemaphoreType.DMA((S // CH,)),
            pltpu.SemaphoreType.DMA((9,)),
            pltpu.SemaphoreType.DMA((3 * G // NCV,)),
            pltpu.SemaphoreType.DMA((2,)),
        ],
        compiler_params=pltpu.CompilerParams(
            vmem_limit_bytes=110 * 1024 * 1024, disable_bounds_checks=True, disable_semaphore_checks=True),
    )(
        A_x.reshape(S, D),
        A_mem0.reshape(M, D),
        A_Wq.reshape(D // 2, 2, H, E),
        A_Wk.reshape(D // 2, 2, H, E),
        A_Wv.reshape(D // 2, 2, H, E),
        A_Wo.reshape(H * E, D),
        B_w1, B_w2, B_w3, B_w4,
    )
    return out.reshape(1, S, D)
```

```python
import jax
import jax.numpy as jnp
import jax.experimental.pallas as pl
import jax.experimental.pallas.tpu as pltpu

S, D, H, E, M, SEG, F = 2048, 1024, 32, 128, 8, 32, 3584
G = H // 2
L = M + SEG
PAIR = 2 * SEG
OB = 4 * SEG
NJ = S // OB
BR = 80
PRE = S - NJ * BR
CH = 256
CH2 = 512
CH3 = 128
NCV = 3 * G // (PRE // CH3)
NV = 2
NCH = 2
KC = 4
PLAN = (
    dict(wo=((0, 0), (0, 2), (0, 3)), cuts=(0, 0, 4, 13, 16), tail=(("u", 5), ("u", 3), None, None),
         end=("u", 4)),
    dict(wo=((0, 1), (1, 0), (1, 1), (1, 2), (1, 3)), cuts=(0, 5, 10, 15, 16), tail=(None,) * 4,
         end=("u", 4)),
    dict(wo=((2, 0), (2, 2), (2, 3)), cuts=(0, 0, 4, 13, 16), tail=(("u", 5), ("u", 3), None, None),
         end=("u", 4)),
    dict(wo=((2, 1), (3, 0), (3, 1), (3, 2), (3, 3)), cuts=(0, 5, 10, 15, 16), tail=(None,) * 4,
         end=("d", 8)),
)
EPS = 1e-5
LOG2E = 1.4426950408889634
F32 = jnp.float32
BF16 = jnp.bfloat16
U32 = jnp.uint32


def _ln(x, dep=None):
    m = jnp.sum(x, axis=-1, keepdims=True) * (1.0 / D)
    if dep is not None:
        m = m + dep
    xc = x - m
    v = jnp.sum(xc * xc, axis=-1, keepdims=True) * (1.0 / D)
    r = jax.lax.rsqrt(v + EPS)
    return xc * r, jnp.where(r < 0.0, 1.0, 0.0)


def _gelu(x):
    c1 = 0.7978845608028654
    c2 = c1 * 0.044715
    t = jnp.tanh(x * (c1 + c2 * (x * x)))
    hx = 0.5 * x
    return hx + hx * t


def _silu(x):
    hx = 0.5 * x
    return hx + hx * jnp.tanh(hx)


def _recip(l):
    r = pl.reciprocal(l, approx=True)
    return r * (2.0 - l * r)


def _w(packed):
    return pltpu.bitcast(packed, BF16)


def _kernel(x_hbm, mem_hbm, wq_hbm, wk_hbm, wv_hbm, wo_hbm, w1_hbm, w2_hbm, w3_hbm, w4_hbm,
            out_hbm,
            x_v, xn_v, h_v, x1_v, x1h_v, za_v, zb_v, zc_v, mem0_v, mem_v, s_v, o_stage, filla_v, fillb_v, kv_v, zero_v,
            wqkv_v, wo_v, w1_v, w2_v, w3_v, w4_v,
            sem_x, sem_w, sem_qkv, sem_o):
    scale = float(E) ** -0.5

    nch = S // CH
    q4 = D // 4
    x_cp = [pltpu.make_async_copy(x_hbm.at[pl.ds(c * CH, CH)], x_v.at[pl.ds(c * CH, CH)], sem_x.at[c])
            for c in range(nch)]
    w1_cp = [pltpu.make_async_copy(w1_hbm.bitcast(U32).at[:, pl.ds(q * q4, q4)],
                                   w1_v.at[:, pl.ds(q * q4, q4)], sem_w.at[q]) for q in range(4)]
    w2_cp = pltpu.make_async_copy(w2_hbm.bitcast(U32), w2_v, sem_w.at[4])
    w3_cp = pltpu.make_async_copy(w3_hbm.bitcast(U32), w3_v, sem_w.at[5])
    w4_cp = pltpu.make_async_copy(w4_hbm.bitcast(U32), w4_v, sem_w.at[6])
    wo_cp = pltpu.make_async_copy(wo_hbm.bitcast(U32), wo_v, sem_w.at[7])
    mem_cp = pltpu.make_async_copy(mem_hbm, mem0_v, sem_w.at[8])
    srcs = [w.bitcast(U32) for w in (wq_hbm, wk_hbm, wv_hbm)]

    def qkv_start(n0, n1):
        for n in range(n0, n1):
            for b in range(2):
                pltpu.make_async_copy(
                    srcs[n // G].at[:, b, n % G, :], wqkv_v.at[n, b], sem_qkv.at[n // NCV]).start()

    x_cp[0].start()
    w1_cp[0].start()
    x_cp[1].start()
    w1_cp[1].start()
    w1_cp[2].start()
    w1_cp[3].start()
    for c in range(2, nch):
        x_cp[c].start()
    w2_cp.start()
    mem_cp.start()
    w3_cp.start()
    w4_cp.start()
    qkv_start(0, 20)

    for ref, nblk in ((filla_v, NV), (fillb_v, 0)):
        lm = L - 8 * nblk
        r = jax.lax.broadcasted_iota(jnp.int32, (2 * lm, 2 * L), 0)
        c = jax.lax.broadcasted_iota(jnp.int32, (2 * lm, 2 * L), 1)
        same = (r < lm) == (c < L)
        rr = jnp.where(r < lm, r, r - lm)
        cc = jnp.where(c < L, c, c - L)
        ok = (rr < M) | (rr + 8 * nblk >= cc)
        ref[...] = jnp.where(same, jnp.where(ok, 0.0, -1e9), -jnp.inf).astype(F32)
    h_v[:, pl.ds(0, 8), :] = jnp.zeros((D // E, 8, E), F32)
    h_v[:, pl.ds(S + 8, 8), :] = jnp.zeros((D // E, 8, E), F32)

    def h_store(r0, c0, val):
        for i in range(val.shape[1] // E):
            h_v[c0 + i, pl.ds(r0, val.shape[0]), :] = val[:, i * E:(i + 1) * E]

    s_v[...] = jnp.zeros((OB, D), F32)
    zero_v[...] = jnp.zeros((8, E), U32)

    def norm_chunk(c, z_ref, paced):
        if not paced:
            xn = _ln(x_v[pl.ds(c * CH, CH), :].astype(F32))[0].astype(BF16).astype(F32)
            xn_v[pl.ds(c * CH, CH), :] = xn
            z_ref[...] = pltpu.bitcast(_ln(xn)[0].astype(BF16), U32)
            return
        deps = [None] * 4
        for t in range(CH // 16):
            r0 = pl.multiple_of(c * CH + t * 16, 16)
            xb = x_v[pl.ds(r0, 16), :].astype(F32)
            zs = []
            for b in (2 * t, 2 * t + 1):
                xn, mid = _ln(xb[(b % 2) * 8:(b % 2) * 8 + 8], deps[b % 4])
                deps[b + 1:] = [mid] * (3 - b) if b < 3 else deps[b + 1:]
                xn = xn.astype(BF16).astype(F32)
                xn_v[pl.ds(r0 + (b % 2) * 8, 8), :] = xn
                z, deps[b % 4] = _ln(xn)
                zs.append(z)
            z_ref[pl.ds(t * 8, 8), :] = pltpu.bitcast(jnp.concatenate(zs, axis=0).astype(BF16), U32)

    def x_wait(c):
        rows = pl.ds(pl.multiple_of(c * CH, CH), CH)
        pltpu.make_async_copy(x_hbm.at[rows], x_v.at[rows], sem_x.at[c]).wait()

    def up1(c, z_ref):
        r0 = pl.multiple_of(c * CH, CH)
        h_store(r0 + 8, 0, _gelu(jnp.dot(_w(z_ref[...]), _w(w1_v[...]), preferred_element_type=F32)))

    def up1q(c, z_ref, q, nq):
        w = _w(w1_v[:, pl.ds(q * q4, nq * q4)])
        h_store(c * CH + 8, 2 * q, _gelu(jnp.dot(_w(z_ref[...]), w, preferred_element_type=F32)))

    x_cp[0].wait()
    norm_chunk(0, zc_v, False)
    w1_cp[0].wait()
    up1q(0, zc_v, 0, 1)
    x_cp[1].wait()
    norm_chunk(1, zb_v, False)
    w1_cp[1].wait()
    up1q(1, zb_v, 0, 1)
    up1q(0, zc_v, 1, 1)
    up1q(1, zb_v, 1, 1)
    w1_cp[2].wait()
    w1_cp[3].wait()
    x_cp[2].wait()
    up1q(0, zc_v, 2, 2)
    up1q(1, zb_v, 2, 2)
    norm_chunk(2, za_v, True)

    def stage1(i, carry):
        cn = jnp.minimum(2 * i + 2, nch - 1)
        x_wait(2 * i + 1)

        @pl.when(2 * i + 2 < nch)
        def _():
            x_wait(cn)

        up1(2 * i, za_v)
        norm_chunk(2 * i + 1, zb_v, True)
        up1(2 * i + 1, zb_v)
        norm_chunk(cn, za_v, True)
        return carry

    jax.lax.fori_loop(1, nch // 2, stage1, 0)
    qkv_start(20, 36)

    w2_cp.wait()

    def norm3(src, r0, rb):
        dep = None
        for b in range(CH3 // rb):
            z, dep = _ln(src[pl.ds(pl.multiple_of(r0 + b * rb, rb), rb), :], dep)
            za_v[pl.ds(b * rb // 2, rb // 2), :] = pltpu.bitcast(z.astype(BF16), U32)

    x1h_v[...] = jnp.zeros((CH3, D), F32)

    def stage2(c, carry):
        norm3(x1h_v, 0, 16)
        r0 = pl.multiple_of(c * CH2, CH2)
        hs = jnp.concatenate([h_v[i, pl.ds(r0 + 8 + (-1, 1, -2, 2)[i // 2], CH2), :] for i in range(D // E)],
                             axis=1).astype(BF16)
        y = xn_v[pl.ds(r0, CH2), :] + jnp.dot(hs, _w(w2_v[...]), preferred_element_type=F32)
        x1_v[pl.ds(r0, CH2), :] = y
        x1h_v[...] = jnp.where(c == 0, y[:CH3], x1h_v[...])
        return carry

    jax.lax.fori_loop(0, S // CH2, stage2, 0)
    qkv_start(36, 48)
    wo_cp.start()

    w3_cp.wait()
    w4_cp.wait()

    def stage3(c, carry):
        blk = wqkv_v.at[pl.ds(c * NCV, NCV)]
        pltpu.make_async_copy(blk, blk, sem_qkv.at[c]).wait()
        r0 = pl.multiple_of(c * CH3, CH3)
        z = _w(za_v[pl.ds(0, CH3 // 2), :])
        h3 = _gelu(jnp.dot(z, _w(w3_v[...]), preferred_element_type=F32)).astype(BF16)
        zero = zero_v[...]
        dep = zero
        for i in range(NCV):
            n = c * NCV + i
            for r in range(0, D // 2, 8):
                a = wqkv_v[n, 0, pl.ds(r, 8), :] | dep
                b = wqkv_v[n, 1, pl.ds(r, 8), :]
                lo = (a & jnp.uint32(0xFFFF)) | (b << 16)
                wqkv_v[n, 0, pl.ds(r, 8), :] = lo
                wqkv_v[n, 1, pl.ds(r, 8), :] = (a >> 16) | (b & jnp.uint32(0xFFFF0000))
                dep = lo & zero
        y = x1_v[pl.ds(r0, CH3), :] + jnp.dot(h3, _w(w4_v[...]), preferred_element_type=F32)
        h_store(r0, 0, _silu(y))
        norm3(x1_v, jnp.minimum(c + 1, PRE // CH3 - 1) * CH3, 16)
        return carry

    jax.lax.fori_loop(0, PRE // CH3, stage3, 0)
    wo_cp.wait()
    mem_cp.wait()
    mem_v[...] = mem0_v[...].astype(F32)

    def out_cp(j):
        return pltpu.make_async_copy(
            o_stage.at[j % 2], out_hbm.at[pl.ds(pl.multiple_of(j * OB, OB), OB)], sem_o.at[j % 2])

    def combine(j):
        t0 = pl.multiple_of(j * OB, OB)
        o_stage[j % 2] = (x_v[pl.ds(t0, OB), :].astype(F32)
                          + s_v[...] * jnp.concatenate([h_v[i, pl.ds(t0, OB), :] for i in range(D // E)], axis=1)
                          ).astype(BF16)

    def zero_of(x):
        return pltpu.bitcast(pltpu.bitcast(x, U32) & zero_v[...], F32)

    def anchor(s, vals):
        t = None
        for v in vals:
            w = pltpu.bitcast(v, U32)
            t = w if t is None else t | w
        zf = pltpu.bitcast(t & zero_v[...], F32)[:, :2 * L]
        return jnp.concatenate([s[:8] + zf, s[8:]], axis=0)

    def vpu_attn(g, h, b, dep):
        row = jax.lax.broadcasted_iota(jnp.int32, (8, 1), 0)
        q = (kv_v[g, h, pl.ds(M + 8 * b, 8), :] + dep) * (scale * LOG2E)
        nk = M + 8 * b + 8
        m = acc = l = None
        for k0 in range(0, nk, KC):
            ss = []
            for k in range(k0, k0 + KC):
                t = jnp.sum(q * kv_v[g, 2 + h, pl.ds(k, 1), :], axis=-1, keepdims=True)
                if k > nk - 8:
                    t = jnp.where(row >= k - (nk - 8), t, -1e9 * LOG2E)
                ss.append(t)
            ms = ss
            while len(ms) > 1:
                ms = [jnp.maximum(ms[i], ms[i + 1]) for i in range(0, len(ms), 2)]
            if m is None:
                m = ms[0]
            else:
                mn = jnp.maximum(m, ms[0])
                a = jnp.exp2(m - mn)
                m, l, acc = mn, l * a, acc * a
            for i, t in enumerate(ss):
                e = jnp.exp2(t - m)
                t = e * kv_v[g, 4 + h, pl.ds(k0 + i, 1), :]
                l = e if l is None else l + e
                acc = t if acc is None else acc + t
        return acc * _recip(l), zero_of(acc)

    def body(j, carry):
        @pl.when(j >= 3)
        def _():
            out_cp(jnp.maximum(j - 3, 0)).wait()

        combine(jnp.maximum(j - 1, 0))

        b0 = pl.multiple_of(PRE + j * BR, 16)
        x1 = x1_v[pl.ds(b0, BR), :]
        z = _ln(x1)[0].astype(BF16)
        h3 = []
        done = [0]

        def fill(spec):
            if spec is None:
                return
            kind, n = spec
            if kind == "u":
                c0 = len(h3) * E
                t = jnp.dot(z, _w(w3_v[:, c0:c0 + n * E]), preferred_element_type=F32)
                u = _gelu(t).astype(BF16)
                h3.extend(u[:, i * E:(i + 1) * E] for i in range(n))
            else:
                c0, c1 = done[0] * E, (done[0] + n) * E
                done[0] += n
                t = jnp.dot(jnp.concatenate(h3, axis=1), _w(w4_v[:, c0:c1]), preferred_element_type=F32)
                h_store(b0, c0 // E, _silu(x1[:, c0:c1] + t))

        o = [[[[None] * 4 for _ in range(2)] for _ in range(G)] for _ in range(4)]
        chain = []

        def get(seg, g, h, blk):
            if o[seg][g][h][blk] is None:
                o[seg][g][h][blk], dep = vpu_attn(g, h, blk, chain.pop(0))
                chain.append(dep)
            return o[seg][g][h][blk]

        def segment(seg, mem, qkv_extra):
            first = seg % 2 == 0
            plan = PLAN[seg]
            t0 = pl.multiple_of(j * OB + (seg // 2) * PAIR, PAIR)
            rows = xn_v[pl.ds(t0, 40), :] if first else xn_v[pl.ds(t0 + 40, 24), :]
            lhs = jnp.concatenate([mem, rows], axis=0).astype(BF16)
            nblk = NV if first else 0
            nv, lm = M + 8 * nblk, L - 8 * nblk
            qkv_left, qkv, sc, o_mem = ([None] * G for _ in range(4))
            chain[:] = [jnp.zeros((8, E), F32)] * NCH

            def do_qkv(g):
                ys = [jnp.dot(lhs, _w(wqkv_v[(c // 2) * G + g, c % 2]), preferred_element_type=F32)
                      for c in range(6)]
                if first:
                    qkv_left[g] = [y[L:] for y in ys]
                    ys = [y[:L] for y in ys]
                else:
                    ys = [jnp.concatenate([y[:M], e, y[M:]], axis=0) for y, e in zip(ys, qkv_extra[g])]
                for i in range(6 if nblk else 0):
                    lo = M if i < 2 else 0
                    kv_v[g, i, pl.ds(lo, nv - lo), :] = ys[i][lo:nv]
                qm = jnp.concatenate([ys[0][:M], ys[0][nv:], ys[1][:M], ys[1][nv:]], axis=0).astype(BF16)
                qkv[g] = [qm] + [jnp.concatenate(ys[c:c + 2], axis=0).astype(BF16) for c in (2, 4)]

            def do_s(g):
                q, k, _ = qkv[g]
                s = jax.lax.dot_general(q, k, (((1,), (1,)), ((), ())), preferred_element_type=F32)
                fl = (filla_v if first else fillb_v)[...]
                s = jnp.where(fl == 0.0, s * scale, fl)
                lag = 4 if first else 8
                vals = []
                if g >= lag:
                    vals += [o_mem[g - lag][h] for h in range(2)]
                    vals += [o[seg][g - lag][h][b] for h in range(2) for b in range(nblk, 4)]
                if first and g >= 1:
                    vals += [get(seg, g - 1, h, b) for b in range(nblk) for h in range(2)]
                if vals:
                    s = anchor(s, vals)
                e = jnp.exp(s - jnp.max(s, axis=-1, keepdims=True))
                sc[g] = (e.astype(BF16), _recip(jnp.sum(e, axis=-1, keepdims=True)))

            def do_pv(g):
                e, rl = sc[g]
                t = jnp.dot(e, qkv[g][2], preferred_element_type=F32) * rl
                o_mem[g] = [t[h * lm:h * lm + M] for h in range(2)]
                for h in range(2):
                    for b in range(nblk, 4):
                        r = h * lm + M + 8 * (b - nblk)
                        o[seg][g][h][b] = t[r:r + 8]

            acc = [None]

            def part(i):
                fill(plan["tail"][i])
                g0, g1 = plan["cuts"][i:i + 2]
                if g0 < g1:
                    a = jnp.concatenate(
                        [jnp.concatenate([o_mem[g][h]] + [get(sg, g, h, b) for sg, b in plan["wo"]], axis=0)
                         for g in range(g0, g1) for h in range(2)], axis=1).astype(BF16)
                    t = jnp.dot(a, _w(wo_v[g0 * E:g1 * E, :]), preferred_element_type=F32)
                    acc[0] = t if acc[0] is None else t + acc[0]

            nb = 2 if first else 4
            for g in range(0, G, nb):
                for i in range(nb):
                    do_qkv(g + i)
                for f, i in ([(do_pv, g - nb - 1 + i) for i in range(nb)]
                             + [(do_s, g - 1 + i) for i in range(nb)]):
                    if i >= 0:
                        f(i)
            part(0)
            do_s(G - 1)
            for i in range(nb):
                do_pv(G - 1 - nb + i)
            part(1)
            do_pv(G - 1)
            part(2)
            part(3)
            for i, (sg, b) in enumerate(plan["wo"]):
                s_v[pl.ds(sg * SEG + 8 * b, 8), :] = acc[0][M + 8 * i:M + 8 * i + 8]
            fill(plan["end"])
            return acc[0][:M].astype(BF16).astype(F32), qkv_left

        mem = mem_v[...]
        left = None
        for seg in range(4):
            mem, left = segment(seg, mem, left)
        assert len(h3) == F // E and done[0] == D // E
        mem_v[...] = mem

        @pl.when(j >= 1)
        def _():
            out_cp(jnp.maximum(j - 1, 0)).start()

        return carry

    jax.lax.fori_loop(0, NJ, body, 0)
    out_cp(NJ - 3).wait()
    combine(NJ - 1)
    out_cp(NJ - 1).start()
    out_cp(NJ - 2).wait()
    out_cp(NJ - 1).wait()


@jax.jit
def pallas_recurrent_scan__memory_aug_recurrent_mem_tr__mixer_s_mlp__prompt_kernel(
    A_x: jax.Array,
    A_mem0: jax.Array,
    A_Wq: jax.Array,
    A_Wk: jax.Array,
    A_Wv: jax.Array,
    A_Wo: jax.Array,
    A_seg_len: jax.Array,
    B_x: jax.Array,
    B_w1: jax.Array,
    B_w2: jax.Array,
    B_w3: jax.Array,
    B_w4: jax.Array,
):
    del A_seg_len, B_x
    assert A_x.shape == (1, S, D) and A_mem0.shape == (1, M, D) and A_Wq.shape == (D, H, E)
    assert B_w3.shape == (D, F)
    any_spec = pl.BlockSpec(memory_space=pl.ANY)
    out = pl.pallas_call(
        _kernel,
        out_shape=jax.ShapeDtypeStruct((S, D), BF16),
        in_specs=[any_spec] * 10,
        out_specs=any_spec,
        scratch_shapes=[
            pltpu.VMEM((S, D), BF16),
            pltpu.VMEM((S, D), F32),
            pltpu.VMEM((D // E, S + 16, E), F32),
            pltpu.VMEM((S, D), F32),
            pltpu.VMEM((CH3, D), F32),
            pltpu.VMEM((CH // 2, D), U32),
            pltpu.VMEM((CH // 2, D), U32),
            pltpu.VMEM((CH // 2, D), U32),
            pltpu.VMEM((M, D), BF16),
            pltpu.VMEM((M, D), F32),
            pltpu.VMEM((OB, D), F32),
            pltpu.VMEM((2, OB, D), BF16),
            pltpu.VMEM((2 * (L - 8 * NV), 2 * L), F32),
            pltpu.VMEM((2 * L, 2 * L), F32),
            pltpu.VMEM((G, 6, M + 8 * NV, E), F32),
            pltpu.VMEM((8, E), U32),
            pltpu.VMEM((3 * G, 2, D // 2, E), U32),
            pltpu.VMEM((H * E // 2, D), U32),
            pltpu.VMEM((D // 2, D), U32),
            pltpu.VMEM((D // 2, D), U32),
            pltpu.VMEM((D // 2, F), U32),
            pltpu.VMEM((F // 2, D), U32),
            pltpu.SemaphoreType.DMA((S // CH,)),
            pltpu.SemaphoreType.DMA((9,)),
            pltpu.SemaphoreType.DMA((3 * G // NCV,)),
            pltpu.SemaphoreType.DMA((2,)),
        ],
        compiler_params=pltpu.CompilerParams(
            vmem_limit_bytes=110 * 1024 * 1024, disable_bounds_checks=True, disable_semaphore_checks=True),
    )(
        A_x.reshape(S, D),
        A_mem0.reshape(M, D),
        A_Wq.reshape(D // 2, 2, H, E),
        A_Wk.reshape(D // 2, 2, H, E),
        A_Wv.reshape(D // 2, 2, H, E),
        A_Wo.reshape(H * E, D),
        B_w1, B_w2, B_w3, B_w4,
    )
    return out.reshape(1, S, D)
```

```python
import jax
import jax.numpy as jnp
import jax.experimental.pallas as pl
import jax.experimental.pallas.tpu as pltpu

S, D, H, E, M, SEG, F = 2048, 1024, 32, 128, 8, 32, 3584
G = H // 2
L = M + SEG
PAIR = 2 * SEG
OB = 4 * SEG
NJ = S // OB
BR = 80
PRE = S - NJ * BR
CH = 256
CH2 = 512
CH3 = 128
NCV = 3 * G // (PRE // CH3)
NV = 2
NCH = 2
KC = 4
PLAN = (
    dict(wo=((0, 0), (0, 2), (0, 3)), cuts=(0, 0, 3, 13, 16), tail=(("u", 5), ("u", 4), None, None),
         end=("u", 3)),
    dict(wo=((0, 1), (1, 0), (1, 1), (1, 2), (1, 3)), cuts=(0, 5, 10, 15, 16), tail=(None,) * 4,
         end=("u", 4)),
    dict(wo=((2, 0), (2, 2), (2, 3)), cuts=(0, 0, 3, 13, 16), tail=(("u", 5), ("u", 4), None, None),
         end=("u", 3)),
    dict(wo=((2, 1), (3, 0), (3, 1), (3, 2), (3, 3)), cuts=(0, 5, 10, 15, 16), tail=(None,) * 4,
         end=("d", 8)),
)
EPS = 1e-5
LOG2E = 1.4426950408889634
F32 = jnp.float32
BF16 = jnp.bfloat16
U32 = jnp.uint32


def _ln(x, dep=None):
    m = jnp.sum(x, axis=-1, keepdims=True) * (1.0 / D)
    if dep is not None:
        m = m + dep
    xc = x - m
    v = jnp.sum(xc * xc, axis=-1, keepdims=True) * (1.0 / D)
    r = jax.lax.rsqrt(v + EPS)
    return xc * r, jnp.where(r < 0.0, 1.0, 0.0)


def _gelu(x):
    c1 = 0.7978845608028654
    c2 = c1 * 0.044715
    t = jnp.tanh(x * (c1 + c2 * (x * x)))
    hx = 0.5 * x
    return hx + hx * t


def _silu(x):
    hx = 0.5 * x
    return hx + hx * jnp.tanh(hx)


def _recip(l):
    r = pl.reciprocal(l, approx=True)
    return r * (2.0 - l * r)


def _w(packed):
    return pltpu.bitcast(packed, BF16)


def _kernel(x_hbm, mem_hbm, wq_hbm, wk_hbm, wv_hbm, wo_hbm, w1_hbm, w2_hbm, w3_hbm, w4_hbm,
            out_hbm,
            x_v, xn_v, h_v, x1_v, x1h_v, za_v, zb_v, zc_v, mem0_v, mem_v, s_v, o_stage, filla_v, fillb_v, kv_v, zero_v,
            wqkv_v, wo_v, w1_v, w2_v, w3_v, w4_v,
            sem_x, sem_w, sem_qkv, sem_o):
    scale = float(E) ** -0.5

    nch = S // CH
    q4 = D // 4
    x_cp = [pltpu.make_async_copy(x_hbm.at[pl.ds(c * CH, CH)], x_v.at[pl.ds(c * CH, CH)], sem_x.at[c])
            for c in range(nch)]
    w1_cp = [pltpu.make_async_copy(w1_hbm.bitcast(U32).at[:, pl.ds(q * q4, q4)],
                                   w1_v.at[:, pl.ds(q * q4, q4)], sem_w.at[q]) for q in range(4)]
    w2_cp = pltpu.make_async_copy(w2_hbm.bitcast(U32), w2_v, sem_w.at[4])
    w3_cp = pltpu.make_async_copy(w3_hbm.bitcast(U32), w3_v, sem_w.at[5])
    w4_cp = pltpu.make_async_copy(w4_hbm.bitcast(U32), w4_v, sem_w.at[6])
    wo_cp = pltpu.make_async_copy(wo_hbm.bitcast(U32), wo_v, sem_w.at[7])
    mem_cp = pltpu.make_async_copy(mem_hbm, mem0_v, sem_w.at[8])
    srcs = [w.bitcast(U32) for w in (wq_hbm, wk_hbm, wv_hbm)]

    def qkv_start(n0, n1):
        for n in range(n0, n1):
            for b in range(2):
                pltpu.make_async_copy(
                    srcs[n // G].at[:, b, n % G, :], wqkv_v.at[n, b], sem_qkv.at[n // NCV]).start()

    x_cp[0].start()
    w1_cp[0].start()
    x_cp[1].start()
    w1_cp[1].start()
    w1_cp[2].start()
    w1_cp[3].start()
    for c in range(2, nch):
        x_cp[c].start()
    w2_cp.start()
    mem_cp.start()
    w3_cp.start()
    w4_cp.start()
    qkv_start(0, 20)

    for ref, nblk in ((filla_v, NV), (fillb_v, 0)):
        lm = L - 8 * nblk
        r = jax.lax.broadcasted_iota(jnp.int32, (2 * lm, 2 * L), 0)
        c = jax.lax.broadcasted_iota(jnp.int32, (2 * lm, 2 * L), 1)
        same = (r < lm) == (c < L)
        rr = jnp.where(r < lm, r, r - lm)
        cc = jnp.where(c < L, c, c - L)
        ok = (rr < M) | (rr + 8 * nblk >= cc)
        ref[...] = jnp.where(same, jnp.where(ok, 0.0, -1e9), -jnp.inf).astype(F32)
    h_v[:, pl.ds(0, 8), :] = jnp.zeros((D // E, 8, E), F32)
    h_v[:, pl.ds(S + 8, 8), :] = jnp.zeros((D // E, 8, E), F32)

    def h_store(r0, c0, val):
        for i in range(val.shape[1] // E):
            h_v[c0 + i, pl.ds(r0, val.shape[0]), :] = val[:, i * E:(i + 1) * E]

    s_v[...] = jnp.zeros((OB, D), F32)
    zero_v[...] = jnp.zeros((8, E), U32)

    def norm_chunk(c, z_ref, paced):
        if not paced:
            xn = _ln(x_v[pl.ds(c * CH, CH), :].astype(F32))[0].astype(BF16).astype(F32)
            xn_v[pl.ds(c * CH, CH), :] = xn
            z_ref[...] = pltpu.bitcast(_ln(xn)[0].astype(BF16), U32)
            return
        deps = [None] * 4
        for t in range(CH // 16):
            r0 = pl.multiple_of(c * CH + t * 16, 16)
            xb = x_v[pl.ds(r0, 16), :].astype(F32)
            zs = []
            for b in (2 * t, 2 * t + 1):
                xn, mid = _ln(xb[(b % 2) * 8:(b % 2) * 8 + 8], deps[b % 4])
                deps[b + 1:] = [mid] * (3 - b) if b < 3 else deps[b + 1:]
                xn = xn.astype(BF16).astype(F32)
                xn_v[pl.ds(r0 + (b % 2) * 8, 8), :] = xn
                z, deps[b % 4] = _ln(xn)
                zs.append(z)
            z_ref[pl.ds(t * 8, 8), :] = pltpu.bitcast(jnp.concatenate(zs, axis=0).astype(BF16), U32)

    def x_wait(c):
        rows = pl.ds(pl.multiple_of(c * CH, CH), CH)
        pltpu.make_async_copy(x_hbm.at[rows], x_v.at[rows], sem_x.at[c]).wait()

    def up1(c, z_ref):
        r0 = pl.multiple_of(c * CH, CH)
        h_store(r0 + 8, 0, _gelu(jnp.dot(_w(z_ref[...]), _w(w1_v[...]), preferred_element_type=F32)))

    def up1q(c, z_ref, q, nq):
        w = _w(w1_v[:, pl.ds(q * q4, nq * q4)])
        h_store(c * CH + 8, 2 * q, _gelu(jnp.dot(_w(z_ref[...]), w, preferred_element_type=F32)))

    x_cp[0].wait()
    norm_chunk(0, zc_v, False)
    w1_cp[0].wait()
    up1q(0, zc_v, 0, 1)
    x_cp[1].wait()
    norm_chunk(1, zb_v, False)
    w1_cp[1].wait()
    up1q(1, zb_v, 0, 1)
    up1q(0, zc_v, 1, 1)
    up1q(1, zb_v, 1, 1)
    w1_cp[2].wait()
    w1_cp[3].wait()
    x_cp[2].wait()
    up1q(0, zc_v, 2, 2)
    up1q(1, zb_v, 2, 2)
    norm_chunk(2, za_v, True)

    def stage1(i, carry):
        cn = jnp.minimum(2 * i + 2, nch - 1)
        x_wait(2 * i + 1)

        @pl.when(2 * i + 2 < nch)
        def _():
            x_wait(cn)

        up1(2 * i, za_v)
        norm_chunk(2 * i + 1, zb_v, True)
        up1(2 * i + 1, zb_v)
        norm_chunk(cn, za_v, True)
        return carry

    jax.lax.fori_loop(1, nch // 2, stage1, 0)
    qkv_start(20, 36)

    w2_cp.wait()

    def norm3(src, r0, rb):
        dep = None
        for b in range(CH3 // rb):
            z, dep = _ln(src[pl.ds(pl.multiple_of(r0 + b * rb, rb), rb), :], dep)
            za_v[pl.ds(b * rb // 2, rb // 2), :] = pltpu.bitcast(z.astype(BF16), U32)

    x1h_v[...] = jnp.zeros((CH3, D), F32)

    def stage2(c, carry):
        norm3(x1h_v, 0, 16)
        r0 = pl.multiple_of(c * CH2, CH2)
        hs = jnp.concatenate([h_v[i, pl.ds(r0 + 8 + (-1, 1, -2, 2)[i // 2], CH2), :] for i in range(D // E)],
                             axis=1).astype(BF16)
        y = xn_v[pl.ds(r0, CH2), :] + jnp.dot(hs, _w(w2_v[...]), preferred_element_type=F32)
        x1_v[pl.ds(r0, CH2), :] = y
        x1h_v[...] = jnp.where(c == 0, y[:CH3], x1h_v[...])
        return carry

    jax.lax.fori_loop(0, S // CH2, stage2, 0)
    qkv_start(36, 48)
    wo_cp.start()

    w3_cp.wait()
    w4_cp.wait()

    def stage3(c, carry):
        blk = wqkv_v.at[pl.ds(c * NCV, NCV)]
        pltpu.make_async_copy(blk, blk, sem_qkv.at[c]).wait()
        r0 = pl.multiple_of(c * CH3, CH3)
        z = _w(za_v[pl.ds(0, CH3 // 2), :])
        h3 = _gelu(jnp.dot(z, _w(w3_v[...]), preferred_element_type=F32)).astype(BF16)
        zero = zero_v[...]
        dep = zero
        for i in range(NCV):
            n = c * NCV + i
            for r in range(0, D // 2, 8):
                a = wqkv_v[n, 0, pl.ds(r, 8), :] | dep
                b = wqkv_v[n, 1, pl.ds(r, 8), :]
                lo = (a & jnp.uint32(0xFFFF)) | (b << 16)
                wqkv_v[n, 0, pl.ds(r, 8), :] = lo
                wqkv_v[n, 1, pl.ds(r, 8), :] = (a >> 16) | (b & jnp.uint32(0xFFFF0000))
                dep = (((lo & zero) | zero) & zero | zero) & zero
        y = x1_v[pl.ds(r0, CH3), :] + jnp.dot(h3, _w(w4_v[...]), preferred_element_type=F32)
        h_store(r0, 0, _silu(y))
        norm3(x1_v, jnp.minimum(c + 1, PRE // CH3 - 1) * CH3, 16)
        return carry

    jax.lax.fori_loop(0, PRE // CH3, stage3, 0)
    wo_cp.wait()
    mem_cp.wait()
    mem_v[...] = mem0_v[...].astype(F32)

    def out_cp(j):
        return pltpu.make_async_copy(
            o_stage.at[j % 2], out_hbm.at[pl.ds(pl.multiple_of(j * OB, OB), OB)], sem_o.at[j % 2])

    def combine(j):
        t0 = pl.multiple_of(j * OB, OB)
        o_stage[j % 2] = (x_v[pl.ds(t0, OB), :].astype(F32)
                          + s_v[...] * jnp.concatenate([h_v[i, pl.ds(t0, OB), :] for i in range(D // E)], axis=1)
                          ).astype(BF16)

    def zero_of(x):
        return pltpu.bitcast(pltpu.bitcast(x, U32) & zero_v[...], F32)

    def anchor(s, vals):
        t = None
        for v in vals:
            w = pltpu.bitcast(v, U32)
            t = w if t is None else t | w
        zf = pltpu.bitcast(t & zero_v[...], F32)[:, :2 * L]
        return jnp.concatenate([s[:8] + zf, s[8:]], axis=0)

    def vpu_attn(g, h, b, dep):
        row = jax.lax.broadcasted_iota(jnp.int32, (8, 1), 0)
        q = (kv_v[g, h, pl.ds(M + 8 * b, 8), :] + dep) * (scale * LOG2E)
        nk = M + 8 * b + 8
        m = acc = l = None
        for k0 in range(0, nk, KC):
            ss = []
            for k in range(k0, k0 + KC):
                t = jnp.sum(q * kv_v[g, 2 + h, pl.ds(k, 1), :], axis=-1, keepdims=True)
                if k > nk - 8:
                    t = jnp.where(row >= k - (nk - 8), t, -1e9 * LOG2E)
                ss.append(t)
            ms = ss
            while len(ms) > 1:
                ms = [jnp.maximum(ms[i], ms[i + 1]) for i in range(0, len(ms), 2)]
            if m is None:
                m = ms[0]
            else:
                mn = jnp.maximum(m, ms[0])
                a = jnp.exp2(m - mn)
                m, l, acc = mn, l * a, acc * a
            for i, t in enumerate(ss):
                e = jnp.exp2(t - m)
                t = e * kv_v[g, 4 + h, pl.ds(k0 + i, 1), :]
                l = e if l is None else l + e
                acc = t if acc is None else acc + t
        return acc * _recip(l), zero_of(acc)

    def body(j, carry):
        @pl.when(j >= 3)
        def _():
            out_cp(jnp.maximum(j - 3, 0)).wait()

        combine(jnp.maximum(j - 1, 0))

        b0 = pl.multiple_of(PRE + j * BR, 16)
        x1 = x1_v[pl.ds(b0, BR), :]
        z = _ln(x1)[0].astype(BF16)
        h3 = []
        done = [0]

        def fill(spec):
            if spec is None:
                return
            kind, n = spec
            if kind == "u":
                c0 = len(h3) * E
                t = jnp.dot(z, _w(w3_v[:, c0:c0 + n * E]), preferred_element_type=F32)
                u = _gelu(t).astype(BF16)
                h3.extend(u[:, i * E:(i + 1) * E] for i in range(n))
            else:
                c0, c1 = done[0] * E, (done[0] + n) * E
                done[0] += n
                t = jnp.dot(jnp.concatenate(h3, axis=1), _w(w4_v[:, c0:c1]), preferred_element_type=F32)
                h_store(b0, c0 // E, _silu(x1[:, c0:c1] + t))

        o = [[[[None] * 4 for _ in range(2)] for _ in range(G)] for _ in range(4)]
        chain = []

        def get(seg, g, h, blk):
            if o[seg][g][h][blk] is None:
                o[seg][g][h][blk], dep = vpu_attn(g, h, blk, chain.pop(0))
                chain.append(dep)
            return o[seg][g][h][blk]

        def segment(seg, mem, qkv_extra):
            first = seg % 2 == 0
            plan = PLAN[seg]
            t0 = pl.multiple_of(j * OB + (seg // 2) * PAIR, PAIR)
            rows = xn_v[pl.ds(t0, 40), :] if first else xn_v[pl.ds(t0 + 40, 24), :]
            lhs = jnp.concatenate([mem, rows], axis=0).astype(BF16)
            nblk = NV if first else 0
            nv, lm = M + 8 * nblk, L - 8 * nblk
            qkv_left, qkv, sc, o_mem = ([None] * G for _ in range(4))
            chain[:] = [jnp.zeros((8, E), F32)] * NCH

            prev = [None]

            def do_qkv(g):
                ys = [jnp.dot(lhs, _w(wqkv_v[(c // 2) * G + g, c % 2]), preferred_element_type=F32)
                      for c in range(6)]
                if first:
                    qkv_left[g] = [y[L:] for y in ys]
                    ys = [y[:L] for y in ys]
                else:
                    ys = [jnp.concatenate([y[:M], e, y[M:]], axis=0) for y, e in zip(ys, qkv_extra[g])]
                for i in range(6 if nblk else 0):
                    lo = M if i < 2 else 0
                    kv_v[g, i, pl.ds(lo, nv - lo), :] = ys[i][lo:nv]
                qm = jnp.concatenate([ys[0][:M], ys[0][nv:], ys[1][:M], ys[1][nv:]], axis=0).astype(BF16)
                qkv[g] = [qm] + [jnp.concatenate(ys[c:c + 2], axis=0).astype(BF16) for c in (2, 4)]

            def do_s(g):
                q, k, _ = qkv[g]
                s = jax.lax.dot_general(q, k, (((1,), (1,)), ((), ())), preferred_element_type=F32)
                fl = (filla_v if first else fillb_v)[...]
                s = jnp.where(fl == 0.0, s * scale, fl)
                lag = 4 if first else 8
                vals = []
                if g >= lag:
                    vals += [o_mem[g - lag][h] for h in range(2)]
                    vals += [o[seg][g - lag][h][b] for h in range(2) for b in range(nblk, 4)]
                if first and g >= 1:
                    vals += [get(seg, g - 1, h, b) for b in range(nblk) for h in range(2)]
                if vals:
                    s = anchor(s, vals)
                mx = jnp.max(s if prev[0] is None else s + prev[0], axis=-1, keepdims=True)
                e = jnp.exp(s - mx)
                l = jnp.sum(e, axis=-1, keepdims=True)
                prev[0] = None if first or g % 4 == 2 else jnp.where(l > jnp.inf, 1.0, 0.0)
                sc[g] = (e.astype(BF16), _recip(l))

            def do_pv(g):
                e, rl = sc[g]
                t = jnp.dot(e, qkv[g][2], preferred_element_type=F32) * rl
                o_mem[g] = [t[h * lm:h * lm + M] for h in range(2)]
                for h in range(2):
                    for b in range(nblk, 4):
                        r = h * lm + M + 8 * (b - nblk)
                        o[seg][g][h][b] = t[r:r + 8]

            acc = [None]

            def part(i):
                fill(plan["tail"][i])
                g0, g1 = plan["cuts"][i:i + 2]
                if g0 < g1:
                    a = jnp.concatenate(
                        [jnp.concatenate([o_mem[g][h]] + [get(sg, g, h, b) for sg, b in plan["wo"]], axis=0)
                         for g in range(g0, g1) for h in range(2)], axis=1).astype(BF16)
                    t = jnp.dot(a, _w(wo_v[g0 * E:g1 * E, :]), preferred_element_type=F32)
                    acc[0] = t if acc[0] is None else t + acc[0]

            nb = 2 if first else 4
            for g in range(0, G, nb):
                for i in range(nb):
                    do_qkv(g + i)
                for f, i in ([(do_pv, g - nb - 1 + i) for i in range(nb)]
                             + [(do_s, g - 1 + i) for i in range(nb)]):
                    if i >= 0:
                        f(i)
            part(0)
            do_s(G - 1)
            for i in range(nb):
                do_pv(G - 1 - nb + i)
            part(1)
            do_pv(G - 1)
            part(2)
            part(3)
            for i, (sg, b) in enumerate(plan["wo"]):
                s_v[pl.ds(sg * SEG + 8 * b, 8), :] = acc[0][M + 8 * i:M + 8 * i + 8]
            fill(plan["end"])
            return acc[0][:M].astype(BF16).astype(F32), qkv_left

        mem = mem_v[...]
        left = None
        for seg in range(4):
            mem, left = segment(seg, mem, left)
        assert len(h3) == F // E and done[0] == D // E
        mem_v[...] = mem

        @pl.when(j >= 1)
        def _():
            out_cp(jnp.maximum(j - 1, 0)).start()

        return carry

    jax.lax.fori_loop(0, NJ, body, 0)
    out_cp(NJ - 3).wait()
    combine(NJ - 1)
    out_cp(NJ - 1).start()
    out_cp(NJ - 2).wait()
    out_cp(NJ - 1).wait()


@jax.jit
def pallas_recurrent_scan__memory_aug_recurrent_mem_tr__mixer_s_mlp__prompt_kernel(
    A_x: jax.Array,
    A_mem0: jax.Array,
    A_Wq: jax.Array,
    A_Wk: jax.Array,
    A_Wv: jax.Array,
    A_Wo: jax.Array,
    A_seg_len: jax.Array,
    B_x: jax.Array,
    B_w1: jax.Array,
    B_w2: jax.Array,
    B_w3: jax.Array,
    B_w4: jax.Array,
):
    del A_seg_len, B_x
    assert A_x.shape == (1, S, D) and A_mem0.shape == (1, M, D) and A_Wq.shape == (D, H, E)
    assert B_w3.shape == (D, F)
    any_spec = pl.BlockSpec(memory_space=pl.ANY)
    out = pl.pallas_call(
        _kernel,
        out_shape=jax.ShapeDtypeStruct((S, D), BF16),
        in_specs=[any_spec] * 10,
        out_specs=any_spec,
        scratch_shapes=[
            pltpu.VMEM((S, D), BF16),
            pltpu.VMEM((S, D), F32),
            pltpu.VMEM((D // E, S + 16, E), F32),
            pltpu.VMEM((S, D), F32),
            pltpu.VMEM((CH3, D), F32),
            pltpu.VMEM((CH // 2, D), U32),
            pltpu.VMEM((CH // 2, D), U32),
            pltpu.VMEM((CH // 2, D), U32),
            pltpu.VMEM((M, D), BF16),
            pltpu.VMEM((M, D), F32),
            pltpu.VMEM((OB, D), F32),
            pltpu.VMEM((2, OB, D), BF16),
            pltpu.VMEM((2 * (L - 8 * NV), 2 * L), F32),
            pltpu.VMEM((2 * L, 2 * L), F32),
            pltpu.VMEM((G, 6, M + 8 * NV, E), F32),
            pltpu.VMEM((8, E), U32),
            pltpu.VMEM((3 * G, 2, D // 2, E), U32),
            pltpu.VMEM((H * E // 2, D), U32),
            pltpu.VMEM((D // 2, D), U32),
            pltpu.VMEM((D // 2, D), U32),
            pltpu.VMEM((D // 2, F), U32),
            pltpu.VMEM((F // 2, D), U32),
            pltpu.SemaphoreType.DMA((S // CH,)),
            pltpu.SemaphoreType.DMA((9,)),
            pltpu.SemaphoreType.DMA((3 * G // NCV,)),
            pltpu.SemaphoreType.DMA((2,)),
        ],
        compiler_params=pltpu.CompilerParams(
            vmem_limit_bytes=110 * 1024 * 1024, disable_bounds_checks=True, disable_semaphore_checks=True),
    )(
        A_x.reshape(S, D),
        A_mem0.reshape(M, D),
        A_Wq.reshape(D // 2, 2, H, E),
        A_Wk.reshape(D // 2, 2, H, E),
        A_Wv.reshape(D // 2, 2, H, E),
        A_Wo.reshape(H * E, D),
        B_w1, B_w2, B_w3, B_w4,
    )
    return out.reshape(1, S, D)
```

```python
import jax
import jax.numpy as jnp
import jax.experimental.pallas as pl
import jax.experimental.pallas.tpu as pltpu

S, D, H, E, M, SEG, F = 2048, 1024, 32, 128, 8, 32, 3584
G = H // 2
L = M + SEG
PAIR = 2 * SEG
OB = 4 * SEG
NJ = S // OB
BR = 80
PRE = S - NJ * BR
CH = 256
CH2 = 512
CH3 = 128
NCV = 3 * G // (PRE // CH3)
NV = 2
NCH = 2
KC = 4
PLAN = (
    dict(wo=((0, 0), (0, 2), (0, 3)), cuts=(0, 0, 2, 13, 16), tail=(("u", 6), ("u", 4), None, None),
         end=("u", 3)),
    dict(wo=((0, 1), (1, 0), (1, 1), (1, 2), (1, 3)), cuts=(0, 5, 10, 15, 16), tail=(None,) * 4,
         end=("u", 2)),
    dict(wo=((2, 0), (2, 2), (2, 3)), cuts=(0, 0, 2, 13, 16), tail=(("u", 6), ("u", 4), None, None),
         end=("u", 3)),
    dict(wo=((2, 1), (3, 0), (3, 1), (3, 2), (3, 3)), cuts=(0, 5, 10, 15, 16), tail=(None,) * 4,
         end=("d", 8)),
)
EPS = 1e-5
LOG2E = 1.4426950408889634
F32 = jnp.float32
BF16 = jnp.bfloat16
U32 = jnp.uint32


def _ln(x, dep=None):
    m = jnp.sum(x, axis=-1, keepdims=True) * (1.0 / D)
    if dep is not None:
        m = m + dep
    xc = x - m
    v = jnp.sum(xc * xc, axis=-1, keepdims=True) * (1.0 / D)
    r = jax.lax.rsqrt(v + EPS)
    return xc * r, jnp.where(r < 0.0, 1.0, 0.0)


def _gelu(x):
    c1 = 0.7978845608028654
    c2 = c1 * 0.044715
    t = jnp.tanh(x * (c1 + c2 * (x * x)))
    hx = 0.5 * x
    return hx + hx * t


def _silu(x):
    hx = 0.5 * x
    return hx + hx * jnp.tanh(hx)


def _recip(l):
    r = pl.reciprocal(l, approx=True)
    return r * (2.0 - l * r)


def _w(packed):
    return pltpu.bitcast(packed, BF16)


def _kernel(x_hbm, mem_hbm, wq_hbm, wk_hbm, wv_hbm, wo_hbm, w1_hbm, w2_hbm, w3_hbm, w4_hbm,
            out_hbm,
            x_v, xn_v, h_v, x1_v, x1h_v, za_v, zb_v, zc_v, mem0_v, mem_v, s_v, o_stage, filla_v, fillb_v, kv_v, zero_v,
            wqkv_v, wo_v, w1_v, w2_v, w3_v, w4_v,
            sem_x, sem_w, sem_qkv, sem_o):
    scale = float(E) ** -0.5

    nch = S // CH
    q4 = D // 4
    x_cp = [pltpu.make_async_copy(x_hbm.at[pl.ds(c * CH, CH)], x_v.at[pl.ds(c * CH, CH)], sem_x.at[c])
            for c in range(nch)]
    w1_cp = [pltpu.make_async_copy(w1_hbm.bitcast(U32).at[:, pl.ds(q * q4, q4)],
                                   w1_v.at[:, pl.ds(q * q4, q4)], sem_w.at[q]) for q in range(4)]
    w2_cp = pltpu.make_async_copy(w2_hbm.bitcast(U32), w2_v, sem_w.at[4])
    w3_cp = pltpu.make_async_copy(w3_hbm.bitcast(U32), w3_v, sem_w.at[5])
    w4_cp = pltpu.make_async_copy(w4_hbm.bitcast(U32), w4_v, sem_w.at[6])
    wo_cp = pltpu.make_async_copy(wo_hbm.bitcast(U32), wo_v, sem_w.at[7])
    mem_cp = pltpu.make_async_copy(mem_hbm, mem0_v, sem_w.at[8])
    srcs = [w.bitcast(U32) for w in (wq_hbm, wk_hbm, wv_hbm)]

    def qkv_start(n0, n1):
        for n in range(n0, n1):
            for b in range(2):
                pltpu.make_async_copy(
                    srcs[n // G].at[:, b, n % G, :], wqkv_v.at[n, b], sem_qkv.at[n // NCV]).start()

    x_cp[0].start()
    w1_cp[0].start()
    x_cp[1].start()
    w1_cp[1].start()
    w1_cp[2].start()
    w1_cp[3].start()
    for c in range(2, nch):
        x_cp[c].start()
    w2_cp.start()
    mem_cp.start()
    w3_cp.start()
    w4_cp.start()
    qkv_start(0, 20)

    for ref, nblk in ((filla_v, NV), (fillb_v, 0)):
        lm = L - 8 * nblk
        r = jax.lax.broadcasted_iota(jnp.int32, (2 * lm, 2 * L), 0)
        c = jax.lax.broadcasted_iota(jnp.int32, (2 * lm, 2 * L), 1)
        same = (r < lm) == (c < L)
        rr = jnp.where(r < lm, r, r - lm)
        cc = jnp.where(c < L, c, c - L)
        ok = (rr < M) | (rr + 8 * nblk >= cc)
        ref[...] = jnp.where(same, jnp.where(ok, 0.0, -1e9), -jnp.inf).astype(F32)
    h_v[:, pl.ds(0, 8), :] = jnp.zeros((D // E, 8, E), F32)
    h_v[:, pl.ds(S + 8, 8), :] = jnp.zeros((D // E, 8, E), F32)

    def h_store(r0, c0, val):
        for i in range(val.shape[1] // E):
            h_v[c0 + i, pl.ds(r0, val.shape[0]), :] = val[:, i * E:(i + 1) * E]

    s_v[...] = jnp.zeros((OB, D), F32)
    x1h_v[...] = jnp.zeros((CH3, D), F32)
    zero_v[...] = jnp.zeros((8, E), U32)
    kv_v[:, :, pl.ds(0, 8), :] = jnp.zeros((G, 6, 8, E), F32)

    def norm_chunk(c, z_ref, paced):
        if not paced:
            xn = _ln(x_v[pl.ds(c * CH, CH), :].astype(F32))[0].astype(BF16).astype(F32)
            xn_v[pl.ds(c * CH, CH), :] = xn
            z_ref[...] = pltpu.bitcast(_ln(xn)[0].astype(BF16), U32)
            return
        deps = [None] * 4
        for t in range(CH // 16):
            r0 = pl.multiple_of(c * CH + t * 16, 16)
            xb = x_v[pl.ds(r0, 16), :].astype(F32)
            zs = []
            for b in (2 * t, 2 * t + 1):
                xn, mid = _ln(xb[(b % 2) * 8:(b % 2) * 8 + 8], deps[b % 4])
                deps[b + 1:] = [mid] * (3 - b) if b < 3 else deps[b + 1:]
                xn = xn.astype(BF16).astype(F32)
                xn_v[pl.ds(r0 + (b % 2) * 8, 8), :] = xn
                z, deps[b % 4] = _ln(xn)
                zs.append(z)
            z_ref[pl.ds(t * 8, 8), :] = pltpu.bitcast(jnp.concatenate(zs, axis=0).astype(BF16), U32)

    def x_wait(c):
        rows = pl.ds(pl.multiple_of(c * CH, CH), CH)
        pltpu.make_async_copy(x_hbm.at[rows], x_v.at[rows], sem_x.at[c]).wait()

    def up1(c, z_ref):
        r0 = pl.multiple_of(c * CH, CH)
        h_store(r0 + 8, 0, _gelu(jnp.dot(_w(z_ref[...]), _w(w1_v[...]), preferred_element_type=F32)))

    def up1q(c, z_ref, q, nq):
        w = _w(w1_v[:, pl.ds(q * q4, nq * q4)])
        h_store(c * CH + 8, 2 * q, _gelu(jnp.dot(_w(z_ref[...]), w, preferred_element_type=F32)))

    x_cp[0].wait()
    norm_chunk(0, zc_v, False)
    w1_cp[0].wait()
    up1q(0, zc_v, 0, 1)
    x_cp[1].wait()
    norm_chunk(1, zb_v, False)
    w1_cp[1].wait()
    up1q(1, zb_v, 0, 1)
    up1q(0, zc_v, 1, 1)
    up1q(1, zb_v, 1, 1)
    w1_cp[2].wait()
    w1_cp[3].wait()
    x_cp[2].wait()
    up1q(0, zc_v, 2, 2)
    up1q(1, zb_v, 2, 2)
    norm_chunk(2, za_v, True)

    def stage1(i, carry):
        cn = jnp.minimum(2 * i + 2, nch - 1)
        x_wait(2 * i + 1)

        @pl.when(2 * i + 2 < nch)
        def _():
            x_wait(cn)

        up1(2 * i, za_v)
        norm_chunk(2 * i + 1, zb_v, True)
        up1(2 * i + 1, zb_v)
        norm_chunk(cn, za_v, True)
        return carry

    jax.lax.fori_loop(1, nch // 2, stage1, 0)
    qkv_start(20, 36)

    w2_cp.wait()

    def norm3(src, r0, rb):
        dep = None
        for b in range(CH3 // rb):
            z, dep = _ln(src[pl.ds(pl.multiple_of(r0 + b * rb, rb), rb), :], dep)
            za_v[pl.ds(b * rb // 2, rb // 2), :] = pltpu.bitcast(z.astype(BF16), U32)

    def stage2(c, carry):
        norm3(x1h_v, 0, 16)
        r0 = pl.multiple_of(c * CH2, CH2)
        hs = jnp.concatenate([h_v[i, pl.ds(r0 + 8 + (-1, 1, -2, 2)[i // 2], CH2), :] for i in range(D // E)],
                             axis=1).astype(BF16)
        y = xn_v[pl.ds(r0, CH2), :] + jnp.dot(hs, _w(w2_v[...]), preferred_element_type=F32)
        x1_v[pl.ds(r0, CH2), :] = y
        x1h_v[...] = jnp.where(c == 0, y[:CH3], x1h_v[...])
        return carry

    jax.lax.fori_loop(0, S // CH2, stage2, 0)
    qkv_start(36, 48)
    wo_cp.start()

    w3_cp.wait()
    w4_cp.wait()

    def stage3(c, carry):
        blk = wqkv_v.at[pl.ds(c * NCV, NCV)]
        pltpu.make_async_copy(blk, blk, sem_qkv.at[c]).wait()
        r0 = pl.multiple_of(c * CH3, CH3)
        z = _w(za_v[pl.ds(0, CH3 // 2), :])
        h3 = _gelu(jnp.dot(z, _w(w3_v[...]), preferred_element_type=F32)).astype(BF16)
        zero = zero_v[...]
        dep = zero
        for i in range(NCV):
            n = c * NCV + i
            for r in range(0, D // 2, 8):
                a = wqkv_v[n, 0, pl.ds(r, 8), :] | dep
                b = wqkv_v[n, 1, pl.ds(r, 8), :]
                lo = (a & jnp.uint32(0xFFFF)) | (b << 16)
                wqkv_v[n, 0, pl.ds(r, 8), :] = lo
                wqkv_v[n, 1, pl.ds(r, 8), :] = (a >> 16) | (b & jnp.uint32(0xFFFF0000))
                dep = (((lo & zero) | zero) & zero | zero) & zero
        y = x1_v[pl.ds(r0, CH3), :] + jnp.dot(h3, _w(w4_v[...]), preferred_element_type=F32)
        h_store(r0, 0, _silu(y))
        norm3(x1_v, jnp.minimum(c + 1, PRE // CH3 - 1) * CH3, 16)
        return carry

    jax.lax.fori_loop(0, PRE // CH3, stage3, 0)
    wo_cp.wait()
    mem_cp.wait()
    mem_v[...] = mem0_v[...].astype(F32)

    def out_cp(t0, n):
        return pltpu.make_async_copy(o_stage.at[pl.ds(t0, n)], out_hbm.at[pl.ds(t0, n)], sem_o.at[0])

    def combine(t0, r0, n):
        gate = jnp.concatenate([h_v[i, pl.ds(t0, n), :] for i in range(D // E)], axis=1)
        o_stage[pl.ds(t0, n), :] = (
            x_v[pl.ds(t0, n), :].astype(F32) + s_v[pl.ds(r0, n), :] * gate).astype(BF16)

    def zero_of(x):
        return pltpu.bitcast(pltpu.bitcast(x, U32) & zero_v[...], F32)

    def anchor(s, vals):
        t = None
        for v in vals:
            w = pltpu.bitcast(v, U32)
            t = w if t is None else t | w
        zf = pltpu.bitcast(t & zero_v[...], F32)[:, :2 * L]
        return jnp.concatenate([s[:8] + zf, s[8:]], axis=0)

    def vpu_attn(g, h, b, dep):
        row = jax.lax.broadcasted_iota(jnp.int32, (8, 1), 0)
        i0 = M + 8 * b
        q = (kv_v[g, h, pl.ds(8 + i0, 8), :] + dep) * (scale * LOG2E)
        m = acc = l = None
        for d0 in range(i0, -8, -KC):
            ss = []
            for d in range(d0, d0 - KC, -1):
                t = jnp.sum(q * kv_v[g, 2 + h, pl.ds(8 + d, 8), :], axis=-1, keepdims=True)
                if d < 0:
                    t = jnp.where(row >= -d, t, -jnp.inf)
                ss.append(t)
            ms = ss
            while len(ms) > 1:
                ms = [jnp.maximum(ms[i], ms[i + 1]) for i in range(0, len(ms), 2)]
            if m is None:
                m = ms[0]
            else:
                mn = jnp.maximum(m, ms[0])
                a = jnp.exp2(m - mn)
                m, l, acc = mn, l * a, acc * a
            for i, t in enumerate(ss):
                e = jnp.exp2(t - m)
                t = e * kv_v[g, 4 + h, pl.ds(8 + d0 - i, 8), :]
                l = e if l is None else l + e
                acc = t if acc is None else acc + t
        return acc * _recip(l), zero_of(acc)

    def body(j, carry):
        tp = pl.multiple_of(jnp.maximum(j - 1, 0) * OB, OB)
        combine(tp, 0, OB)

        b0 = pl.multiple_of(PRE + j * BR, 16)
        x1 = x1_v[pl.ds(b0, BR), :]
        z = _ln(x1)[0].astype(BF16)
        h3 = []
        done = [0]

        def fill(spec):
            if spec is None:
                return
            kind, n = spec
            if kind == "u":
                c0 = len(h3) * E
                t = jnp.dot(z, _w(w3_v[:, c0:c0 + n * E]), preferred_element_type=F32)
                u = _gelu(t).astype(BF16)
                h3.extend(u[:, i * E:(i + 1) * E] for i in range(n))
            else:
                c0, c1 = done[0] * E, (done[0] + n) * E
                done[0] += n
                t = jnp.dot(jnp.concatenate(h3, axis=1), _w(w4_v[:, c0:c1]), preferred_element_type=F32)
                h_store(b0, c0 // E, _silu(x1[:, c0:c1] + t))

        o = [[[[None] * 4 for _ in range(2)] for _ in range(G)] for _ in range(4)]
        chain = []

        def get(seg, g, h, blk):
            if o[seg][g][h][blk] is None:
                o[seg][g][h][blk], dep = vpu_attn(g, h, blk, chain.pop(0))
                chain.append(dep)
            return o[seg][g][h][blk]

        def segment(seg, mem, qkv_extra):
            first = seg % 2 == 0
            plan = PLAN[seg]
            t0 = pl.multiple_of(j * OB + (seg // 2) * PAIR, PAIR)
            rows = xn_v[pl.ds(t0, 40), :] if first else xn_v[pl.ds(t0 + 40, 24), :]
            lhs = jnp.concatenate([mem, rows], axis=0).astype(BF16)
            nblk = NV if first else 0
            nv, lm = M + 8 * nblk, L - 8 * nblk
            qkv_left, qkv, sc, o_mem = ([None] * G for _ in range(4))
            chain[:] = [jnp.zeros((8, E), F32)] * NCH

            prev = [None]

            def do_qkv(g):
                ys = [jnp.dot(lhs, _w(wqkv_v[(c // 2) * G + g, c % 2]), preferred_element_type=F32)
                      for c in range(6)]
                if first:
                    qkv_left[g] = [y[L:] for y in ys]
                    ys = [y[:L] for y in ys]
                else:
                    ys = [jnp.concatenate([y[:M], e, y[M:]], axis=0) for y, e in zip(ys, qkv_extra[g])]
                for i in range(6 if nblk else 0):
                    lo = M if i < 2 else 0
                    kv_v[g, i, pl.ds(8 + lo, nv - lo), :] = ys[i][lo:nv]
                qm = jnp.concatenate([ys[0][:M], ys[0][nv:], ys[1][:M], ys[1][nv:]], axis=0).astype(BF16)
                qkv[g] = [qm] + [jnp.concatenate(ys[c:c + 2], axis=0).astype(BF16) for c in (2, 4)]

            def do_s(g):
                q, k, _ = qkv[g]
                s = jax.lax.dot_general(q, k, (((1,), (1,)), ((), ())), preferred_element_type=F32)
                fl = (filla_v if first else fillb_v)[...]
                s = jnp.where(fl == 0.0, s * scale, fl)
                lag = 4 if first else 8
                vals = []
                if g >= lag:
                    vals += [o_mem[g - lag][h] for h in range(2)]
                    vals += [o[seg][g - lag][h][b] for h in range(2) for b in range(nblk, 4)]
                if first and g >= 1:
                    vals += [get(seg, g - 1, h, b) for b in range(nblk) for h in range(2)]
                if vals:
                    s = anchor(s, vals)
                mx = jnp.max(s if prev[0] is None else s + prev[0], axis=-1, keepdims=True)
                e = jnp.exp(s - mx)
                l = jnp.sum(e, axis=-1, keepdims=True)
                prev[0] = None if first or g % 4 == 2 else jnp.where(l > jnp.inf, 1.0, 0.0)
                sc[g] = (e.astype(BF16), _recip(l))

            def do_pv(g):
                e, rl = sc[g]
                t = jnp.dot(e, qkv[g][2], preferred_element_type=F32) * rl
                o_mem[g] = [t[h * lm:h * lm + M] for h in range(2)]
                for h in range(2):
                    for b in range(nblk, 4):
                        r = h * lm + M + 8 * (b - nblk)
                        o[seg][g][h][b] = t[r:r + 8]

            acc = [None]

            def part(i):
                fill(plan["tail"][i])
                g0, g1 = plan["cuts"][i:i + 2]
                if g0 < g1:
                    a = jnp.concatenate(
                        [jnp.concatenate([o_mem[g][h]] + [get(sg, g, h, b) for sg, b in plan["wo"]], axis=0)
                         for g in range(g0, g1) for h in range(2)], axis=1).astype(BF16)
                    t = jnp.dot(a, _w(wo_v[g0 * E:g1 * E, :]), preferred_element_type=F32)
                    acc[0] = t if acc[0] is None else t + acc[0]

            nb = 2 if first else 4
            for g in range(0, G, nb):
                for i in range(nb):
                    do_qkv(g + i)
                for f, i in ([(do_pv, g - nb - 1 + i) for i in range(nb)]
                             + [(do_s, g - 1 + i) for i in range(nb)]):
                    if i >= 0:
                        f(i)
            part(0)
            do_s(G - 1)
            for i in range(nb):
                do_pv(G - 1 - nb + i)
            part(1)
            do_pv(G - 1)
            part(2)
            part(3)
            for i, (sg, b) in enumerate(plan["wo"]):
                s_v[pl.ds(sg * SEG + 8 * b, 8), :] = acc[0][M + 8 * i:M + 8 * i + 8]
            fill(plan["end"])
            return acc[0][:M].astype(BF16).astype(F32), qkv_left

        mem = mem_v[...]
        left = None
        for seg in range(4):
            mem, left = segment(seg, mem, left)
        assert len(h3) == F // E and done[0] == D // E
        mem_v[...] = mem

        @pl.when(j >= 1)
        def _():
            out_cp(tp, OB).start()

        return carry

    jax.lax.fori_loop(0, NJ, body, 0)
    for r in range(0, OB, SEG):
        combine(S - OB + r, r, SEG)
        out_cp(S - OB + r, SEG).start()
    pltpu.make_async_copy(o_stage, out_hbm, sem_o.at[0]).wait()


@jax.jit
def pallas_recurrent_scan__memory_aug_recurrent_mem_tr__mixer_s_mlp__prompt_kernel(
    A_x: jax.Array,
    A_mem0: jax.Array,
    A_Wq: jax.Array,
    A_Wk: jax.Array,
    A_Wv: jax.Array,
    A_Wo: jax.Array,
    A_seg_len: jax.Array,
    B_x: jax.Array,
    B_w1: jax.Array,
    B_w2: jax.Array,
    B_w3: jax.Array,
    B_w4: jax.Array,
):
    del A_seg_len, B_x
    assert A_x.shape == (1, S, D) and A_mem0.shape == (1, M, D) and A_Wq.shape == (D, H, E)
    assert B_w3.shape == (D, F)
    any_spec = pl.BlockSpec(memory_space=pl.ANY)
    out = pl.pallas_call(
        _kernel,
        out_shape=jax.ShapeDtypeStruct((S, D), BF16),
        in_specs=[any_spec] * 10,
        out_specs=any_spec,
        scratch_shapes=[
            pltpu.VMEM((S, D), BF16),
            pltpu.VMEM((S, D), F32),
            pltpu.VMEM((D // E, S + 16, E), F32),
            pltpu.VMEM((S, D), F32),
            pltpu.VMEM((CH3, D), F32),
            pltpu.VMEM((CH // 2, D), U32),
            pltpu.VMEM((CH // 2, D), U32),
            pltpu.VMEM((CH // 2, D), U32),
            pltpu.VMEM((M, D), BF16),
            pltpu.VMEM((M, D), F32),
            pltpu.VMEM((OB, D), F32),
            pltpu.VMEM((S, D), BF16),
            pltpu.VMEM((2 * (L - 8 * NV), 2 * L), F32),
            pltpu.VMEM((2 * L, 2 * L), F32),
            pltpu.VMEM((G, 6, 16 + M + 8 * NV, E), F32),
            pltpu.VMEM((8, E), U32),
            pltpu.VMEM((3 * G, 2, D // 2, E), U32),
            pltpu.VMEM((H * E // 2, D), U32),
            pltpu.VMEM((D // 2, D), U32),
            pltpu.VMEM((D // 2, D), U32),
            pltpu.VMEM((D // 2, F), U32),
            pltpu.VMEM((F // 2, D), U32),
            pltpu.SemaphoreType.DMA((S // CH,)),
            pltpu.SemaphoreType.DMA((9,)),
            pltpu.SemaphoreType.DMA((3 * G // NCV,)),
            pltpu.SemaphoreType.DMA((1,)),
        ],
        compiler_params=pltpu.CompilerParams(
            vmem_limit_bytes=110 * 1024 * 1024, disable_bounds_checks=True, disable_semaphore_checks=True),
    )(
        A_x.reshape(S, D),
        A_mem0.reshape(M, D),
        A_Wq.reshape(D // 2, 2, H, E),
        A_Wk.reshape(D // 2, 2, H, E),
        A_Wv.reshape(D // 2, 2, H, E),
        A_Wo.reshape(H * E, D),
        B_w1, B_w2, B_w3, B_w4,
    )
    return out.reshape(1, S, D)
```
